```python
import jax
import jax.numpy as jnp

def _softmax(x, axis=-1):
    return jax.nn.softmax(x, axis=axis)

def _gelu(x):
    return jax.nn.gelu(x, approximate=True)

def _silu(x):
    return jax.nn.silu(x)

def _sigmoid(x):
    return jax.nn.sigmoid(x)

def _layernorm(x, axis=-1, eps=1e-05):
    m = jnp.mean(x, axis=axis, keepdims=True)
    v = jnp.var(x, axis=axis, keepdims=True)
    return (x - m) / jnp.sqrt(v + eps)

def _scatter_add(tgt, idx, src, axis=0):
    return tgt.at[idx].add(src)

def _segment_sum(src, seg, n):
    return jax.ops.segment_sum(src, seg, n)

class _Rng:

    def __init__(self, key):
        self._k = key

    def _next(self):
        self._k, sub = jax.random.split(self._k)
        return sub

    def normal(self, shape):
        return jax.random.normal(self._next(), shape, dtype=jnp.bfloat16)

    def randint(self, lo, hi, shape):
        return jax.random.randint(self._next(), shape, lo, hi, dtype=jnp.int32)

    def uniform(self, shape, lo=0.0, hi=1.0):
        return jax.random.uniform(self._next(), shape, jnp.bfloat16, lo, hi)

    def permutation(self, n):
        return jax.random.permutation(self._next(), n)
kernel_name = 'adaLN_cond__spectral_gfnet__mixer_token_mlp__prompt'

def setup_inputs():
    _rng = _Rng(jax.random.key(int.from_bytes(__import__("os").urandom(4), "little")))
    _w = lambda a: (lambda t: t.astype(jnp.bfloat16) if jnp.issubdtype(t.dtype, jnp.floating) else t)(jnp.asarray(a))

    def _A_setup():
        B, S, D = (1, 2048, 576)
        Df = D // 2 + 1
        return {'x': _w((lambda *s: _rng.normal(s) * 0.05)(B, S, D)), 'w_r': _w((lambda *s: _rng.normal(s) * 0.05)(S, Df) * 0.02), 'w_i': _w((lambda *s: _rng.normal(s) * 0.05)(S, Df) * 0.02)}
    _A_in = _A_setup()

    def _B_setup():
        B, S, D, F = (1, 2048, 576, 4608)
        return {'x': _w((lambda *s: _rng.normal(s) * 0.05)(B, S, D)), 'w1': _w((lambda *s: _rng.normal(s) * 0.05)(S, F) * S ** (-0.5)), 'b1': _w((lambda *s: _rng.normal(s) * 0.05)(F) * 0.02), 'w2': _w((lambda *s: _rng.normal(s) * 0.05)(F, S) * F ** (-0.5)), 'b2': _w((lambda *s: _rng.normal(s) * 0.05)(S) * 0.02)}
    _B_in = _B_setup()
    return {'A_x': _A_in['x'], 'A_w_r': _A_in['w_r'], 'A_w_i': _A_in['w_i'], 'B_x': _B_in['x'], 'B_w1': _B_in['w1'], 'B_b1': _B_in['b1'], 'B_w2': _B_in['w2'], 'B_b2': _B_in['b2'], 'c': _w((lambda *s: _rng.normal(s) * 0.05)(1, 576)), 'w_mod': _w((lambda *s: _rng.normal(s) * 0.05)(576, 6 * 576) * 576 ** (-0.5))}

def reference(A_x, A_w_r, A_w_i, B_x, B_w1, B_b1, B_w2, B_b2, c, w_mod):

    def _A_ref(x, w_r, w_i):
        B, S, D = x.shape
        X = (lambda x, axes=(-2, -1): jnp.fft.rfft2(x.astype(jnp.float32), axes=axes))(x, axes=(-2, -1))
        W = w_r + 1j * w_i
        X = X * W
        y = (lambda x, s, axes=(-2, -1): jnp.fft.irfft2(x, s=s, axes=axes).astype(jnp.bfloat16))(X, (S, D), axes=(-2, -1))
        return y

    def _B_ref(x, w1, b1, w2, b2):
        B, S, D = x.shape
        h = _layernorm(x, axis=-1)
        u = jnp.einsum('bsd,sf->bdf', h, w1) + b1
        u = _gelu(u)
        y = jnp.einsum('bdf,fs->bds', u, w2) + b2
        return (lambda x, *d: x.transpose(*d))(y, 0, 2, 1)
    x = A_x
    mod = (_silu(c) @ w_mod).reshape(c.shape[0], 6, 1, -1)
    sa, ca, ga, sb, cb, gb = (mod[:, 0].copy(), mod[:, 1].copy(), mod[:, 2].copy(), mod[:, 3].copy(), mod[:, 4].copy(), mod[:, 5].copy())
    h = _layernorm(x, axis=-1) * (1 + ca) + sa
    x = x + ga * _A_ref(h, A_w_r, A_w_i)
    h = _layernorm(x, axis=-1) * (1 + cb) + sb
    x = x + gb * _B_ref(h, B_w1, B_b1, B_w2, B_b2)
    return x
```

```python
import jax
import jax.numpy as jnp
import numpy as np
from jax import lax
from jax.experimental import pallas as pl
from jax.experimental.pallas import tpu as pltpu

D, S, F = 576, 2048, 4608
DF = D // 2 + 1
NT = S // 128
NRB = 37
EPS = 1e-5
TF = 512
NCH = F // TF
XCH = 4

f32, bf16, u32 = jnp.float32, jnp.bfloat16, jnp.uint32

_Q = np.sqrt(3.0) / 2
_C1, _C2, _C4 = (float(np.cos(2 * np.pi * k / 9)) for k in (1, 2, 4))
_S1, _S2, _S4 = (float(np.sin(2 * np.pi * k / 9) / _Q) for k in (1, 2, 4))


def _row_runs():
    runs = []
    for g in (1, 2, 3, 4):
        for r in (g, 9 - g):
            runs += [r, r + 9]
    return runs + [0, 9]


def _channel_mats():
    kd_all = [k0 + 18 * j for k0 in _row_runs() for j in range(16)] + [D // 2] + [-1] * 7
    kd_all = np.array(kd_all)
    b = np.arange(64)
    mats = np.zeros((10, 128, 128))
    for g in (1, 2, 3, 4):
        kd = kd_all[64 * (g - 1):64 * g]
        sg = np.where(kd % 9 == g, -1.0, 1.0).reshape(8, 8, 1, 1)
        th = (2 * np.pi / D) * ((kd[:, None] * b[None, :]) % D)
        c, s = np.cos(th).reshape(8, 8, 8, 8), np.sin(th).reshape(8, 8, 8, 8)
        m = np.zeros((8, 2, 8, 8, 2, 8))
        m[:, 0, :, :, 0, :] = c
        m[:, 0, :, :, 1, :] = sg * _Q * s
        m[:, 1, :, :, 0, :] = -s
        m[:, 1, :, :, 1, :] = sg * _Q * c
        mats[g - 1] = m.reshape(128, 128)
        mats[4 + g - 1] = m.reshape(128, 128).T
    kd = kd_all[256:]
    valid = (kd >= 0)[:, None]
    th = (2 * np.pi / D) * ((kd[:, None] * b[None, :]) % D)
    m = np.zeros((5, 2, 8, 64))
    m[:, 0] = (np.cos(th) * valid).reshape(5, 8, 64)
    m[:, 1] = (-np.sin(th) * valid * (kd != D // 2)[:, None]).reshape(5, 8, 64)
    half = np.where((kd == 0) | (kd == D // 2), 0.5, 1.0).reshape(5, 1, 8, 1)
    mats[8, :80, :64] = m.reshape(80, 64)
    mats[9, :64, :80] = (m * half).reshape(80, 64).T
    return mats.astype(np.float32).astype(jnp.bfloat16)


def _token_tables():
    l = np.arange(128)
    ph = (2 * np.pi / 128) * ((l[:, None] * l[None, :]) % 128)
    tw = (2 * np.pi / S) * l
    ones = np.ones((128, 1))
    parts = [np.cos(ph), -np.sin(ph),
             np.cos(tw)[:, None] * ones.T, -np.sin(tw)[:, None] * ones.T,
             ones[:8] * np.cos(tw)[None, :], -ones[:8] * np.sin(tw)[None, :]]
    return np.concatenate(parts, axis=0).astype(np.float32)


_CH_MATS = _channel_mats()
_TOK_TAB = _token_tables()


def _dot(a, b):
    return jnp.dot(a, b, preferred_element_type=f32)


def _radix9(x):
    s1, s2, s3, s4 = x[1] + x[8], x[2] + x[7], x[3] + x[6], x[4] + x[5]
    d1, d2, d3, d4 = x[1] - x[8], x[2] - x[7], x[3] - x[6], x[4] - x[5]
    p = x[0] - 0.5 * s3
    a, b = s1 - s4, s2 - s4
    r1 = _C1 * a + _C2 * b
    r2 = _C2 * a + _C4 * b
    e, g = d1 + d2, d2 + d4
    i1 = _S1 * e + _S4 * g
    i2 = _S2 * e - _S1 * g
    t, u = s1 + s2 + s4, x[0] + s3
    return u + t, [(p + r1, i1 + d3), (p + r2, i2 - d3),
                   (u - 0.5 * t, d1 - d2 + d4), ((p - r1) - r2, (i2 - i1) + d3)]


def _radix9_t(x0, uv):
    (u1, v1), (u2, v2), (u3, v3), (u4, v4) = uv
    u, t = x0 + u3, x0 - 0.5 * u3
    p, r1, r2 = u1 + u2 + u4, u1 - u4, u2 - u4
    a = _C1 * r1 + _C2 * r2
    b = _C2 * r1 + _C4 * r2
    s1, s2, s3, s4 = t + a, t + b, u - 0.5 * p, (t - a) - b
    i1, i2, d3 = v1 - v4, v2 + v4, v1 - v2 + v4
    e = _S1 * i1 + _S2 * i2
    g = _S4 * i1 - _S1 * i2
    d1, d2, d4 = e + v3, (e + g) - v3, g + v3
    return [u + p, s1 + d1, s2 + d2, s3 + d3, s4 + d4, s4 - d4, s3 - d3, s2 - d2, s1 - d1]


def _radix4(x, sign):
    (ar, ai), (br, bi), (cr, ci), (dr, di) = x
    pr, pi, mr, mi = ar + cr, ai + ci, ar - cr, ai - ci
    qr, qi, nr, ni = br + dr, bi + di, br - dr, bi - di
    plus, minus = (mr - ni, mi + nr), (mr + ni, mi - nr)
    k1, k3 = (plus, minus) if sign > 0 else (minus, plus)
    return [(pr + qr, pi + qi), k1, (pr - qr, pi - qi), k3]


def _twiddle16(z, e, sign):
    re, im = z
    if e == 0:
        return z
    c, s = float(np.cos(2 * np.pi * e / 16)), float(sign * np.sin(2 * np.pi * e / 16))
    if e == 4:
        return (-im, re) if sign > 0 else (im, -re)
    if e % 2 == 0:
        if c * s > 0:
            return c * (re - im), c * (re + im)
        return c * (re + im), c * (im - re)
    return c * re - s * im, s * re + c * im


def _radix16(x, sign):
    y = [_radix4(x[t0::4], sign) for t0 in range(4)]
    out = [None] * 16
    for q0 in range(4):
        col = _radix4([_twiddle16(y[t0][q0], t0 * q0, sign) for t0 in range(4)], sign)
        for q1 in range(4):
            out[q0 + 4 * q1] = col[q1]
    return out


def _pair(a, b):
    return jnp.concatenate([a, b], axis=0).astype(bf16)


def _split(z):
    z = z.reshape(NRB, 16, 128)
    return z[:, :8, :], z[:, 8:, :]


def _merge(re, im):
    return jnp.concatenate([re, im], axis=1).reshape(NRB * 16, 128)


def _normalize(x):
    m = jnp.sum(x, axis=0, keepdims=True) * (1.0 / D)
    xc = x - m
    v = jnp.sum(xc * xc, axis=0, keepdims=True) * (1.0 / D)
    return xc * lax.rsqrt(v + EPS)


def _gelu(x):
    inner = x * (0.7978845608028654 + (0.7978845608028654 * 0.044715) * (x * x))
    hx = 0.5 * x
    return hx + hx * jnp.tanh(inner)


def _lhs_forms(a11, a12, a21, a22):
    return [a11 + a22, a21 + a22, a11, a22, a11 + a12, a21 - a11, a12 - a22]


def _rhs_forms(b11, b12, b21, b22):
    f11, f12, f21, f22 = (b.astype(f32) for b in (b11, b12, b21, b22))
    return [(f11 + f22).astype(bf16), b11, (f12 - f22).astype(bf16), (f21 - f11).astype(bf16),
            b22, (f11 + f12).astype(bf16), (f21 + f22).astype(bf16)]


def _out_forms(m):
    return m[0] + m[3] - m[4] + m[6], m[2] + m[4], m[1] + m[3], m[0] - m[1] + m[2] + m[5]


def _kernel(x_hbm, wr_hbm, wi_hbm, w1_hbm, b1_hbm, w2_hbm, b2_hbm, c_hbm, wm_hbm, chm_hbm, tok_hbm,
            o_hbm,
            x_v, wr_v, wi_v, w1_v, b1_v, w2_v, b2_v, c_v, wma_v, wmb_v, chm_v, tok_v,
            mod_v, mf_v, mi_v, wt_v, wp_v, fa_v, fb_v, x1_v, a_v, acc_v, o_v,
            sem_in, sem_x, sem_w1, sem_w2, sem_o):
    xw = S // XCH
    small = [
        (c_hbm, c_v), (wm_hbm.at[:, pl.ds(0, 2 * D)], wma_v), (tok_hbm, tok_v), (chm_hbm, chm_v),
        (wr_hbm, wr_v), (wi_hbm, wi_v), (wm_hbm.at[:, pl.ds(2 * D, 4 * D)], wmb_v),
        (b1_hbm, b1_v), (b2_hbm, b2_v),
    ]
    cp = [pltpu.make_async_copy(s, d, sem_in.at[i]) for i, (s, d) in enumerate(small)]
    cp_c, cp_wma, cp_tok, cp_chm, cp_wr, cp_wi, cp_wmb, cp_b1, cp_b2 = cp
    cp_x = [pltpu.make_async_copy(x_hbm.at[:, pl.ds(i * xw, xw)], x_v.at[:, pl.ds(i * xw, xw)],
                                  sem_x.at[i]) for i in range(XCH)]

    def cp_w1(j):
        return pltpu.make_async_copy(w1_hbm.at[:, pl.ds(j * TF, TF)], w1_v.at[j], sem_w1.at[j])

    def cp_w2(j):
        return pltpu.make_async_copy(w2_hbm.at[pl.ds(j * TF, TF), :], w2_v.at[j], sem_w2.at[j])

    for c in (cp_c, cp_tok, cp_wma, cp_chm, *cp_x, cp_wr, cp_wi, cp_wmb, cp_b1, cp_b2):
        c.start()

    def lanes(t):
        return pl.ds(pl.multiple_of(t * 128, 128), 128)

    cp_tok.wait()
    tcr, tci = tok_v[256:384, :], tok_v[384:512, :]
    trr, tri = tok_v[512:513, :], tok_v[520:521, :]

    def gen(k, carry):
        ar, ai, br, bi = carry
        mf_v[k, :, 0:128] = ar.astype(bf16)
        mf_v[k, :, 128:256] = ai.astype(bf16)
        mi_v[k, :, 0:128] = br.astype(bf16)
        mi_v[k, :, 128:256] = bi.astype(bf16)
        return (ar * tcr - ai * tci, ar * tci + ai * tcr, br * trr - bi * tri, br * tri + bi * trr)

    fr, fi = tok_v[0:128, :], tok_v[128:256, :]
    lax.fori_loop(0, NT, gen, (fr, fi, fr, fi))

    cp_c.wait()
    cf = c_v[...].astype(f32)
    sc = jnp.broadcast_to(cf * jax.nn.sigmoid(cf), (16, D)).astype(bf16)

    def store_mod(w_ref, first):
        row = _dot(sc, w_ref[...])[0:8, :]
        n = first + lax.broadcasted_iota(jnp.int32, row.shape, 1)
        scale = jnp.logical_or(jnp.logical_and(n >= D, n < 2 * D),
                               jnp.logical_and(n >= 4 * D, n < 5 * D))
        row = jnp.where(scale, row + 1.0, row)
        row = jnp.where(jnp.logical_and(n >= 2 * D, n < 3 * D), row * (2.0 / (S * D)), row)
        for j in range(row.shape[1] // 128):
            tile = jnp.concatenate([row[:, 128 * j:128 * (j + 1)]] * 16, axis=0)
            mod_v[pl.ds(first + 128 * j, 128), :] = tile.T

    def mod(i):
        return mod_v[pl.ds(i * D, D), :]

    cp_wma.wait()
    store_mod(wma_v, 0)

    cp_chm.wait()
    zeros64 = jnp.zeros((64, 128), bf16)

    def fwd_channel(t, _):
        h = _normalize(x_v[:, lanes(t)].astype(f32)) * mod(1) + mod(0)
        dc, groups = [], [[], [], [], []]
        for p in range(8):
            x0, uv = _radix9([h[64 * a + 8 * p:64 * a + 8 * p + 8, :] for a in range(9)])
            dc.append(x0)
            for g in range(4):
                groups[g].append(_pair(*uv[g]))
        for g in range(4):
            fa_v[t, pl.ds(128 * g, 128), :] = _dot(chm_v[g], jnp.concatenate(groups[g], axis=0))
        rhs = jnp.concatenate([jnp.concatenate(dc, axis=0).astype(bf16), zeros64], axis=0)
        fa_v[t, pl.ds(512, 80), :] = _dot(chm_v[8, 0:80, :], rhs)

    per = NT // XCH
    for i in range(XCH):
        cp_x[i].wait()
        lax.fori_loop(i * per, (i + 1) * per, fwd_channel, None)

    cp_w1(0).start()
    cp_w2(0).start()

    cp_wr.wait()
    cp_wi.wait()

    def filt_a(t, _):
        a = pltpu.bitcast(wr_v[0:DF - 1, lanes(t)], f32)
        b = pltpu.bitcast(wi_v[0:DF - 1, lanes(t)], f32)
        nr = wr_v[DF - 1:DF, lanes(t)].astype(f32)
        ni = wi_v[DF - 1:DF, lanes(t)].astype(f32)
        r = lax.broadcasted_iota(jnp.int32, (8, 128), 0)
        nyq = jnp.where(r == 0, nr, jnp.where(r == 1, ni, 0.0))
        rest = jnp.concatenate([a[128:], b[128:], nyq, jnp.zeros((88, 128), f32)], axis=0)
        wt_v[0, lanes(t), :] = a[:128].T
        wt_v[1, lanes(t), :] = b[:128].T
        wt_v[2, lanes(t), :] = rest.T

    def filt_b(k, _):
        wp_v[k, 0:128, :] = wt_v[0, pl.ds(k, 128, stride=NT), :].T
        wp_v[k, 144:272, :] = wt_v[1, pl.ds(k, 128, stride=NT), :].T
        rest = wt_v[2, pl.ds(k, 128, stride=NT), :].T
        wp_v[k, 128:144, :] = rest[0:16]
        wp_v[k, 272:296, :] = rest[16:40]

    lax.fori_loop(0, NT, filt_a, None)
    lax.fori_loop(0, NT, filt_b, None)

    def filt(k, base, nyq_row):
        parts = []
        for k0 in _row_runs():
            w = pltpu.bitcast(wp_v[k, pl.ds(base + k0 // 2, 16, stride=9), :], u32)
            w = (w & np.uint32(0xFFFF0000)) if k0 % 2 else (w << 16)
            parts.append(pltpu.bitcast(w, f32))
        parts.append(jnp.broadcast_to(wp_v[k, nyq_row:nyq_row + 1, :], (8, 128)))
        return jnp.concatenate(parts, axis=0).reshape(NRB, 8, 128)

    def butterflies(sign):
        def body(rb, _):
            r = pl.multiple_of(rb * 16, 16)
            z = [(fa_v[t, pl.ds(r, 8), :], fa_v[t, pl.ds(r + 8, 8), :]) for t in range(NT)]
            for k, (re, im) in enumerate(_radix16(z, sign)):
                fb_v[k, pl.ds(r, 16), :] = _pair(re, im)
        return body

    lax.fori_loop(0, NRB, butterflies(-1), None)

    def spectral(k, _):
        y = _dot(fb_v[k], mf_v[k])
        (pr, pi), (qr, qi) = _split(y[:, :128]), _split(y[:, 128:])
        yr, yi = pr - qi, qr + pi
        wr, wi = filt(k, 0, 288), filt(k, 144, 289)
        z = _merge(yr * wr - yi * wi, yr * wi + yi * wr).astype(bf16)
        v = _dot(z, mi_v[k])
        (pr, pi), (qr, qi) = _split(v[:, :128]), _split(v[:, 128:])
        fa_v[k] = _merge(pr + qi, pi - qr)

    lax.fori_loop(0, NT, spectral, None)
    lax.fori_loop(0, NRB, butterflies(+1), None)

    cp_wmb.wait()
    store_mod(wmb_v, 2 * D)
    for j in range(1, NCH):
        cp_w1(j).start()
        cp_w2(j).start()
    zeros48 = jnp.zeros((48, 128), bf16)
    hd = D // 2

    def inv_channel(t):
        ch = [_dot(chm_v[4 + g], fb_v[t, pl.ds(128 * g, 128), :]) for g in range(4)]
        dc = _dot(chm_v[9, 0:64, :], jnp.concatenate([fb_v[t, pl.ds(512, 80), :], zeros48], axis=0))
        blocks = [[] for _ in range(9)]
        for p in range(8):
            uv = [(c[16 * p:16 * p + 8], c[16 * p + 8:16 * p + 16]) for c in ch]
            for a, y in enumerate(_radix9_t(dc[8 * p:8 * p + 8], uv)):
                blocks[a].append(y)
        y = jnp.concatenate([b for blk in blocks for b in blk], axis=0)
        x1 = x_v[:, lanes(t)].astype(f32) + mod(2) * y
        x1_v[t] = x1
        return _normalize(_normalize(x1) * mod(4) + mod(3))

    def norm_pair(j, _):
        lo, hi = inv_channel(j), inv_channel(j + NT // 2)
        for i, a in enumerate(_lhs_forms(lo[:hd], hi[:hd], lo[hd:], hi[hd:])):
            a_v[i, :, lanes(j)] = a.astype(bf16)

    lax.fori_loop(0, NT // 2, norm_pair, None)

    cp_b1.wait()
    cp_b2.wait()
    hs, hf = S // 2, TF // 2
    acc_v[...] = jnp.zeros(acc_v.shape, f32)

    def chunk(j, _):
        cp_w1(j).wait()
        cp_w2(j).wait()
        rhs = _rhs_forms(w1_v[j, :hs, :hf], w1_v[j, :hs, hf:], w1_v[j, hs:, :hf], w1_v[j, hs:, hf:])
        u11, u12, u21, u22 = _out_forms([_dot(a_v[i], rhs[i]) for i in range(7)])
        nb = TF // 128
        bias = [b1_f[pl.ds(j * nb + i, 1), :] for i in range(nb)]
        bl = jnp.concatenate(bias[:nb // 2], axis=1)
        br = jnp.concatenate(bias[nb // 2:], axis=1)
        lhs = _lhs_forms(_gelu(u11 + bl), _gelu(u12 + br), _gelu(u21 + bl), _gelu(u22 + br))
        rhs = _rhs_forms(w2_v[j, :hf, :hs], w2_v[j, :hf, hs:], w2_v[j, hf:, :hs], w2_v[j, hf:, hs:])
        for i in range(7):
            acc_v[i] += _dot(lhs[i].astype(bf16), rhs[i])

    b1_f = tok_v.at[pl.ds(0, 40), :]
    b1_f[0:F // 128, :] = b1_v[...].astype(f32)
    lax.fori_loop(0, NCH, chunk, None)

    b2 = b2_v[...].astype(f32)
    gate = mod(5)
    for j in range(NT // 2):
        y11, y12, y21, y22 = _out_forms([acc_v[i, :, 128 * j:128 * (j + 1)] for i in range(7)])
        for t, top, bot in ((j, y11, y21), (j + NT // 2, y12, y22)):
            y = jnp.concatenate([top, bot], axis=0) + b2[t:t + 1, :]
            o_v[:, 128 * t:128 * (t + 1)] = (x1_v[t] + gate * y).astype(bf16)
    cp_o = pltpu.make_async_copy(o_v, o_hbm, sem_o.at[0])
    cp_o.start()
    cp_o.wait()


@jax.jit
def pallas_adaLN_cond__spectral_gfnet__mixer_token_mlp__prompt_kernel(
    A_x: jax.Array,
    A_w_r: jax.Array,
    A_w_i: jax.Array,
    B_x: jax.Array,
    B_w1: jax.Array,
    B_b1: jax.Array,
    B_w2: jax.Array,
    B_b2: jax.Array,
    c: jax.Array,
    w_mod: jax.Array,
):
    del B_x
    vmem = pltpu.VMEM
    scratch = [
        vmem((D, S), bf16), vmem((DF, S), bf16), vmem((DF, S), bf16),
        vmem((NCH, S, TF), bf16), vmem((F // 128, 128), bf16),
        vmem((NCH, TF, S), bf16), vmem((S // 128, 128), bf16),
        vmem((1, D), bf16), vmem((D, 2 * D), bf16), vmem((D, 4 * D), bf16),
        vmem(_CH_MATS.shape, bf16), vmem(_TOK_TAB.shape, f32),
        vmem((6 * D, 128), f32),
        vmem((NT, 128, 256), bf16),
        vmem((NT, 128, 256), bf16),
        vmem((3, S, 128), f32),
        vmem((NT, 296, 128), f32),
        vmem((NT, NRB * 16, 128), f32),
        vmem((NT, NRB * 16, 128), bf16),
        vmem((NT, D, 128), f32),
        vmem((7, D // 2, S // 2), bf16),
        vmem((7, D // 2, S // 2), f32),
        vmem((D, S), bf16),
        pltpu.SemaphoreType.DMA((9,)), pltpu.SemaphoreType.DMA((XCH,)),
        pltpu.SemaphoreType.DMA((NCH,)), pltpu.SemaphoreType.DMA((NCH,)),
        pltpu.SemaphoreType.DMA((XCH,)),
    ]
    out = pl.pallas_call(
        _kernel,
        in_specs=[pl.BlockSpec(memory_space=pl.ANY)] * 11,
        out_specs=pl.BlockSpec(memory_space=pl.ANY),
        out_shape=jax.ShapeDtypeStruct((D, S), bf16),
        scratch_shapes=scratch,
        compiler_params=pltpu.CompilerParams(vmem_limit_bytes=120 * 1024 * 1024),
    )(A_x[0].T, A_w_r.T, A_w_i.T, B_w1, B_b1.reshape(F // 128, 128), B_w2,
      B_b2.reshape(S // 128, 128), c, w_mod, _CH_MATS, _TOK_TAB)
    return out.T[None]
```

```python
import itertools

import jax
import jax.numpy as jnp
import numpy as np
from jax import lax
from jax.experimental import pallas as pl
from jax.experimental.pallas import tpu as pltpu

D, S, F = 576, 2048, 4608
DF = D // 2 + 1
NT = S // 128
NRB = 37
EPS = 1e-5
TF = 512
NCH = F // TF
WCH = 4
OCH = 4
MOD_PARTS = ((0, 9), (9, 23), (23, 27))

f32, bf16, u32 = jnp.float32, jnp.bfloat16, jnp.uint32

_Q = np.sqrt(3.0) / 2
_C1, _C2, _C4 = (float(np.cos(2 * np.pi * k / 9)) for k in (1, 2, 4))
_S1, _S2, _S4 = (float(np.sin(2 * np.pi * k / 9) / _Q) for k in (1, 2, 4))


def _row_runs():
    runs = []
    for g in (1, 2, 3, 4):
        for r in (g, 9 - g):
            runs += [r, r + 9]
    return runs + [0, 9]


def _pack_rows(m):
    b = m.astype(np.float32).astype(jnp.bfloat16).view(np.uint16).astype(np.uint32)
    return b[..., 0::2, :] | (b[..., 1::2, :] << np.uint32(16))


def _channel_mats():
    kd_all = [k0 + 18 * j for k0 in _row_runs() for j in range(16)] + [D // 2] + [-1] * 7
    kd_all = np.array(kd_all)
    b = np.arange(64)
    mats = np.zeros((10, 128, 128))
    for g in (1, 2, 3, 4):
        kd = kd_all[64 * (g - 1):64 * g]
        sg = np.where(kd % 9 == g, -1.0, 1.0).reshape(8, 8, 1, 1)
        th = (2 * np.pi / D) * ((kd[:, None] * b[None, :]) % D)
        c, s = np.cos(th).reshape(8, 8, 8, 8), np.sin(th).reshape(8, 8, 8, 8)
        m = np.zeros((8, 2, 8, 8, 2, 8))
        m[:, 0, :, :, 0, :] = c
        m[:, 0, :, :, 1, :] = sg * _Q * s
        m[:, 1, :, :, 0, :] = -s
        m[:, 1, :, :, 1, :] = sg * _Q * c
        mats[g - 1] = m.reshape(128, 128)
        mats[5 + g - 1] = m.reshape(128, 128).T
    kd = kd_all[256:]
    valid = (kd >= 0)[:, None]
    th = (2 * np.pi / D) * ((kd[:, None] * b[None, :]) % D)
    m = np.zeros((5, 2, 8, 64))
    m[:, 0] = (np.cos(th) * valid).reshape(5, 8, 64)
    m[:, 1] = (-np.sin(th) * valid * (kd != D // 2)[:, None]).reshape(5, 8, 64)
    half = np.where((kd == 0) | (kd == D // 2), 0.5, 1.0).reshape(5, 1, 8, 1)
    mats[4, :80, :64] = m.reshape(80, 64)
    mats[9, :64, :80] = (m * half).reshape(80, 64).T
    return _pack_rows(mats)


def _token_tables():
    l = np.arange(128)
    ones = np.ones((8, 1))
    angles = [(2 * np.pi / 128) * ((l[:8, None] * l[None, :]) % 128),
              (2 * np.pi / 128) * ((8 * l) % 128) * ones, (2 * np.pi / S) * l * ones]
    return np.concatenate([p for a in angles for p in (np.cos(a), -np.sin(a))]).astype(np.float32)


_CH_MATS = _channel_mats()
_TOK_TAB = _token_tables()


def _dot(a, b):
    return jnp.dot(a, b, preferred_element_type=f32)


def _radix9(x):
    s1, s2, s3, s4 = x[1] + x[8], x[2] + x[7], x[3] + x[6], x[4] + x[5]
    d1, d2, d3, d4 = x[1] - x[8], x[2] - x[7], x[3] - x[6], x[4] - x[5]
    p = x[0] - 0.5 * s3
    a, b = s1 - s4, s2 - s4
    r1 = _C1 * a + _C2 * b
    r2 = _C2 * a + _C4 * b
    e, g = d1 + d2, d2 + d4
    i1 = _S1 * e + _S4 * g
    i2 = _S2 * e - _S1 * g
    t, u = s1 + s2 + s4, x[0] + s3
    return u + t, [(p + r1, i1 + d3), (p + r2, i2 - d3),
                   (u - 0.5 * t, d1 - d2 + d4), ((p - r1) - r2, (i2 - i1) + d3)]


def _radix9_t(x0, uv):
    (u1, v1), (u2, v2), (u3, v3), (u4, v4) = uv
    u, t = x0 + u3, x0 - 0.5 * u3
    p, r1, r2 = u1 + u2 + u4, u1 - u4, u2 - u4
    a = _C1 * r1 + _C2 * r2
    b = _C2 * r1 + _C4 * r2
    s1, s2, s3, s4 = t + a, t + b, u - 0.5 * p, (t - a) - b
    i1, i2, d3 = v1 - v4, v2 + v4, v1 - v2 + v4
    e = _S1 * i1 + _S2 * i2
    g = _S4 * i1 - _S1 * i2
    d1, d2, d4 = e + v3, (e + g) - v3, g + v3
    return [u + p, s1 + d1, s2 + d2, s3 + d3, s4 + d4, s4 - d4, s3 - d3, s2 - d2, s1 - d1]


def _radix4(x, sign):
    (ar, ai), (br, bi), (cr, ci), (dr, di) = x
    pr, pi, mr, mi = ar + cr, ai + ci, ar - cr, ai - ci
    qr, qi, nr, ni = br + dr, bi + di, br - dr, bi - di
    plus, minus = (mr - ni, mi + nr), (mr + ni, mi - nr)
    k1, k3 = (plus, minus) if sign > 0 else (minus, plus)
    return [(pr + qr, pi + qi), k1, (pr - qr, pi - qi), k3]


def _twiddle16(z, e, sign):
    re, im = z
    if e == 0:
        return z
    c, s = float(np.cos(2 * np.pi * e / 16)), float(sign * np.sin(2 * np.pi * e / 16))
    if e == 4:
        return (-im, re) if sign > 0 else (im, -re)
    if e % 2 == 0:
        if c * s > 0:
            return c * (re - im), c * (re + im)
        return c * (re + im), c * (im - re)
    return c * re - s * im, s * re + c * im


def _radix16(x, sign):
    y = [_radix4(x[t0::4], sign) for t0 in range(4)]
    out = [None] * 16
    for q0 in range(4):
        col = _radix4([_twiddle16(y[t0][q0], t0 * q0, sign) for t0 in range(4)], sign)
        for q1 in range(4):
            out[q0 + 4 * q1] = col[q1]
    return out


def _halves(w):
    return pltpu.bitcast(w, bf16)


def _pair(a, b):
    return jnp.concatenate([a, b], axis=0).astype(bf16)


class _RowMean:
    def __init__(self, lanes=2):
        self.acc, self.n = [None] * lanes, 0

    def add(self, v):
        i = self.n % len(self.acc)
        self.acc[i] = v if self.acc[i] is None else self.acc[i] + v
        self.n += 1

    def mean(self):
        acc = self.acc
        while len(acc) > 1:
            acc = [acc[i] + acc[i + 1] for i in range(0, len(acc), 2)]
        return jnp.sum(acc[0], axis=0, keepdims=True) * (1.0 / D)


def _gelu(x):
    inner = x * (0.7978845608028654 + (0.7978845608028654 * 0.044715) * (x * x))
    hx = 0.5 * x
    return hx + hx * jnp.tanh(inner)


def _lhs_forms(a11, a12, a21, a22):
    return [a11 + a22, a21 + a22, a11, a22, a11 + a12, a21 - a11, a12 - a22]


def _rhs_forms(b11, b12, b21, b22):
    f11, f12, f21, f22 = (b.astype(f32) for b in (b11, b12, b21, b22))
    return [(f11 + f22).astype(bf16), b11, (f12 - f22).astype(bf16), (f21 - f11).astype(bf16),
            b22, (f11 + f12).astype(bf16), (f21 + f22).astype(bf16)]


def _out_forms(m):
    return m[0] + m[3] - m[4] + m[6], m[2] + m[4], m[1] + m[3], m[0] - m[1] + m[2] + m[5]


def _kernel(x_hbm, wr_hbm, wi_hbm, w1_hbm, b1_hbm, w2_hbm, b2_hbm, c_hbm, wm_hbm, chm_hbm, tok_hbm,
            o_hbm,
            x_v, wr_v, wi_v, w1_v, b1_v, w2_v, b2_v, c_v, wm_v, chm_v, tok_v,
            mod_v, mf_v, mi_v, wt_v, wp_v, r_v, fa_v, fb_v, fc_v, fd_v, x1_v, a_v, acc_v, o_v, b1_f, st_v,
            sem):
    slots = itertools.count()

    def copy(src, dst):
        return pltpu.make_async_copy(src, dst, sem.at[next(slots)])

    def cols(ref, lo, n):
        return ref.at[:, pl.ds(lo, n)]

    def copy_cols(src, dst, lo, n):
        return copy(cols(src, lo, n), cols(dst, lo, n))

    cp_tok, cp_c = copy(tok_hbm, tok_v), copy(c_hbm, c_v)
    cp_mod = [copy_cols(wm_hbm, wm_v, 128 * lo, 128 * (hi - lo)) for lo, hi in MOD_PARTS]
    cp_chm = [copy(chm_hbm.at[pl.ds(5 * i, 5)], chm_v.at[pl.ds(5 * i, 5)]) for i in range(2)]
    cp_w = [copy_cols(h, v, i * (S // WCH), S // WCH)
            for i in range(WCH) for h, v in ((wr_hbm, wr_v), (wi_hbm, wi_v))]
    cp_b1, cp_b2 = copy(b1_hbm, b1_v), copy(b2_hbm, b2_v)
    sem_x, sem_w1, sem_w2, sem_o = (
        [next(slots) for _ in range(n)][0] for n in (NT // 2, NCH, NCH, 2 * OCH))

    def cp_x(i):
        lo = i * 256 if isinstance(i, int) else pl.multiple_of(i * 256, 256)
        return pltpu.make_async_copy(cols(x_hbm, lo, 256), cols(x_v, lo, 256), sem.at[sem_x + i])

    def cp_w1(j):
        return pltpu.make_async_copy(cols(w1_hbm, j * TF, TF), w1_v.at[j], sem.at[sem_w1 + j])

    def cp_w2(j):
        return pltpu.make_async_copy(w2_hbm.at[pl.ds(j * TF, TF), :], w2_v.at[j],
                                     sem.at[sem_w2 + j])

    for c in (cp_tok, cp_c, cp_mod[0], cp_chm[0], *map(cp_x, range(NT // 2)), *cp_w,
              cp_chm[1], cp_mod[1], cp_b1, cp_w1(0), cp_w2(0), cp_b2, cp_mod[2]):
        c.start()
    for j in range(1, NCH):
        cp_w1(j).start()
        cp_w2(j).start()

    def lanes(t):
        if isinstance(t, int):
            return slice(128 * t, 128 * (t + 1))
        return pl.ds(pl.multiple_of(t * 128, 128), 128)

    def blk(i):
        return slice(8 * i, 8 * i + 8)

    def cmul(a, b):
        return a[0] * b[0] - a[1] * b[1], a[0] * b[1] + a[1] * b[0]

    with jax.named_scope("gen"):
        cp_tok.wait()
        rows = [(tok_v[blk(0), :], tok_v[blk(1), :])]
        for _ in range(15):
            rows.append(cmul(rows[-1], (tok_v[blk(2), :], tok_v[blk(3), :])))
        dft = tuple(jnp.concatenate([r[i] for r in rows], axis=0) for i in range(2))
        along = tuple(jnp.concatenate([tok_v[blk(i), :]] * 16, axis=0) for i in (4, 5))
        down = tuple(a.T for a in along)

        def gen(k, carry):
            for ref, m in zip((mf_v, mi_v), carry):
                ref[k, 0], ref[k, 1] = m[0].astype(bf16), m[1].astype(bf16)
            return cmul(carry[0], down), cmul(carry[1], along)

        lax.fori_loop(0, NT, gen, (dft, dft))

    cp_c.wait()
    cf = c_v[...].astype(f32)
    sc = jnp.broadcast_to(cf * jax.nn.sigmoid(cf), (16, D)).astype(bf16)

    def store_mod(j):
        row = _dot(sc, wm_v[:, lanes(j)])[0:8, :]
        n = 128 * j + lax.broadcasted_iota(jnp.int32, row.shape, 1)
        scale = jnp.logical_or(jnp.logical_and(n >= D, n < 2 * D),
                               jnp.logical_and(n >= 4 * D, n < 5 * D))
        row = jnp.where(scale, row + 1.0, row)
        row = jnp.where(jnp.logical_and(n >= 2 * D, n < 3 * D), row * (2.0 / (S * D)), row)
        mod_v[lanes(j), :] = jnp.concatenate([row] * 16, axis=0).T

    def mod(i, b=None):
        return mod_v[i * D:(i + 1) * D, :] if b is None else mod_v[blk(i * D // 8 + b), :]

    with jax.named_scope("modA"):
        cp_mod[0].wait()
        for j in range(*MOD_PARTS[0]):
            store_mod(j)

    def stage(pair, slot, values, finish=lambda m: m):
        means = [_RowMean() for _ in pair]
        for vs in zip(*map(values, pair)):
            for m, v in zip(means, vs):
                m.add(v)
        for t, m in zip(pair, means):
            st_v[slot, t] = jnp.broadcast_to(finish(m.mean()), (8, 128))

    def inv_std(var):
        return lax.rsqrt(var + EPS)

    def tokens(t, i):
        x = x_v[16 * i:16 * i + 16, lanes(t)].astype(f32)
        return x[:8], x[8:]

    def a_mean(t):
        for i in range(D // 16):
            for b, x in enumerate(tokens(t, i), 2 * i):
                fc_v[t, blk(b), :] = x
                yield x

    def squares(src, slot, dst=None):
        def values(t):
            mean = st_v[slot, t]
            for b in range(D // 8):
                c = src[t, blk(b), :] - mean
                if dst is not None:
                    dst[t, blk(b), :] = c
                yield c * c
        return values

    def fwd_butterflies(pair):
        for t in pair:
            rstd = st_v[1, t]
            for p in range(8):
                x0, uv = _radix9([x1_v[t, blk(b), :] * rstd * mod(1, b) + mod(0, b)
                                  for b in range(p, D // 8, 8)])
                for g in range(4):
                    r_v[t, 128 * g + 16 * p:128 * g + 16 * p + 16, :] = _pair(*uv[g])
                if p % 2:
                    r_v[t, 504 + 8 * p:520 + 8 * p, :] = _pair(prev, x0)
                prev = x0

    def skewed(stages, n):
        def step(i, active):
            for s in active:
                stages[s](i - s)
        depth = len(stages) - 1
        for i in range(depth):
            step(i, range(i + 1))
        lax.fori_loop(depth, n, lambda i, _: step(i, range(depth + 1)), None)
        for i in range(n, n + depth):
            step(i, range(i - n + 1, depth + 1))

    def adjacent(i):
        return 2 * i, 2 * i + 1

    def a_first(i):
        cp_x(i).wait()
        stage(adjacent(i), 0, a_mean)

    with jax.named_scope("A"):
        skewed([a_first, lambda i: stage(adjacent(i), 1, squares(fc_v, 0, x1_v), inv_std),
                lambda i: fwd_butterflies(adjacent(i))], NT // 2)

    def filt_a(t):
        a = pltpu.bitcast(wr_v[0:DF - 1, lanes(t)], f32)
        b = pltpu.bitcast(wi_v[0:DF - 1, lanes(t)], f32)
        nr = wr_v[DF - 1:DF, lanes(t)].astype(f32)
        ni = wi_v[DF - 1:DF, lanes(t)].astype(f32)
        r = lax.broadcasted_iota(jnp.int32, (8, 128), 0)
        nyq = jnp.where(r == 0, nr, jnp.where(r == 1, ni, 0.0))
        rest = jnp.concatenate([a[128:], b[128:], nyq, jnp.zeros((88, 128), f32)], axis=0)
        for c, tile in enumerate((a[:128].T, b[:128].T, rest.T)):
            for j in range(8):
                lo = (NT + 1) * (8 * t + j)
                wt_v[c, lo:lo + NT, :] = tile[NT * j:NT * (j + 1)]

    def filt_b(k):
        wp_v[k, 0:128, :] = wt_v[0, pl.ds(k, 128, stride=NT + 1), :].T
        wp_v[k, 144:272, :] = wt_v[1, pl.ds(k, 128, stride=NT + 1), :].T
        rest = wt_v[2, pl.ds(k, 128, stride=NT + 1), :].T
        wp_v[k, 128:144, :] = rest[0:16]
        wp_v[k, 272:296, :] = rest[16:40]

    def filt(k, rb, base, nyq_row):
        if rb == NRB - 1:
            return jnp.broadcast_to(wp_v[k, nyq_row:nyq_row + 1, :], (8, 128))
        k0 = _row_runs()[rb // 2]
        w = pltpu.bitcast(wp_v[k, pl.ds(base + k0 // 2 + 72 * (rb % 2), 8, stride=9), :], u32)
        w = (w & np.uint32(0xFFFF0000)) if k0 % 2 else (w << 16)
        return pltpu.bitcast(w, f32)

    groups = [range(8 * g, min(8 * g + 8, NRB)) for g in range(5)]

    def rows(g):
        return slice(16 * groups[g][0], 16 * groups[g][-1] + 16)

    def fwd_channel(g, t):
        if g < 4:
            fa_v[t, rows(g), :] = _dot(_halves(chm_v[g]), r_v[t, rows(g), :])
        else:
            rhs = jnp.concatenate([r_v[t, 512:576, :], jnp.zeros((64, 128), bf16)], axis=0)
            fa_v[t, rows(g), :] = _dot(_halves(chm_v[4, 0:40, :]), rhs)

    def inv_channel(g, t):
        if g < 4:
            fc_v[t, rows(g), :] = _dot(_halves(chm_v[5 + g]), fd_v[t, rows(g), :])
        else:
            rhs = jnp.concatenate([fd_v[t, rows(g), :], jnp.zeros((48, 128), bf16)], axis=0)
            fc_v[t, 512:576, :] = _dot(_halves(chm_v[9, 0:32, :]), rhs)

    def butterflies(src, dst, sign, rb):
        z = [(src[t, blk(2 * rb), :], src[t, blk(2 * rb + 1), :]) for t in range(NT)]
        for k, (re, im) in enumerate(_radix16(z, sign)):
            dst[k, 16 * rb:16 * rb + 16, :] = _pair(re, im)

    def fwd_token(g, k):
        lhs = fb_v[k, rows(g), :]
        p, q = _dot(lhs, mf_v[k, 0]), _dot(lhs, mf_v[k, 1])
        for i, rb in enumerate(groups[g]):
            re, im = blk(2 * i), blk(2 * i + 1)
            fc_v[k, blk(2 * rb), :] = p[re] - q[im]
            fc_v[k, blk(2 * rb + 1), :] = q[re] + p[im]

    def inv_token(g, k):
        z = []
        for rb in groups[g]:
            yr, yi = fc_v[k, blk(2 * rb), :], fc_v[k, blk(2 * rb + 1), :]
            wr, wi = filt(k, rb, 0, 288), filt(k, rb, 144, 289)
            z += [yr * wr - yi * wi, yr * wi + yi * wr]
        lhs = jnp.concatenate(z, axis=0).astype(bf16)
        p, q = _dot(lhs, mi_v[k, 0]), _dot(lhs, mi_v[k, 1])
        for i, rb in enumerate(groups[g]):
            re, im = blk(2 * i), blk(2 * i + 1)
            fa_v[k, blk(2 * rb), :] = p[re] + q[im]
            fa_v[k, blk(2 * rb + 1), :] = p[im] - q[re]

    def spread(items, i, n=NT):
        return items[len(items) * i // n:len(items) * (i + 1) // n]

    def filt_step(i):
        if i < NT and i % (NT // WCH) == 0:
            cp_w[2 * i * WCH // NT].wait()
            cp_w[2 * i * WCH // NT + 1].wait()
        (filt_a if i < NT else filt_b)(i % NT)

    with jax.named_scope("F"):
        cp_chm[0].wait()
        for s in range(7):
            for k in range(NT):
                if s < 5:
                    fwd_channel(s, k)
                if 2 <= s:
                    fwd_token(s - 2, k)
                if 1 <= s < 6:
                    for rb in spread(groups[s - 1], k):
                        butterflies(fa_v, fb_v, -1, rb)
                for i in spread(range(2 * NT), NT * s + k, 6 * NT):
                    filt_step(i)
    with jax.named_scope("I"):
        cp_chm[1].wait()
        cp_mod[1].wait()
        for s in range(7):
            for k in range(NT):
                if s < 5:
                    inv_token(s, k)
                if 2 <= s:
                    inv_channel(s - 2, k)
                if 1 <= s < 6:
                    for rb in spread(groups[s - 1], k):
                        butterflies(fa_v, fd_v, +1, rb)
                for j in spread(range(*MOD_PARTS[1]), NT * s + k, 6 * NT):
                    store_mod(j)

    def opposite(j):
        return j, j + NT // 2

    def residual(t):
        for p in range(0, 8, 2):
            ys = []
            for q in (p, p + 1):
                uv = [(fc_v[t, blk(16 * g + 2 * q), :], fc_v[t, blk(16 * g + 2 * q + 1), :])
                      for g in range(4)]
                ys.append(_radix9_t(fc_v[t, blk(64 + q), :], uv))
            for a in range(9):
                for b, x, y in zip((8 * a + p, 8 * a + p + 1), tokens(t, 4 * a + p // 2), ys):
                    x1 = x + mod(2, b) * y[a]
                    x1_v[t, blk(b), :] = x1
                    yield x1

    def modulated(t):
        mean, rstd = st_v[0, t], st_v[1, t]
        for b in range(D // 8):
            h = (x1_v[t, blk(b), :] - mean) * rstd * mod(4, b) + mod(3, b)
            fa_v[t, blk(b), :] = h
            yield h

    def mlp_operands(j):
        stats = [(t, st_v[2, t], st_v[3, t]) for t in opposite(j)]
        for r in range(0, D // 2, 16):
            quads = [jnp.concatenate([(fa_v[t, q:q + 8, :] - mean) * rstd for q in (lo, lo + 8)],
                                     axis=0)
                     for lo in (r, D // 2 + r) for t, mean, rstd in stats]
            for i, a in enumerate(_lhs_forms(*quads)):
                a_v[i, r:r + 16, lanes(j)] = a.astype(bf16)

    with jax.named_scope("C"):
        skewed([lambda j: stage(opposite(j), 0, residual),
                lambda j: stage(opposite(j), 1, squares(x1_v, 0), inv_std)], NT // 2)
        skewed([lambda j: stage(opposite(j), 2, modulated),
                lambda j: stage(opposite(j), 3, squares(fa_v, 2), inv_std),
                mlp_operands], NT // 2)

    hs, hf = S // 2, TF // 2

    def hidden(j):
        rhs = _rhs_forms(w1_v[j, :hs, :hf], w1_v[j, :hs, hf:], w1_v[j, hs:, :hf], w1_v[j, hs:, hf:])
        u11, u12, u21, u22 = _out_forms([_dot(a_v[i], rhs[i]) for i in range(7)])
        nb = TF // 128
        bias = [b1_f[pl.ds(j * nb + i, 1), :] for i in range(nb)]
        bl = jnp.concatenate(bias[:nb // 2], axis=1)
        br = jnp.concatenate(bias[nb // 2:], axis=1)
        lhs = _lhs_forms(_gelu(u11 + bl), _gelu(u12 + br), _gelu(u21 + bl), _gelu(u22 + br))
        return [a.astype(bf16) for a in lhs]

    def w2_forms(j, lo, n):
        return _rhs_forms(w2_v[j, :hf, lo:lo + n], w2_v[j, :hf, hs + lo:hs + lo + n],
                          w2_v[j, hf:, lo:lo + n], w2_v[j, hf:, hs + lo:hs + lo + n])

    def chunk(j, _):
        cp_w1(j).wait()
        cp_w2(j).wait()
        lhs, rhs = hidden(j), w2_forms(j, 0, hs)
        for i in range(7):
            acc_v[i] += _dot(lhs[i], rhs[i])

    with jax.named_scope("MLP0"):
        cp_b1.wait()
        b1_f[0:F // 128, :] = b1_v[...].astype(f32)
        cp_w1(0).wait()
        cp_w2(0).wait()
        lhs, rhs = hidden(0), w2_forms(0, 0, hs)
        for i in range(7):
            acc_v[i] = _dot(lhs[i], rhs[i])
    with jax.named_scope("MLP"):
        lax.fori_loop(1, NCH - 1, chunk, None)

    with jax.named_scope("MLPlast"):
        cp_w1(NCH - 1).wait()
        cp_w2(NCH - 1).wait()
        cp_b2.wait()
        cp_mod[2].wait()
        for j in range(*MOD_PARTS[2]):
            store_mod(j)
        lhs = hidden(NCH - 1)
        b2 = b2_v[...].astype(f32)
        cp_o = []
        for j in range(OCH):
            n = hs // OCH
            rhs = w2_forms(NCH - 1, j * n, n)
            y11, y12, y21, y22 = _out_forms(
                [acc_v[i, :, j * n:(j + 1) * n] + _dot(lhs[i], rhs[i]) for i in range(7)])
            for half, top, bot in ((0, y11, y21), (1, y12, y22)):
                y = jnp.concatenate([top, bot], axis=0)
                for q in range(n // 128):
                    t = (half * hs + j * n) // 128 + q
                    o_v[:, lanes(t)] = (
                        x1_v[t] + mod(5) * (y[:, lanes(q)] + b2[t:t + 1, :])).astype(bf16)
                lo = half * hs + j * n
                cp_o.append(pltpu.make_async_copy(cols(o_v, lo, n), cols(o_hbm, lo, n),
                                                  sem.at[sem_o + 2 * j + half]))
                cp_o[-1].start()
        for c in cp_o:
            c.wait()


@jax.jit
def pallas_adaLN_cond__spectral_gfnet__mixer_token_mlp__prompt_kernel(
    A_x: jax.Array,
    A_w_r: jax.Array,
    A_w_i: jax.Array,
    B_x: jax.Array,
    B_w1: jax.Array,
    B_b1: jax.Array,
    B_w2: jax.Array,
    B_b2: jax.Array,
    c: jax.Array,
    w_mod: jax.Array,
):
    del B_x
    vmem = pltpu.VMEM
    scratch = [
        vmem((D, S), bf16), vmem((DF, S), bf16), vmem((DF, S), bf16),
        vmem((NCH, S, TF), bf16), vmem((F // 128, 128), bf16),
        vmem((NCH, TF, S), bf16), vmem((S // 128, 128), bf16),
        vmem((1, D), bf16), vmem((D, 6 * D), bf16),
        vmem(_CH_MATS.shape, u32), vmem(_TOK_TAB.shape, f32),
        vmem((6 * D, 128), f32),
        vmem((NT, 2, 128, 128), bf16),
        vmem((NT, 2, 128, 128), bf16),
        vmem((3, S + 128, 128), f32),
        vmem((NT, 296, 128), f32),
        vmem((NT, D, 128), bf16),
        vmem((NT, NRB * 16, 128), f32),
        vmem((NT, NRB * 16, 128), bf16),
        vmem((NT, NRB * 16, 128), f32),
        vmem((NT, NRB * 16, 128), bf16),
        vmem((NT, D, 128), f32),
        vmem((7, D // 2, S // 2), bf16),
        vmem((7, D // 2, S // 2), f32),
        vmem((D, S), bf16),
        vmem((40, 128), f32),
        vmem((4, NT, 8, 128), f32),
        pltpu.SemaphoreType.DMA((64,)),
    ]
    out = pl.pallas_call(
        _kernel,
        in_specs=[pl.BlockSpec(memory_space=pl.ANY)] * 11,
        out_specs=pl.BlockSpec(memory_space=pl.ANY),
        out_shape=jax.ShapeDtypeStruct((D, S), bf16),
        scratch_shapes=scratch,
        compiler_params=pltpu.CompilerParams(vmem_limit_bytes=120 * 1024 * 1024),
    )(A_x[0].T, A_w_r.T, A_w_i.T, B_w1, B_b1.reshape(F // 128, 128), B_w2,
      B_b2.reshape(S // 128, 128), c, w_mod, _CH_MATS, _TOK_TAB)
    return out.T[None]
```

```python
import itertools

import jax
import jax.numpy as jnp
import numpy as np
from jax import lax
from jax.experimental import pallas as pl
from jax.experimental.pallas import tpu as pltpu

D, S, F = 576, 2048, 4608
DF = D // 2 + 1
NT = S // 128
NRB = 37
EPS = 1e-5
CHUNKS = (512, 1024, 1024, 1024, 1024)
STARTS = tuple(sum(CHUNKS[:j]) for j in range(len(CHUNKS)))
WCH = 4
MOD_PARTS = ((0, 9), (9, 27))

f32, bf16, u32 = jnp.float32, jnp.bfloat16, jnp.uint32

_Q = np.sqrt(3.0) / 2
_C1, _C2, _C4 = (float(np.cos(2 * np.pi * k / 9)) for k in (1, 2, 4))
_S1, _S2, _S4 = (float(np.sin(2 * np.pi * k / 9) / _Q) for k in (1, 2, 4))


def _row_runs():
    runs = []
    for g in (1, 2, 3, 4):
        for r in (g, 9 - g):
            runs += [r, r + 9]
    return runs + [0, 9]


def _pack_rows(m):
    b = m.astype(np.float32).astype(jnp.bfloat16).view(np.uint16).astype(np.uint32)
    return b[..., 0::2, :] | (b[..., 1::2, :] << np.uint32(16))


def _channel_mats():
    kd_all = [k0 + 18 * j for k0 in _row_runs() for j in range(16)] + [D // 2] + [-1] * 7
    kd_all = np.array(kd_all)
    b = np.arange(64)
    mats = np.zeros((10, 128, 128))
    for g in (1, 2, 3, 4):
        kd = kd_all[64 * (g - 1):64 * g]
        sg = np.where(kd % 9 == g, -1.0, 1.0).reshape(8, 8, 1, 1)
        th = (2 * np.pi / D) * ((kd[:, None] * b[None, :]) % D)
        c, s = np.cos(th).reshape(8, 8, 8, 8), np.sin(th).reshape(8, 8, 8, 8)
        m = np.zeros((8, 2, 8, 8, 2, 8))
        m[:, 0, :, :, 0, :] = c
        m[:, 0, :, :, 1, :] = sg * _Q * s
        m[:, 1, :, :, 0, :] = -s
        m[:, 1, :, :, 1, :] = sg * _Q * c
        mats[g - 1] = m.reshape(128, 128)
        mats[5 + g - 1] = m.reshape(128, 128).T
    kd = kd_all[256:]
    valid = (kd >= 0)[:, None]
    th = (2 * np.pi / D) * ((kd[:, None] * b[None, :]) % D)
    m = np.zeros((5, 2, 8, 64))
    m[:, 0] = (np.cos(th) * valid).reshape(5, 8, 64)
    m[:, 1] = (-np.sin(th) * valid * (kd != D // 2)[:, None]).reshape(5, 8, 64)
    half = np.where((kd == 0) | (kd == D // 2), 0.5, 1.0).reshape(5, 1, 8, 1)
    mats[4, :80, :64] = m.reshape(80, 64)
    mats[9, :64, :80] = (m * half).reshape(80, 64).T
    return _pack_rows(mats)


def _token_tables():
    l = np.arange(128)
    ones = np.ones((8, 1))
    angles = [(2 * np.pi / 128) * ((l[:8, None] * l[None, :]) % 128),
              (2 * np.pi / 128) * ((8 * l) % 128) * ones, (2 * np.pi / S) * l * ones]
    return np.concatenate([p for a in angles for p in (np.cos(a), -np.sin(a))]).astype(np.float32)


_CH_MATS = _channel_mats()
_TOK_TAB = _token_tables()


def _dot(a, b):
    return jnp.dot(a, b, preferred_element_type=f32)


def _radix9(x):
    s1, s2, s3, s4 = x[1] + x[8], x[2] + x[7], x[3] + x[6], x[4] + x[5]
    d1, d2, d3, d4 = x[1] - x[8], x[2] - x[7], x[3] - x[6], x[4] - x[5]
    p = x[0] - 0.5 * s3
    a, b = s1 - s4, s2 - s4
    r1 = _C1 * a + _C2 * b
    r2 = _C2 * a + _C4 * b
    e, g = d1 + d2, d2 + d4
    i1 = _S1 * e + _S4 * g
    i2 = _S2 * e - _S1 * g
    t, u = s1 + s2 + s4, x[0] + s3
    return u + t, [(p + r1, i1 + d3), (p + r2, i2 - d3),
                   (u - 0.5 * t, d1 - d2 + d4), ((p - r1) - r2, (i2 - i1) + d3)]


def _radix9_t(x0, uv):
    (u1, v1), (u2, v2), (u3, v3), (u4, v4) = uv
    u, t = x0 + u3, x0 - 0.5 * u3
    p, r1, r2 = u1 + u2 + u4, u1 - u4, u2 - u4
    a = _C1 * r1 + _C2 * r2
    b = _C2 * r1 + _C4 * r2
    s1, s2, s3, s4 = t + a, t + b, u - 0.5 * p, (t - a) - b
    i1, i2, d3 = v1 - v4, v2 + v4, v1 - v2 + v4
    e = _S1 * i1 + _S2 * i2
    g = _S4 * i1 - _S1 * i2
    d1, d2, d4 = e + v3, (e + g) - v3, g + v3
    return [u + p, s1 + d1, s2 + d2, s3 + d3, s4 + d4, s4 - d4, s3 - d3, s2 - d2, s1 - d1]


def _radix4(x, sign):
    (ar, ai), (br, bi), (cr, ci), (dr, di) = x
    pr, pi, mr, mi = ar + cr, ai + ci, ar - cr, ai - ci
    qr, qi, nr, ni = br + dr, bi + di, br - dr, bi - di
    plus, minus = (mr - ni, mi + nr), (mr + ni, mi - nr)
    k1, k3 = (plus, minus) if sign > 0 else (minus, plus)
    return [(pr + qr, pi + qi), k1, (pr - qr, pi - qi), k3]


def _twiddle16(z, e, sign):
    re, im = z
    if e == 0:
        return z
    c, s = float(np.cos(2 * np.pi * e / 16)), float(sign * np.sin(2 * np.pi * e / 16))
    if e == 4:
        return (-im, re) if sign > 0 else (im, -re)
    if e % 2 == 0:
        if c * s > 0:
            return c * (re - im), c * (re + im)
        return c * (re + im), c * (im - re)
    return c * re - s * im, s * re + c * im


def _radix16(x, sign):
    y = [_radix4(x[t0::4], sign) for t0 in range(4)]
    out = [None] * 16
    for q0 in range(4):
        col = _radix4([_twiddle16(y[t0][q0], t0 * q0, sign) for t0 in range(4)], sign)
        for q1 in range(4):
            out[q0 + 4 * q1] = col[q1]
    return out


def _halves(w):
    return pltpu.bitcast(w, bf16)


def _pair(a, b):
    return jnp.concatenate([a, b], axis=0).astype(bf16)


class _RowMean:
    def __init__(self, lanes=2):
        self.acc, self.n = [None] * lanes, 0

    def add(self, v):
        i = self.n % len(self.acc)
        self.acc[i] = v if self.acc[i] is None else self.acc[i] + v
        self.n += 1

    def mean(self):
        acc = self.acc
        while len(acc) > 1:
            acc = [acc[i] + acc[i + 1] for i in range(0, len(acc), 2)]
        return jnp.sum(acc[0], axis=0, keepdims=True) * (1.0 / D)


def _gelu(x):
    inner = x * (0.7978845608028654 + (0.7978845608028654 * 0.044715) * (x * x))
    hx = 0.5 * x
    return hx + hx * jnp.tanh(inner)


def _lhs_forms(a11, a12, a21, a22):
    return [a11 + a22, a21 + a22, a11, a22, a11 + a12, a21 - a11, a12 - a22]


def _rhs_form(i, quad):
    if i in (1, 4):
        return quad(i // 4, i // 4)
    a, sign, b = {0: ((0, 0), 1, (1, 1)), 2: ((0, 1), -1, (1, 1)), 3: ((1, 0), -1, (0, 0)),
                  5: ((0, 0), 1, (0, 1)), 6: ((1, 0), 1, (1, 1))}[i]
    a, b = quad(*a).astype(f32), quad(*b).astype(f32)
    return (a + b if sign > 0 else a - b).astype(bf16)


def _out_forms(m):
    return m[0] + m[3] - m[4] + m[6], m[2] + m[4], m[1] + m[3], m[0] - m[1] + m[2] + m[5]


def _kernel(x_hbm, wr_hbm, wi_hbm, w1_hbm, b1_hbm, w2_hbm, b2_hbm, c_hbm, wm_hbm, chm_hbm, tok_hbm,
            o_hbm,
            x_v, wr_v, wi_v, w1_v, b1_v, w2_v, b2_v, c_v, wm_v, chm_v, tok_v,
            mod_v, mf_v, mi_v, wt_v, wp_v, r_v, fa_v, fb_v, fc_v, fd_v, x1_v, a_v, acc_v, o_v, b1_f, st_v,
            sem):
    slots = itertools.count()

    def copy(src, dst):
        return pltpu.make_async_copy(src, dst, sem.at[next(slots)])

    def cols(ref, lo, n):
        return ref.at[:, pl.ds(lo, n)]

    def copy_cols(src, dst, lo, n):
        return copy(cols(src, lo, n), cols(dst, lo, n))

    cp_tok, cp_c = copy(tok_hbm, tok_v), copy(c_hbm, c_v)
    cp_mod = [copy_cols(wm_hbm, wm_v, 128 * lo, 128 * (hi - lo)) for lo, hi in MOD_PARTS]
    cp_chm = [copy(chm_hbm.at[pl.ds(5 * i, 5)], chm_v.at[pl.ds(5 * i, 5)]) for i in range(2)]
    cp_w = [copy_cols(h, v, i * (S // WCH), S // WCH)
            for i in range(WCH) for h, v in ((wr_hbm, wr_v), (wi_hbm, wi_v))]
    cp_b1, cp_b2 = copy(b1_hbm, b1_v), copy(b2_hbm, b2_v)
    cp_w1 = [copy_cols(w1_hbm, w1_v, lo, n) for lo, n in zip(STARTS, CHUNKS)]
    cp_w2 = [copy(w2_hbm.at[pl.ds(lo, n)], w2_v.at[pl.ds(lo, n)]) for lo, n in zip(STARTS, CHUNKS)]
    cp_o = [copy_cols(o_v, o_hbm, 128 * t, 128) for t in range(NT)]
    sem_x = next(slots)

    def cp_x(i):
        lo = i * 256 if isinstance(i, int) else pl.multiple_of(i * 256, 256)
        return pltpu.make_async_copy(cols(x_hbm, lo, 256), cols(x_v, lo, 256), sem.at[sem_x + i])

    for c in (cp_tok, cp_c, cp_x(0), cp_x(1), cp_mod[0], *map(cp_x, range(2, NT // 2)), cp_chm[0],
              *cp_w, cp_chm[1], cp_mod[1], cp_b1, cp_b2, *itertools.chain(*zip(cp_w1, cp_w2))):
        c.start()

    def lanes(t):
        if isinstance(t, int):
            return slice(128 * t, 128 * (t + 1))
        return pl.ds(pl.multiple_of(t * 128, 128), 128)

    def blk(i):
        return slice(8 * i, 8 * i + 8)

    def cmul(a, b):
        return a[0] * b[0] - a[1] * b[1], a[0] * b[1] + a[1] * b[0]

    with jax.named_scope("gen"):
        cp_tok.wait()
        rows = [(tok_v[blk(0), :], tok_v[blk(1), :])]
        for _ in range(15):
            rows.append(cmul(rows[-1], (tok_v[blk(2), :], tok_v[blk(3), :])))
        dft = tuple(jnp.concatenate([r[i] for r in rows], axis=0) for i in range(2))
        along = tuple(jnp.concatenate([tok_v[blk(i), :]] * 16, axis=0) for i in (4, 5))
        down = tuple(a.T for a in along)

        def gen(k, carry):
            for ref, m in zip((mf_v, mi_v), carry):
                ref[k, 0], ref[k, 1] = m[0].astype(bf16), m[1].astype(bf16)
            return cmul(carry[0], down), cmul(carry[1], along)

        lax.fori_loop(0, NT, gen, (dft, dft))

    cp_c.wait()
    cf = c_v[...].astype(f32)
    sc = jnp.broadcast_to(cf * jax.nn.sigmoid(cf), (16, D)).astype(bf16)

    def store_mod(j):
        row = _dot(sc, wm_v[:, lanes(j)])[0:8, :]
        n = 128 * j + lax.broadcasted_iota(jnp.int32, row.shape, 1)
        scale = jnp.logical_or(jnp.logical_and(n >= D, n < 2 * D),
                               jnp.logical_and(n >= 4 * D, n < 5 * D))
        row = jnp.where(scale, row + 1.0, row)
        row = jnp.where(jnp.logical_and(n >= 2 * D, n < 3 * D), row * (2.0 / (S * D)), row)
        mod_v[lanes(j), :] = jnp.concatenate([row] * 16, axis=0).T

    def mod(i, b=None):
        return mod_v[i * D:(i + 1) * D, :] if b is None else mod_v[blk(i * D // 8 + b), :]

    def first_mod():
        cp_mod[0].wait()
        for j in range(*MOD_PARTS[0]):
            store_mod(j)

    def stage(pair, slot, values, finish=lambda m: m):
        means = [_RowMean() for _ in pair]
        for vs in zip(*map(values, pair)):
            for m, v in zip(means, vs):
                m.add(v)
            yield
        for t, m in zip(pair, means):
            st_v[slot, t] = jnp.broadcast_to(finish(m.mean()), (8, 128))

    def in_turn(gens):
        for g, _ in gens:
            for _ in g:
                pass

    def in_step(gens):
        n = D // 8
        for q in range(n):
            for g, cuts in gens:
                for _ in range(cuts * q // n, cuts * (q + 1) // n):
                    next(g)
        in_turn(gens)

    def skewed(stages, emit, n, after_fill=lambda: None):
        depth = len(stages) - 1

        def step(oldest, lo, hi):
            emit([(fn(oldest + (depth - lag)), cuts)
                  for lag, cuts, fn in stages if lo <= lag <= hi])

        for i in range(depth):
            step(i - depth, 0, i)
        after_fill()
        lax.fori_loop(0, n - depth, lambda i, _: step(i, 0, depth), None)
        for i in range(n, n + depth):
            step(i - depth, i - n + 1, depth)

    def inv_std(var):
        return lax.rsqrt(var + EPS)

    def squares(src, slot, dst=None):
        def values(t):
            mean = st_v[slot, t]
            for b in range(D // 8):
                c = src[t, blk(b), :] - mean
                if dst is not None:
                    dst[t, blk(b), :] = c
                yield c * c
        return values

    def adjacent(i):
        return 2 * i, 2 * i + 1

    def tokens(t):
        for i in range(D // 16):
            x = x_v[16 * i:16 * i + 16, lanes(t)].astype(f32)
            for b, half in enumerate((x[:8], x[8:]), 2 * i):
                x1_v[t, blk(b), :] = half
                yield half

    def load_tokens(i):
        cp_x(i).wait()
        return stage(adjacent(i), 0, tokens)

    def fwd_butterflies(i):
        for t in adjacent(i):
            rstd = st_v[1, t]
            for p in range(8):
                x0, uv = _radix9([fc_v[t, blk(b), :] * rstd * mod(1, b) + mod(0, b)
                                  for b in range(p, D // 8, 8)])
                for g in range(4):
                    r_v[t, 128 * g + 16 * p:128 * g + 16 * p + 16, :] = _pair(*uv[g])
                if p % 2:
                    r_v[t, 504 + 8 * p:520 + 8 * p, :] = _pair(prev, x0)
                prev = x0
                yield

    with jax.named_scope("A"):
        skewed([(1, D // 8, lambda i: stage(adjacent(i), 1, squares(x1_v, 0, fc_v), inv_std)),
                (0, D // 8, load_tokens), (2, 16, fwd_butterflies)],
               in_step, NT // 2, first_mod)

    def filt_a(t):
        a = pltpu.bitcast(wr_v[0:DF - 1, lanes(t)], f32)
        b = pltpu.bitcast(wi_v[0:DF - 1, lanes(t)], f32)
        nr = wr_v[DF - 1:DF, lanes(t)].astype(f32)
        ni = wi_v[DF - 1:DF, lanes(t)].astype(f32)
        r = lax.broadcasted_iota(jnp.int32, (8, 128), 0)
        nyq = jnp.where(r == 0, nr, jnp.where(r == 1, ni, 0.0))
        rest = jnp.concatenate([a[128:], b[128:], nyq, jnp.zeros((88, 128), f32)], axis=0)
        for c, tile in enumerate((a[:128].T, b[:128].T, rest.T)):
            for j in range(8):
                lo = (NT + 1) * (8 * t + j)
                wt_v[c, lo:lo + NT, :] = tile[NT * j:NT * (j + 1)]

    def filt_b(k):
        wp_v[k, 0:128, :] = wt_v[0, pl.ds(k, 128, stride=NT + 1), :].T
        wp_v[k, 144:272, :] = wt_v[1, pl.ds(k, 128, stride=NT + 1), :].T
        rest = wt_v[2, pl.ds(k, 128, stride=NT + 1), :].T
        wp_v[k, 128:144, :] = rest[0:16]
        wp_v[k, 272:296, :] = rest[16:40]

    def filt(k, rb, base, nyq_row):
        if rb == NRB - 1:
            return jnp.broadcast_to(wp_v[k, nyq_row:nyq_row + 1, :], (8, 128))
        k0 = _row_runs()[rb // 2]
        w = pltpu.bitcast(wp_v[k, pl.ds(base + k0 // 2 + 72 * (rb % 2), 8, stride=9), :], u32)
        w = (w & np.uint32(0xFFFF0000)) if k0 % 2 else (w << 16)
        return pltpu.bitcast(w, f32)

    groups = [range(8 * g, min(8 * g + 8, NRB)) for g in range(5)]

    def rows(rbs):
        return slice(16 * rbs[0], 16 * rbs[-1] + 16)

    def fwd_channel(g, t):
        if g < 4:
            fa_v[t, lanes(g), :] = _dot(_halves(chm_v[g]), r_v[t, lanes(g), :])
        else:
            rhs = jnp.concatenate([r_v[t, 512:576, :], jnp.zeros((64, 128), bf16)], axis=0)
            fa_v[t, 512:592, :] = _dot(_halves(chm_v[4, 0:40, :]), rhs)

    def inv_channel(g, t):
        if g < 4:
            fc_v[t, lanes(g), :] = _dot(_halves(chm_v[5 + g]), fd_v[t, lanes(g), :])
        else:
            rhs = jnp.concatenate([fd_v[t, 512:592, :], jnp.zeros((48, 128), bf16)], axis=0)
            fc_v[t, 512:576, :] = _dot(_halves(chm_v[9, 0:32, :]), rhs)

    def butterflies(src, dst, sign, rb):
        z = [(src[t, blk(2 * rb), :], src[t, blk(2 * rb + 1), :]) for t in range(NT)]
        for k, (re, im) in enumerate(_radix16(z, sign)):
            dst[k, 16 * rb:16 * rb + 16, :] = _pair(re, im)

    def fwd_token(rbs, k):
        lhs = fb_v[k, rows(rbs), :]
        p, q = _dot(lhs, mf_v[k, 0]), _dot(lhs, mf_v[k, 1])
        for i, rb in enumerate(rbs):
            re, im = blk(2 * i), blk(2 * i + 1)
            fc_v[k, blk(2 * rb), :] = p[re] - q[im]
            fc_v[k, blk(2 * rb + 1), :] = q[re] + p[im]

    def inv_token(rbs, k):
        z = []
        for rb in rbs:
            yr, yi = fc_v[k, blk(2 * rb), :], fc_v[k, blk(2 * rb + 1), :]
            wr, wi = filt(k, rb, 0, 288), filt(k, rb, 144, 289)
            z += [yr * wr - yi * wi, yr * wi + yi * wr]
        lhs = jnp.concatenate(z, axis=0).astype(bf16)
        p, q = _dot(lhs, mi_v[k, 0]), _dot(lhs, mi_v[k, 1])
        for i, rb in enumerate(rbs):
            re, im = blk(2 * i), blk(2 * i + 1)
            fa_v[k, blk(2 * rb), :] = p[re] + q[im]
            fa_v[k, blk(2 * rb + 1), :] = p[im] - q[re]

    def spread(items, i, n=NT):
        return items[len(items) * i // n:len(items) * (i + 1) // n]

    def filt_step(i):
        if i < NT and i % (NT // WCH) == 0:
            cp_w[2 * i * WCH // NT].wait()
            cp_w[2 * i * WCH // NT + 1].wait()
        (filt_a if i < NT else filt_b)(i % NT)

    with jax.named_scope("F"):
        cp_chm[0].wait()
        for g in range(5):
            for k in range(NT):
                fwd_channel(g, k)
                for rb in spread(groups[g - 1] if g else (), k):
                    butterflies(fa_v, fb_v, -1, rb)
        for k in range(NT):
            fwd_token(range(32), k)
            for rb in spread(groups[4], k):
                butterflies(fa_v, fb_v, -1, rb)
            filt_step(2 * k)
            filt_step(2 * k + 1)
        for k in range(NT):
            fwd_token(groups[4], k)
    with jax.named_scope("I"):
        cp_chm[1].wait()
        cp_mod[1].wait()
        for g in range(5):
            for k in range(NT):
                inv_token(groups[g], k)
                for rb in spread(groups[g - 1] if g else (), k):
                    butterflies(fa_v, fd_v, +1, rb)
        for g in range(5):
            for k in range(NT):
                inv_channel(g, k)
                for rb in spread(() if g else groups[4], k):
                    butterflies(fa_v, fd_v, +1, rb)
                for j in spread(range(*MOD_PARTS[1]), NT * g + k, 5 * NT):
                    store_mod(j)

    def opposite(j):
        return j, j + NT // 2

    def residual(t):
        for p in range(8):
            uv = [(fc_v[t, blk(16 * g + 2 * p), :], fc_v[t, blk(16 * g + 2 * p + 1), :])
                  for g in range(4)]
            for a, y in enumerate(_radix9_t(fc_v[t, blk(64 + p), :], uv)):
                b = 8 * a + p
                x1 = x1_v[t, blk(b), :] + mod(2, b) * y
                x1_v[t, blk(b), :] = x1
                yield x1

    def modulated(t):
        rstd = st_v[1, t]
        for b in range(D // 8):
            h = fa_v[t, blk(b), :] * rstd * mod(4, b) + mod(3, b)
            fc_v[t, blk(b), :] = h
            yield h

    def mlp_operands(j):
        stats = [(t, st_v[2, t], st_v[3, t]) for t in opposite(j)]
        for r in range(0, D // 2, 16):
            quads = [jnp.concatenate([(fc_v[t, q:q + 8, :] - mean) * rstd for q in (lo, lo + 8)],
                                     axis=0)
                     for lo in (r, D // 2 + r) for t, mean, rstd in stats]
            for i, a in enumerate(_lhs_forms(*quads)):
                a_v[i, r:r + 16, lanes(j)] = a.astype(bf16)
            yield

    with jax.named_scope("C"):
        skewed([(1, D // 8, lambda j: stage(opposite(j), 1, squares(x1_v, 0, fa_v), inv_std)),
                (0, D // 8, lambda j: stage(opposite(j), 0, residual))], in_turn, NT // 2)
        skewed([(2, 18, mlp_operands),
                (1, D // 8, lambda j: stage(opposite(j), 3, squares(fc_v, 2), inv_std)),
                (0, D // 8, lambda j: stage(opposite(j), 2, modulated))], in_turn, NT // 2)

    hs = S // 2

    def hidden(j):
        lo, n = STARTS[j], CHUNKS[j] // 2
        prods = []
        for i in range(7):
            if i == 2:
                for c in late.get(j, ()):
                    c.wait()
            prods.append(_dot(a_v[i], _rhs_form(i, lambda r, c: w1_v[
                r * hs:(r + 1) * hs, lo + c * n:lo + (c + 1) * n])))
        u11, u12, u21, u22 = _out_forms(prods)
        bias = [b1[t:t + 1, :] for t in range(lo // 128, (lo + 2 * n) // 128)]
        bl = jnp.concatenate(bias[:n // 128], axis=1)
        br = jnp.concatenate(bias[n // 128:], axis=1)
        lhs = _lhs_forms(_gelu(u11 + bl), _gelu(u12 + br), _gelu(u21 + bl), _gelu(u22 + br))
        return [a.astype(bf16) for a in lhs]

    def product(j, i, lhs, lo, n):
        top, m = STARTS[j], CHUNKS[j] // 2
        return _dot(lhs[i], _rhs_form(i, lambda r, c: w2_v[
            top + r * m:top + (r + 1) * m, c * hs + lo:c * hs + lo + n]))

    late = {1: (cp_w2[1], cp_w1[2]), 2: (*cp_w2[2:4], *cp_w1[3:]), 3: (cp_w2[4],)}
    with jax.named_scope("MLP"):
        for c in (cp_b1, cp_b2, cp_w1[0], cp_w2[0], cp_w1[1]):
            c.wait()
        b1, b2 = b1_v[...].astype(f32), b2_v[...].astype(f32)
        last = len(CHUNKS) - 1
        for j in range(last):
            lhs = hidden(j)
            for i in range(7):
                if j == 0:
                    acc_v[i] = product(j, i, lhs, 0, hs)
                else:
                    acc_v[i] += product(j, i, lhs, 0, hs)
        lhs = hidden(last)
        for j in range(NT // 2):
            y11, y12, y21, y22 = _out_forms(
                [acc_v[i, :, lanes(j)] + product(last, i, lhs, 128 * j, 128) for i in range(7)])
            for t, top, bot in zip(opposite(j), (y11, y12), (y21, y22)):
                y = jnp.concatenate([top, bot], axis=0) + b2[t:t + 1, :]
                o_v[:, lanes(t)] = (x1_v[t] + mod(5) * y).astype(bf16)
                cp_o[t].start()
        for c in cp_o:
            c.wait()


@jax.jit
def pallas_adaLN_cond__spectral_gfnet__mixer_token_mlp__prompt_kernel(
    A_x: jax.Array,
    A_w_r: jax.Array,
    A_w_i: jax.Array,
    B_x: jax.Array,
    B_w1: jax.Array,
    B_b1: jax.Array,
    B_w2: jax.Array,
    B_b2: jax.Array,
    c: jax.Array,
    w_mod: jax.Array,
):
    del B_x
    vmem = pltpu.VMEM
    scratch = [
        vmem((D, S), bf16), vmem((DF, S), bf16), vmem((DF, S), bf16),
        vmem((S, F), bf16), vmem((F // 128, 128), bf16),
        vmem((F, S), bf16), vmem((S // 128, 128), bf16),
        vmem((1, D), bf16), vmem((D, 6 * D), bf16),
        vmem(_CH_MATS.shape, u32), vmem(_TOK_TAB.shape, f32),
        vmem((6 * D, 128), f32),
        vmem((NT, 2, 128, 128), bf16),
        vmem((NT, 2, 128, 128), bf16),
        vmem((3, S + 128, 128), f32),
        vmem((NT, 296, 128), f32),
        vmem((NT, D, 128), bf16),
        vmem((NT, NRB * 16, 128), f32),
        vmem((NT, NRB * 16, 128), bf16),
        vmem((NT, NRB * 16, 128), f32),
        vmem((NT, NRB * 16, 128), bf16),
        vmem((NT, D, 128), f32),
        vmem((7, D // 2, S // 2), bf16),
        vmem((7, D // 2, S // 2), f32),
        vmem((D, S), bf16),
        vmem((40, 128), f32),
        vmem((4, NT, 8, 128), f32),
        pltpu.SemaphoreType.DMA((64,)),
    ]
    out = pl.pallas_call(
        _kernel,
        in_specs=[pl.BlockSpec(memory_space=pl.ANY)] * 11,
        out_specs=pl.BlockSpec(memory_space=pl.ANY),
        out_shape=jax.ShapeDtypeStruct((D, S), bf16),
        scratch_shapes=scratch,
        compiler_params=pltpu.CompilerParams(vmem_limit_bytes=120 * 1024 * 1024),
    )(A_x[0].T, A_w_r.T, A_w_i.T, B_w1, B_b1.reshape(F // 128, 128), B_w2,
      B_b2.reshape(S // 128, 128), c, w_mod, _CH_MATS, _TOK_TAB)
    return out.T[None]
```

```python
import itertools

import jax
import jax.numpy as jnp
import numpy as np
from jax import lax
from jax.experimental import pallas as pl
from jax.experimental.pallas import tpu as pltpu

D, S, F = 576, 2048, 4608
DF = D // 2 + 1
NT = S // 128
NRB = 37
EPS = 1e-5
CHUNKS = (512, 1024, 1024, 1024, 1024)
STARTS = tuple(sum(CHUNKS[:j]) for j in range(len(CHUNKS)))
MOD_PARTS = ((0, 9), (9, 27))

f32, bf16, u32 = jnp.float32, jnp.bfloat16, jnp.uint32

_Q = np.sqrt(3.0) / 2
_C1, _C2, _C4 = (float(np.cos(2 * np.pi * k / 9)) for k in (1, 2, 4))
_S1, _S2, _S4 = (float(np.sin(2 * np.pi * k / 9) / _Q) for k in (1, 2, 4))


def _row_runs():
    runs = []
    for g in (1, 2, 3, 4):
        for r in (g, 9 - g):
            runs += [r, r + 9]
    return runs + [0, 9]


def _pack_rows(m):
    b = m.astype(np.float32).astype(jnp.bfloat16).view(np.uint16).astype(np.uint32)
    return b[..., 0::2, :] | (b[..., 1::2, :] << np.uint32(16))


def _channel_mats():
    kd_all = [k0 + 18 * j for k0 in _row_runs() for j in range(16)] + [D // 2] + [-1] * 7
    kd_all = np.array(kd_all)
    b = np.arange(64)
    mats = np.zeros((10, 128, 128))
    for g in (1, 2, 3, 4):
        kd = kd_all[64 * (g - 1):64 * g]
        sg = np.where(kd % 9 == g, -1.0, 1.0).reshape(8, 8, 1, 1)
        th = (2 * np.pi / D) * ((kd[:, None] * b[None, :]) % D)
        c, s = np.cos(th).reshape(8, 8, 8, 8), np.sin(th).reshape(8, 8, 8, 8)
        m = np.zeros((8, 2, 8, 8, 2, 8))
        m[:, 0, :, :, 0, :] = c
        m[:, 0, :, :, 1, :] = sg * _Q * s
        m[:, 1, :, :, 0, :] = -s
        m[:, 1, :, :, 1, :] = sg * _Q * c
        mats[g - 1] = m.reshape(128, 128)
        mats[5 + g - 1] = m.reshape(128, 128).T
    kd = kd_all[256:]
    valid = (kd >= 0)[:, None]
    th = (2 * np.pi / D) * ((kd[:, None] * b[None, :]) % D)
    m = np.zeros((5, 2, 8, 64))
    m[:, 0] = (np.cos(th) * valid).reshape(5, 8, 64)
    m[:, 1] = (-np.sin(th) * valid * (kd != D // 2)[:, None]).reshape(5, 8, 64)
    half = np.where((kd == 0) | (kd == D // 2), 0.5, 1.0).reshape(5, 1, 8, 1)
    mats[4, :80, :64] = m.reshape(80, 64)
    mats[9, :64, :80] = (m * half).reshape(80, 64).T
    return _pack_rows(mats)


def _token_tables():
    l = np.arange(128)
    ones = np.ones((8, 1))
    angles = [(2 * np.pi / 128) * ((l[:8, None] * l[None, :]) % 128),
              (2 * np.pi / 128) * ((8 * l) % 128) * ones, (2 * np.pi / S) * l * ones]
    return np.concatenate([p for a in angles for p in (np.cos(a), -np.sin(a))]).astype(np.float32)


_CH_MATS = _channel_mats()
_TOK_TAB = _token_tables()


def _dot(a, b):
    return jnp.dot(a, b, preferred_element_type=f32)


def _radix9(x):
    s1, s2, s3, s4 = x[1] + x[8], x[2] + x[7], x[3] + x[6], x[4] + x[5]
    d1, d2, d3, d4 = x[1] - x[8], x[2] - x[7], x[3] - x[6], x[4] - x[5]
    p = x[0] - 0.5 * s3
    a, b = s1 - s4, s2 - s4
    r1 = _C1 * a + _C2 * b
    r2 = _C2 * a + _C4 * b
    e, g = d1 + d2, d2 + d4
    i1 = _S1 * e + _S4 * g
    i2 = _S2 * e - _S1 * g
    t, u = s1 + s2 + s4, x[0] + s3
    return u + t, [(p + r1, i1 + d3), (p + r2, i2 - d3),
                   (u - 0.5 * t, d1 - d2 + d4), ((p - r1) - r2, (i2 - i1) + d3)]


def _radix9_t(x0, uv):
    (u1, v1), (u2, v2), (u3, v3), (u4, v4) = uv
    u, t = x0 + u3, x0 - 0.5 * u3
    p, r1, r2 = u1 + u2 + u4, u1 - u4, u2 - u4
    a = _C1 * r1 + _C2 * r2
    b = _C2 * r1 + _C4 * r2
    s1, s2, s3, s4 = t + a, t + b, u - 0.5 * p, (t - a) - b
    i1, i2, d3 = v1 - v4, v2 + v4, v1 - v2 + v4
    e = _S1 * i1 + _S2 * i2
    g = _S4 * i1 - _S1 * i2
    d1, d2, d4 = e + v3, (e + g) - v3, g + v3
    return [u + p, s1 + d1, s2 + d2, s3 + d3, s4 + d4, s4 - d4, s3 - d3, s2 - d2, s1 - d1]


def _cadd(a, b):
    return a[0] + b[0], a[1] + b[1]


def _csub(a, b):
    return a[0] - b[0], a[1] - b[1]


def _cmul(a, b):
    return a[0] * b[0] - a[1] * b[1], a[0] * b[1] + a[1] * b[0]


def _cross(a, b):
    return (a[0] - b[1], a[1] + b[0]), (a[0] + b[1], a[1] - b[0])


def _radix4(x, sign):
    a, b, c, d = x
    u, v = _cadd(a, c), _cadd(b, d)
    k1, k3 = _cross(_csub(a, c), _csub(b, d))[::sign]
    return [_cadd(u, v), k1, _csub(u, v), k3]


def _twiddle16(z, e, sign):
    re, im = z
    if e == 0:
        return z
    c, s = float(np.cos(2 * np.pi * e / 16)), float(sign * np.sin(2 * np.pi * e / 16))
    if e == 4:
        return (-im, re) if sign > 0 else (im, -re)
    if e % 2 == 0:
        if c * s > 0:
            return c * (re - im), c * (re + im)
        return c * (re + im), c * (im - re)
    return c * re - s * im, s * re + c * im


def _halves(w):
    return pltpu.bitcast(w, bf16)


def _pair(a, b):
    return jnp.concatenate([a, b], axis=0).astype(bf16)


class _RowMean:
    def __init__(self, lanes=2):
        self.acc, self.n = [None] * lanes, 0

    def add(self, v):
        i = self.n % len(self.acc)
        self.acc[i] = v if self.acc[i] is None else self.acc[i] + v
        self.n += 1

    def mean(self):
        acc = self.acc
        while len(acc) > 1:
            acc = [acc[i] + acc[i + 1] for i in range(0, len(acc), 2)]
        return jnp.sum(acc[0], axis=0, keepdims=True) * (1.0 / D)


def _gelu(x):
    inner = x * (0.7978845608028654 + (0.7978845608028654 * 0.044715) * (x * x))
    hx = 0.5 * x
    return hx + hx * jnp.tanh(inner)


def _lhs_forms(a11, a12, a21, a22):
    return [a11 + a22, a21 + a22, a11, a22, a11 + a12, a21 - a11, a12 - a22]


def _rhs_form(i, quad):
    if i in (1, 4):
        return quad(i // 4, i // 4)
    a, sign, b = {0: ((0, 0), 1, (1, 1)), 2: ((0, 1), -1, (1, 1)), 3: ((1, 0), -1, (0, 0)),
                  5: ((0, 0), 1, (0, 1)), 6: ((1, 0), 1, (1, 1))}[i]
    a, b = quad(*a).astype(f32), quad(*b).astype(f32)
    return (a + b if sign > 0 else a - b).astype(bf16)


def _out_forms(m):
    return m[0] + m[3] - m[4] + m[6], m[2] + m[4], m[1] + m[3], m[0] - m[1] + m[2] + m[5]


def _kernel(x_hbm, wr_hbm, wi_hbm, w1_hbm, b1_hbm, w2_hbm, b2_hbm, c_hbm, wm_hbm, chm_hbm, tok_hbm,
            o_hbm,
            x_v, wr_v, wi_v, w1_v, b1_v, w2_v, b2_v, c_v, wm_v, chm_v, tok_v,
            mod_v, mf_v, mi_v, wt_v, wp_v, r_v, fa_v, fc_v, x1_v, a_v, acc_v, o_v, st_v,
            sem):
    slots = itertools.count()

    def copy(src, dst):
        return pltpu.make_async_copy(src, dst, sem.at[next(slots)])

    def cols(ref, lo, n):
        return ref.at[:, pl.ds(lo, n)]

    def copy_cols(src, dst, lo, n):
        return copy(cols(src, lo, n), cols(dst, lo, n))

    cp_tok, cp_c = copy(tok_hbm, tok_v), copy(c_hbm, c_v)
    cp_mod = [copy_cols(wm_hbm, wm_v, 128 * lo, 128 * (hi - lo)) for lo, hi in MOD_PARTS]
    cp_chm = [copy(chm_hbm.at[pl.ds(5 * i, 5)], chm_v.at[pl.ds(5 * i, 5)]) for i in range(2)]
    cp_w = [copy(wr_hbm, wr_v), copy(wi_hbm, wi_v)]
    cp_b1, cp_b2 = copy(b1_hbm, b1_v), copy(b2_hbm, b2_v)
    cp_w1 = [copy_cols(w1_hbm, w1_v, lo, n) for lo, n in zip(STARTS, CHUNKS)]
    cp_w2 = [copy(w2_hbm.at[pl.ds(lo, n)], w2_v.at[pl.ds(lo, n)]) for lo, n in zip(STARTS, CHUNKS)]
    cp_o = [copy(o_v.at[t], cols(o_hbm, 128 * t, 128)) for t in range(NT)]
    sem_x = next(slots)

    def cp_x(i):
        lo = i * 256 if isinstance(i, int) else pl.multiple_of(i * 256, 256)
        return pltpu.make_async_copy(cols(x_hbm, lo, 256), cols(x_v, lo, 256), sem.at[sem_x + i])

    for c in (cp_tok, cp_c, cp_x(0), cp_x(1), cp_mod[0], *map(cp_x, range(2, NT // 2)), cp_chm[0],
              *cp_w, cp_chm[1], cp_mod[1], cp_b1, cp_b2, *itertools.chain(*zip(cp_w1, cp_w2))):
        c.start()

    def lanes(t):
        if isinstance(t, int):
            return slice(128 * t, 128 * (t + 1))
        return pl.ds(pl.multiple_of(t * 128, 128), 128)

    def blk(i):
        return slice(8 * i, 8 * i + 8)

    with jax.named_scope("gen"):
        cp_tok.wait()
        rows = [(tok_v[blk(0), :], tok_v[blk(1), :])]
        for _ in range(15):
            rows.append(_cmul(rows[-1], (tok_v[blk(2), :], tok_v[blk(3), :])))
        dft = tuple(jnp.concatenate([r[i] for r in rows], axis=0) for i in range(2))
        along = tuple(jnp.concatenate([tok_v[blk(i), :]] * 16, axis=0) for i in (4, 5))
        down = tuple(a.T for a in along)

        def gen(k, carry):
            for ref, m in zip((mf_v, mi_v), carry):
                ref[k, 0], ref[k, 1] = m[0].astype(bf16), m[1].astype(bf16)
            return _cmul(carry[0], down), _cmul(carry[1], along)

        lax.fori_loop(0, NT, gen, (dft, dft))

    cp_c.wait()
    cf = c_v[...].astype(f32)
    sc = jnp.broadcast_to(cf * jax.nn.sigmoid(cf), (16, D)).astype(bf16)

    def store_mod(j):
        row = _dot(sc, wm_v[:, lanes(j)])[0:8, :]
        n = 128 * j + lax.broadcasted_iota(jnp.int32, row.shape, 1)
        scale = jnp.logical_or(jnp.logical_and(n >= D, n < 2 * D),
                               jnp.logical_and(n >= 4 * D, n < 5 * D))
        row = jnp.where(scale, row + 1.0, row)
        row = jnp.where(jnp.logical_and(n >= 2 * D, n < 3 * D), row * (2.0 / (S * D)), row)
        mod_v[lanes(j), :] = jnp.concatenate([row] * 16, axis=0).T

    def mod(i, b=None):
        return mod_v[i * D:(i + 1) * D, :] if b is None else mod_v[blk(i * D // 8 + b), :]

    def first_mod():
        cp_mod[0].wait()
        for j in range(*MOD_PARTS[0]):
            store_mod(j)

    def stage(pair, slot, values, finish=lambda m: m):
        means = [_RowMean() for _ in pair]
        for vs in zip(*map(values, pair)):
            for m, v in zip(means, vs):
                m.add(v)
            yield
        for t, m in zip(pair, means):
            st_v[slot, t] = jnp.broadcast_to(finish(m.mean()), (8, 128))

    def in_turn(gens):
        for g, _ in gens:
            for _ in g:
                pass

    def in_step(gens):
        n = D // 8
        for q in range(n):
            for g, cuts in gens:
                for _ in range(cuts * q // n, cuts * (q + 1) // n):
                    next(g)
        in_turn(gens)

    def skewed(stages, emit, n, after_fill=lambda: None):
        depth = len(stages) - 1

        def step(oldest, lo, hi):
            emit([(fn(oldest + (depth - lag)), cuts)
                  for lag, cuts, fn in stages if lo <= lag <= hi])

        for i in range(depth):
            step(i - depth, 0, i)
        after_fill()
        lax.fori_loop(0, n - depth, lambda i, _: step(i, 0, depth), None)
        for i in range(n, n + depth):
            step(i - depth, i - n + 1, depth)

    def inv_std(var):
        return lax.rsqrt(var + EPS)

    def squares(src, slot, dst=None):
        def values(t):
            mean = st_v[slot, t]
            for b in range(D // 8):
                c = src[t, blk(b), :] - mean
                if dst is not None:
                    dst[t, blk(b), :] = c
                yield c * c
        return values

    def adjacent(i):
        return 2 * i, 2 * i + 1

    def tokens(t):
        for i in range(D // 16):
            x = x_v[16 * i:16 * i + 16, lanes(t)].astype(f32)
            for b, half in enumerate((x[:8], x[8:]), 2 * i):
                x1_v[t, blk(b), :] = half
                yield half

    def load_tokens(i):
        cp_x(i).wait()
        return stage(adjacent(i), 0, tokens)

    def fwd_butterflies(i):
        for t in adjacent(i):
            rstd = st_v[1, t]
            for p in range(8):
                x0, uv = _radix9([fc_v[t, blk(b), :] * rstd * mod(1, b) + mod(0, b)
                                  for b in range(p, D // 8, 8)])
                for g in range(4):
                    r_v[t, 128 * g + 16 * p:128 * g + 16 * p + 16, :] = _pair(*uv[g])
                if p % 2:
                    r_v[t, 504 + 8 * p:520 + 8 * p, :] = _pair(prev, x0)
                prev = x0
                yield

    with jax.named_scope("A"):
        skewed([(1, D // 8, lambda i: stage(adjacent(i), 1, squares(x1_v, 0, fc_v), inv_std)),
                (0, D // 8, load_tokens), (2, 16, fwd_butterflies)],
               in_step, NT // 2, first_mod)

    def filt_a(t):
        a = pltpu.bitcast(wr_v[0:DF - 1, lanes(t)], f32)
        b = pltpu.bitcast(wi_v[0:DF - 1, lanes(t)], f32)
        nr = wr_v[DF - 1:DF, lanes(t)].astype(f32)
        ni = wi_v[DF - 1:DF, lanes(t)].astype(f32)
        r = lax.broadcasted_iota(jnp.int32, (8, 128), 0)
        nyq = jnp.where(r == 0, nr, jnp.where(r == 1, ni, 0.0))
        rest = jnp.concatenate([a[128:], b[128:], nyq, jnp.zeros((88, 128), f32)], axis=0)
        for c, tile in enumerate((a[:128].T, b[:128].T, rest.T)):
            for j in range(8):
                lo = (NT + 1) * (8 * t + j)
                wt_v[c, lo:lo + NT, :] = tile[NT * j:NT * (j + 1)]

    def filt_b(k):
        wp_v[k, 0:128, :] = wt_v[0, pl.ds(k, 128, stride=NT + 1), :].T
        wp_v[k, 144:272, :] = wt_v[1, pl.ds(k, 128, stride=NT + 1), :].T
        rest = wt_v[2, pl.ds(k, 128, stride=NT + 1), :].T
        wp_v[k, 128:144, :] = rest[0:16]
        wp_v[k, 272:296, :] = rest[16:40]

    def filt(k, rb, base, nyq_row):
        if rb == NRB - 1:
            return jnp.broadcast_to(wp_v[k, nyq_row:nyq_row + 1, :], (8, 128))
        k0 = _row_runs()[rb // 2]
        w = pltpu.bitcast(wp_v[k, pl.ds(base + k0 // 2 + 72 * (rb % 2), 8, stride=9), :], u32)
        w = (w & np.uint32(0xFFFF0000)) if k0 % 2 else (w << 16)
        return pltpu.bitcast(w, f32)

    groups = [range(8 * g, min(8 * g + 8, NRB)) for g in range(5)]
    rounds = [(q, odd) for q in range(4) for odd in (0, 1)]

    def harmonics(q, odd):
        return q + 4 * odd, q + 4 * odd + 8

    def get(ref, i, rb):
        return ref[i, blk(2 * rb), :], ref[i, blk(2 * rb + 1), :]

    def put(ref, i, rb, z):
        ref[i, blk(2 * rb), :], ref[i, blk(2 * rb + 1), :] = z

    def token_dft(z, m_ref, k, sign):
        lhs = jnp.concatenate([v for pair in z for v in pair], axis=0).astype(bf16)
        p, q = _dot(lhs, m_ref[k, 0]), _dot(lhs, m_ref[k, 1])
        out = []
        for rb in range(NRB):
            re, im = blk(2 * rb), blk(2 * rb + 1)
            out.append((p[re] - q[im], q[re] + p[im]) if sign < 0
                       else (p[re] + q[im], p[im] - q[re]))
        return out

    def fwd_channel(g, t0):
        tiles = range(t0, NT, 4)
        if g < 4:
            outs = [_dot(_halves(chm_v[g]), r_v[t, lanes(g), :]) for t in tiles]
        else:
            pad = jnp.zeros((64, 128), bf16)
            outs = [_dot(_halves(chm_v[4, 0:40, :]),
                         jnp.concatenate([r_v[t, 512:576, :], pad], axis=0)) for t in tiles]
        for i, rb in enumerate(groups[g]):
            y = _radix4([(o[blk(2 * i)], o[blk(2 * i + 1)]) for o in outs], -1)
            for q in range(4):
                put(fa_v, 4 * q + t0, rb, _twiddle16(y[q], t0 * q, -1))

    def fwd_token(q, odd):
        z = []
        for rb in range(NRB):
            a, b, c, d = (get(fa_v, 4 * q + t0, rb) for t0 in range(4))
            if odd:
                z.append(_cross(_csub(a, c), _csub(b, d))[::-1])
            else:
                u, v = _cadd(a, c), _cadd(b, d)
                z.append((_cadd(u, v), _csub(u, v)))
        for k, zk in zip(harmonics(q, odd), zip(*z)):
            for rb, y in enumerate(token_dft(zk, mf_v, k, -1)):
                put(fc_v, k, rb, y)

    def inv_token(q, odd):
        outs = []
        for k in harmonics(q, odd):
            z = [_cmul(get(fc_v, k, rb), (filt(k, rb, 0, 288), filt(k, rb, 144, 289)))
                 for rb in range(NRB)]
            outs.append(token_dft(z, mi_v, k, +1))
        for rb, (a, c) in enumerate(zip(*outs)):
            u, v = _cadd(a, c), _csub(a, c)
            if odd:
                p, m = get(fa_v, q, rb), get(fa_v, 4 + q, rb)
                y1, y3 = _cross(m, v)
                for t0, y in enumerate((_cadd(p, u), y1, _csub(p, u), y3)):
                    put(fa_v, 4 * t0 + q, rb, _twiddle16(y, t0 * q, +1))
            else:
                put(fa_v, q, rb, u)
                put(fa_v, 4 + q, rb, v)

    def inv_channel(g, t0):
        z = [_radix4([get(fa_v, 4 * t0 + q, rb) for q in range(4)], +1) for rb in groups[g]]
        for t, zt in zip(range(t0, NT, 4), zip(*z)):
            parts = [v for pair in zt for v in pair]
            if g < 4:
                fc_v[t, lanes(g), :] = _dot(_halves(chm_v[5 + g]),
                                            jnp.concatenate(parts, axis=0).astype(bf16))
            else:
                parts.append(jnp.zeros((48, 128), f32))
                fc_v[t, 512:576, :] = _dot(_halves(chm_v[9, 0:32, :]),
                                           jnp.concatenate(parts, axis=0).astype(bf16))

    with jax.named_scope("F"):
        cp_chm[0].wait()
        for g in range(5):
            for t0 in range(4):
                fwd_channel(g, t0)
        for i, r in enumerate(rounds):
            if i == 2:
                for c in cp_w:
                    c.wait()
            fwd_token(*r)
            if 2 <= i < 6:
                for t in range(4 * i - 8, 4 * i - 4):
                    filt_a(t)
            elif i >= 6:
                for k in harmonics(*rounds[2 * i - 12]) + harmonics(*rounds[2 * i - 11]):
                    filt_b(k)
    with jax.named_scope("I"):
        for i, r in enumerate(rounds):
            if i < 4:
                for k in harmonics(*rounds[i + 4]):
                    filt_b(k)
            inv_token(*r)
        cp_chm[1].wait()
        cp_mod[1].wait()
        lo, hi = MOD_PARTS[1]
        for i in range(20):
            inv_channel(*divmod(i, 4))
            if lo + i < hi:
                store_mod(lo + i)

    def opposite(j):
        return j, j + NT // 2

    def residual(t):
        for p in range(8):
            uv = [(fc_v[t, blk(16 * g + 2 * p), :], fc_v[t, blk(16 * g + 2 * p + 1), :])
                  for g in range(4)]
            for a, y in enumerate(_radix9_t(fc_v[t, blk(64 + p), :], uv)):
                b = 8 * a + p
                x1 = x1_v[t, blk(b), :] + mod(2, b) * y
                x1_v[t, blk(b), :] = x1
                yield x1

    def modulated(t):
        rstd = st_v[1, t]
        for b in range(D // 8):
            h = fa_v[t, blk(b), :] * rstd * mod(4, b) + mod(3, b)
            fc_v[t, blk(b), :] = h
            yield h

    def mlp_operands(j):
        stats = [(t, st_v[2, t], st_v[3, t]) for t in opposite(j)]
        for r in range(0, D // 2, 16):
            quads = [jnp.concatenate([(fc_v[t, q:q + 8, :] - mean) * rstd for q in (lo, lo + 8)],
                                     axis=0)
                     for lo in (r, D // 2 + r) for t, mean, rstd in stats]
            for i, a in enumerate(_lhs_forms(*quads)):
                a_v[i, j, r:r + 16, :] = a.astype(bf16)
            yield

    with jax.named_scope("C"):
        skewed([(1, D // 8, lambda j: stage(opposite(j), 1, squares(x1_v, 0, fa_v), inv_std)),
                (0, D // 8, lambda j: stage(opposite(j), 0, residual))], in_turn, NT // 2)
        skewed([(2, 18, mlp_operands),
                (1, D // 8, lambda j: stage(opposite(j), 3, squares(fc_v, 2), inv_std)),
                (0, D // 8, lambda j: stage(opposite(j), 2, modulated))], in_turn, NT // 2)

    hs = S // 2

    def hidden(j):
        lo, n = STARTS[j], CHUNKS[j] // 2
        for c in needed.get(j, ()):
            c.wait()
        prods = []
        for i in range(7):
            lhs = jnp.concatenate([a_v[i, t] for t in range(NT // 2)], axis=1)
            prods.append(_dot(lhs, _rhs_form(i, lambda r, c: w1_v[
                r * hs:(r + 1) * hs, lo + c * n:lo + (c + 1) * n])))
        u11, u12, u21, u22 = _out_forms(prods)
        bias = [b1[t:t + 1, :] for t in range(lo // 128, (lo + 2 * n) // 128)]
        bl = jnp.concatenate(bias[:n // 128], axis=1)
        br = jnp.concatenate(bias[n // 128:], axis=1)
        lhs = _lhs_forms(_gelu(u11 + bl), _gelu(u12 + br), _gelu(u21 + bl), _gelu(u22 + br))
        return [a.astype(bf16) for a in lhs]

    def product(j, i, lhs, lo, n):
        top, m = STARTS[j], CHUNKS[j] // 2
        return _dot(lhs[i], _rhs_form(i, lambda r, c: w2_v[
            top + r * m:top + (r + 1) * m, c * hs + lo:c * hs + lo + n]))

    needed = {1: (cp_w1[1], cp_w2[1]), 2: (cp_w1[2], cp_w2[2]), 3: (*cp_w1[3:], *cp_w2[3:])}
    with jax.named_scope("MLP"):
        for c in (cp_b1, cp_b2, cp_w1[0], cp_w2[0]):
            c.wait()
        b1, b2 = b1_v[...].astype(f32), b2_v[...].astype(f32)
        last = len(CHUNKS) - 1
        for j in range(last):
            lhs = hidden(j)
            for i in range(7):
                if j == 0:
                    acc_v[i] = product(j, i, lhs, 0, hs)
                else:
                    acc_v[i] += product(j, i, lhs, 0, hs)
        lhs = hidden(last)
        for j in range(NT // 2):
            y11, y12, y21, y22 = _out_forms(
                [acc_v[i, :, lanes(j)] + product(last, i, lhs, 128 * j, 128) for i in range(7)])
            for t, top, bot in zip(opposite(j), (y11, y12), (y21, y22)):
                y = jnp.concatenate([top, bot], axis=0) + b2[t:t + 1, :]
                o_v[t] = (x1_v[t] + mod(5) * y).astype(bf16)
                cp_o[t].start()
        for c in cp_o:
            c.wait()


@jax.jit
def pallas_adaLN_cond__spectral_gfnet__mixer_token_mlp__prompt_kernel(
    A_x: jax.Array,
    A_w_r: jax.Array,
    A_w_i: jax.Array,
    B_x: jax.Array,
    B_w1: jax.Array,
    B_b1: jax.Array,
    B_w2: jax.Array,
    B_b2: jax.Array,
    c: jax.Array,
    w_mod: jax.Array,
):
    del B_x
    vmem = pltpu.VMEM
    scratch = [
        vmem((D, S), bf16), vmem((DF, S), bf16), vmem((DF, S), bf16),
        vmem((S, F), bf16), vmem((F // 128, 128), bf16),
        vmem((F, S), bf16), vmem((S // 128, 128), bf16),
        vmem((1, D), bf16), vmem((D, 6 * D), bf16),
        vmem(_CH_MATS.shape, u32), vmem(_TOK_TAB.shape, f32),
        vmem((6 * D, 128), f32),
        vmem((NT, 2, 128, 128), bf16),
        vmem((NT, 2, 128, 128), bf16),
        vmem((3, S + 128, 128), f32),
        vmem((NT, 296, 128), f32),
        vmem((NT, D, 128), bf16),
        vmem((NT, NRB * 16, 128), f32),
        vmem((NT, NRB * 16, 128), f32),
        vmem((NT, D, 128), f32),
        vmem((7, NT // 2, D // 2, 128), bf16),
        vmem((7, D // 2, S // 2), f32),
        vmem((NT, D, 128), bf16),
        vmem((4, NT, 8, 128), f32),
        pltpu.SemaphoreType.DMA((64,)),
    ]
    out = pl.pallas_call(
        _kernel,
        in_specs=[pl.BlockSpec(memory_space=pl.ANY)] * 11,
        out_specs=pl.BlockSpec(memory_space=pl.ANY),
        out_shape=jax.ShapeDtypeStruct((D, S), bf16),
        scratch_shapes=scratch,
        compiler_params=pltpu.CompilerParams(vmem_limit_bytes=120 * 1024 * 1024),
    )(A_x[0].T, A_w_r.T, A_w_i.T, B_w1, B_b1.reshape(F // 128, 128), B_w2,
      B_b2.reshape(S // 128, 128), c, w_mod, _CH_MATS, _TOK_TAB)
    return out.T[None]
```

```python
import itertools

import jax
import jax.numpy as jnp
import numpy as np
from jax import lax
from jax.experimental import pallas as pl
from jax.experimental.pallas import tpu as pltpu

D, S, F = 576, 2048, 4608
DF = D // 2 + 1
NT = S // 128
NRB = 37
EPS = 1e-5
HB, SB = D // 4, S // 4
CHUNKS = (512, 1024, 1024, 2048)
STARTS = tuple(sum(CHUNKS[:j]) for j in range(len(CHUNKS)))
MOD_PARTS = ((0, 9), (9, 27))

f32, bf16, u32 = jnp.float32, jnp.bfloat16, jnp.uint32

_Q = np.sqrt(3.0) / 2
_C1, _C2, _C4 = (float(np.cos(2 * np.pi * k / 9)) for k in (1, 2, 4))
_S1, _S2, _S4 = (float(np.sin(2 * np.pi * k / 9) / _Q) for k in (1, 2, 4))


def _row_runs():
    runs = []
    for g in (1, 2, 3, 4):
        for r in (g, 9 - g):
            runs += [r, r + 9]
    return runs + [0, 9]


def _pack_rows(m):
    b = m.astype(np.float32).astype(jnp.bfloat16).view(np.uint16).astype(np.uint32)
    return b[..., 0::2, :] | (b[..., 1::2, :] << np.uint32(16))


def _channel_mats():
    kd_all = [k0 + 18 * j for k0 in _row_runs() for j in range(16)] + [D // 2] + [-1] * 7
    kd_all = np.array(kd_all)
    b = np.arange(64)
    mats = np.zeros((10, 128, 128))
    for g in (1, 2, 3, 4):
        kd = kd_all[64 * (g - 1):64 * g]
        sg = np.where(kd % 9 == g, -1.0, 1.0).reshape(8, 8, 1, 1)
        th = (2 * np.pi / D) * ((kd[:, None] * b[None, :]) % D)
        c, s = np.cos(th).reshape(8, 8, 8, 8), np.sin(th).reshape(8, 8, 8, 8)
        m = np.zeros((8, 2, 8, 8, 2, 8))
        m[:, 0, :, :, 0, :] = c
        m[:, 0, :, :, 1, :] = sg * _Q * s
        m[:, 1, :, :, 0, :] = -s
        m[:, 1, :, :, 1, :] = sg * _Q * c
        mats[g - 1] = m.reshape(128, 128)
        mats[5 + g - 1] = m.reshape(128, 128).T
    kd = kd_all[256:]
    valid = (kd >= 0)[:, None]
    th = (2 * np.pi / D) * ((kd[:, None] * b[None, :]) % D)
    m = np.zeros((5, 2, 8, 64))
    m[:, 0] = (np.cos(th) * valid).reshape(5, 8, 64)
    m[:, 1] = (-np.sin(th) * valid * (kd != D // 2)[:, None]).reshape(5, 8, 64)
    half = np.where((kd == 0) | (kd == D // 2), 0.5, 1.0).reshape(5, 1, 8, 1)
    mats[4, :80, :64] = m.reshape(80, 64)
    mats[9, :64, :80] = (m * half).reshape(80, 64).T
    return _pack_rows(mats)


def _token_tables():
    l = np.arange(128)
    ones = np.ones((8, 1))
    angles = [(2 * np.pi / 128) * ((l[:8, None] * l[None, :]) % 128),
              (2 * np.pi / 128) * ((8 * l) % 128) * ones, (2 * np.pi / S) * l * ones]
    return np.concatenate([p for a in angles for p in (np.cos(a), -np.sin(a))]).astype(np.float32)


_CH_MATS = _channel_mats()
_TOK_TAB = _token_tables()


def _dot(a, b):
    return jnp.dot(a, b, preferred_element_type=f32)


def _radix9(x):
    s1, s2, s3, s4 = x[1] + x[8], x[2] + x[7], x[3] + x[6], x[4] + x[5]
    d1, d2, d3, d4 = x[1] - x[8], x[2] - x[7], x[3] - x[6], x[4] - x[5]
    p = x[0] - 0.5 * s3
    a, b = s1 - s4, s2 - s4
    r1 = _C1 * a + _C2 * b
    r2 = _C2 * a + _C4 * b
    e, g = d1 + d2, d2 + d4
    i1 = _S1 * e + _S4 * g
    i2 = _S2 * e - _S1 * g
    t, u = s1 + s2 + s4, x[0] + s3
    return u + t, [(p + r1, i1 + d3), (p + r2, i2 - d3),
                   (u - 0.5 * t, d1 - d2 + d4), ((p - r1) - r2, (i2 - i1) + d3)]


def _radix9_t(x0, uv):
    (u1, v1), (u2, v2), (u3, v3), (u4, v4) = uv
    u, t = x0 + u3, x0 - 0.5 * u3
    p, r1, r2 = u1 + u2 + u4, u1 - u4, u2 - u4
    a = _C1 * r1 + _C2 * r2
    b = _C2 * r1 + _C4 * r2
    s1, s2, s3, s4 = t + a, t + b, u - 0.5 * p, (t - a) - b
    i1, i2, d3 = v1 - v4, v2 + v4, v1 - v2 + v4
    e = _S1 * i1 + _S2 * i2
    g = _S4 * i1 - _S1 * i2
    d1, d2, d4 = e + v3, (e + g) - v3, g + v3
    return [u + p, s1 + d1, s2 + d2, s3 + d3, s4 + d4, s4 - d4, s3 - d3, s2 - d2, s1 - d1]


def _cadd(a, b):
    return a[0] + b[0], a[1] + b[1]


def _csub(a, b):
    return a[0] - b[0], a[1] - b[1]


def _cmul(a, b):
    return a[0] * b[0] - a[1] * b[1], a[0] * b[1] + a[1] * b[0]


def _cross(a, b):
    return (a[0] - b[1], a[1] + b[0]), (a[0] + b[1], a[1] - b[0])


def _radix4(x, sign):
    a, b, c, d = x
    u, v = _cadd(a, c), _cadd(b, d)
    k1, k3 = _cross(_csub(a, c), _csub(b, d))[::sign]
    return [_cadd(u, v), k1, _csub(u, v), k3]


def _twiddle16(z, e, sign):
    re, im = z
    if e == 0:
        return z
    c, s = float(np.cos(2 * np.pi * e / 16)), float(sign * np.sin(2 * np.pi * e / 16))
    if e == 4:
        return (-im, re) if sign > 0 else (im, -re)
    if e % 2 == 0:
        if c * s > 0:
            return c * (re - im), c * (re + im)
        return c * (re + im), c * (im - re)
    return c * re - s * im, s * re + c * im


def _halves(w):
    return pltpu.bitcast(w, bf16)


def _pair(a, b):
    return jnp.concatenate([a, b], axis=0).astype(bf16)


class _RowMean:
    def __init__(self, lanes=2):
        self.acc, self.n = [None] * lanes, 0

    def add(self, v):
        i = self.n % len(self.acc)
        self.acc[i] = v if self.acc[i] is None else self.acc[i] + v
        self.n += 1

    def mean(self):
        acc = self.acc
        while len(acc) > 1:
            acc = [acc[i] + acc[i + 1] for i in range(0, len(acc), 2)]
        return jnp.sum(acc[0], axis=0, keepdims=True) * (1.0 / D)


def _gelu(x):
    inner = x * (0.7978845608028654 + (0.7978845608028654 * 0.044715) * (x * x))
    hx = 0.5 * x
    return hx + hx * jnp.tanh(inner)


_LEFT = (((0, 0), 1, (1, 1)), ((1, 0), 1, (1, 1)), ((0, 0), 0, None), ((1, 1), 0, None),
         ((0, 0), 1, (0, 1)), ((1, 0), -1, (0, 0)), ((0, 1), -1, (1, 1)))
_RIGHT = (((0, 0), 1, (1, 1)), ((0, 0), 0, None), ((0, 1), -1, (1, 1)), ((1, 0), -1, (0, 0)),
          ((1, 1), 0, None), ((0, 0), 1, (0, 1)), ((1, 0), 1, (1, 1)))


def _signed_sum(term, quad):
    a, sign, b = term
    if sign == 0:
        return quad(*a)
    return quad(*a) + quad(*b) if sign > 0 else quad(*a) - quad(*b)


def _operands(table, block, order=range(7)):
    for i in order:
        outer = table[i]
        if outer[1]:
            sums = {(u, v): _signed_sum(outer, lambda r, c: block(i, 2 * r + u, 2 * c + v))
                    for u in range(2) for v in range(2)}
        for j, inner in enumerate(table):
            def quad(u, v):
                if outer[1]:
                    return sums[u, v]
                return block(7 * i + j, 2 * outer[0][0] + u, 2 * outer[0][1] + v)
            yield _signed_sum(inner, quad).astype(bf16)


_RESULT = {(0, 0): {0: 1, 3: 1, 4: -1, 6: 1}, (0, 1): {2: 1, 4: 1},
           (1, 0): {1: 1, 3: 1}, (1, 1): {0: 1, 1: -1, 2: 1, 5: 1}}


def _completed(i, have):
    for quadrant, terms in _RESULT.items():
        if i in terms and all(j in have for j in terms):
            first, *rest = terms
            x = have[first]
            for j in rest:
                x = x + have[j] if terms[j] > 0 else x - have[j]
            yield quadrant, x


def _blocks(products, order=range(7)):
    outer = {quadrant: {} for quadrant in _RESULT}
    for i in order:
        inner = {}
        for j in range(7):
            inner[j] = next(products)
            for (u, v), x in _completed(j, inner):
                outer[u, v][i] = x
                for (r, c), y in _completed(i, outer[u, v]):
                    yield (2 * r + u, 2 * c + v), y


def _kernel(x_hbm, wr_hbm, wi_hbm, w1_hbm, b1_hbm, w2_hbm, b2_hbm, c_hbm, wm_hbm, chm_hbm, tok_hbm,
            o_hbm,
            x_v, wr_v, wi_v, w1_v, b1_v, w2_v, b2_v, c_v, wm_v, chm_v, tok_v,
            mod_v, mf_v, mi_v, wt_v, wp_v, r_v, fa_v, fc_v, x1_v, a_v, acc_v, o_v, st_v,
            sem):
    slots = itertools.count()

    def copy(src, dst):
        return pltpu.make_async_copy(src, dst, sem.at[next(slots)])

    def cols(ref, lo, n):
        return ref.at[:, pl.ds(lo, n)]

    def copy_cols(src, dst, lo, n):
        return copy(cols(src, lo, n), cols(dst, lo, n))

    cp_tok, cp_c = copy(tok_hbm, tok_v), copy(c_hbm, c_v)
    cp_mod = [copy_cols(wm_hbm, wm_v, 128 * lo, 128 * (hi - lo)) for lo, hi in MOD_PARTS]
    cp_chm = [copy(chm_hbm.at[pl.ds(5 * i, 5)], chm_v.at[pl.ds(5 * i, 5)]) for i in range(2)]
    cp_w = [copy(wr_hbm, wr_v), copy(wi_hbm, wi_v)]
    cp_b1, cp_b2 = copy(b1_hbm, b1_v), copy(b2_hbm, b2_v)

    def batch(pairs):
        slot = next(slots)
        return [pltpu.make_async_copy(src, dst, sem.at[slot]) for src, dst in pairs]

    cp_mlp = [batch([(cols(w1_hbm, 128 * t, 128), w1_v.at[t])
                     for t in range(lo // 128, (lo + n) // 128)]
                    + [(w2_hbm.at[pl.ds(lo, n), pl.ds(128 * t, 128)], w2_v.at[t, pl.ds(lo, n)])
                       for t in range(NT)]) for lo, n in zip(STARTS, CHUNKS)]
    sem_o, sem_x = next(slots), next(slots)

    def cp_x(i):
        lo = i * 256 if isinstance(i, int) else pl.multiple_of(i * 256, 256)
        return pltpu.make_async_copy(cols(x_hbm, lo, 256), cols(x_v, lo, 256), sem.at[sem_x + i])

    for c in (cp_tok, cp_c, cp_x(0), cp_x(1), cp_mod[0], *map(cp_x, range(2, NT // 2)), cp_chm[0],
              *cp_w, cp_chm[1], cp_mod[1], cp_b1, cp_b2, *cp_mlp[0]):
        c.start()

    def lanes(t):
        if isinstance(t, int):
            return slice(128 * t, 128 * (t + 1))
        return pl.ds(pl.multiple_of(t * 128, 128), 128)

    def blk(i):
        return slice(8 * i, 8 * i + 8)

    with jax.named_scope("gen"):
        cp_tok.wait()
        rows = [(tok_v[blk(0), :], tok_v[blk(1), :])]
        for _ in range(15):
            rows.append(_cmul(rows[-1], (tok_v[blk(2), :], tok_v[blk(3), :])))
        dft = tuple(jnp.concatenate([r[i] for r in rows], axis=0) for i in range(2))
        along = tuple(jnp.concatenate([tok_v[blk(i), :]] * 16, axis=0) for i in (4, 5))
        down = tuple(a.T for a in along)

        def gen(k, carry):
            for ref, m in zip((mf_v, mi_v), carry):
                ref[k, 0], ref[k, 1] = m[0].astype(bf16), m[1].astype(bf16)
            return _cmul(carry[0], down), _cmul(carry[1], along)

        lax.fori_loop(0, NT, gen, (dft, dft))

    cp_c.wait()
    cf = c_v[...].astype(f32)
    sc = jnp.broadcast_to(cf * jax.nn.sigmoid(cf), (16, D)).astype(bf16)

    def store_mod(j):
        row = _dot(sc, wm_v[:, lanes(j)])[0:8, :]
        n = 128 * j + lax.broadcasted_iota(jnp.int32, row.shape, 1)
        scale = jnp.logical_or(jnp.logical_and(n >= D, n < 2 * D),
                               jnp.logical_and(n >= 4 * D, n < 5 * D))
        row = jnp.where(scale, row + 1.0, row)
        row = jnp.where(jnp.logical_and(n >= 2 * D, n < 3 * D), row * (2.0 / (S * D)), row)
        mod_v[lanes(j), :] = jnp.concatenate([row] * 16, axis=0).T

    def mod(i, b=None):
        return mod_v[i * D:(i + 1) * D, :] if b is None else mod_v[blk(i * D // 8 + b), :]

    def first_mod():
        cp_mod[0].wait()
        for j in range(*MOD_PARTS[0]):
            store_mod(j)

    def stage(pair, slot, values, finish=lambda m: m):
        means = [_RowMean() for _ in pair]
        for vs in zip(*map(values, pair)):
            for m, v in zip(means, vs):
                m.add(v)
            yield
        for t, m in zip(pair, means):
            st_v[slot, t] = jnp.broadcast_to(finish(m.mean()), (8, 128))

    def in_turn(gens):
        for g, _ in gens:
            for _ in g:
                pass

    def in_step(gens):
        n = D // 8
        for q in range(n):
            for g, cuts in gens:
                for _ in range(cuts * q // n, cuts * (q + 1) // n):
                    next(g)
        in_turn(gens)

    def skewed(stages, emit, n, after_fill=lambda: None):
        depth = len(stages) - 1

        def step(oldest, lo, hi):
            emit([(fn(oldest + (depth - lag)), cuts)
                  for lag, cuts, fn in stages if lo <= lag <= hi])

        for i in range(depth):
            step(i - depth, 0, i)
        after_fill()
        lax.fori_loop(0, n - depth, lambda i, _: step(i, 0, depth), None)
        for i in range(n, n + depth):
            step(i - depth, i - n + 1, depth)

    def inv_std(var):
        return lax.rsqrt(var + EPS)

    def squares(src, slot, dst=None):
        def values(t):
            mean = st_v[slot, t]
            for b in range(D // 8):
                c = src[t, blk(b), :] - mean
                if dst is not None:
                    dst[t, blk(b), :] = c
                yield c * c
        return values

    def adjacent(i):
        return 2 * i, 2 * i + 1

    def tokens(t):
        for i in range(D // 16):
            x = x_v[16 * i:16 * i + 16, lanes(t)].astype(f32)
            for b, half in enumerate((x[:8], x[8:]), 2 * i):
                x1_v[t, blk(b), :] = half
                yield half

    def load_tokens(i):
        cp_x(i).wait()
        return stage(adjacent(i), 0, tokens)

    def fwd_butterflies(i):
        for t in adjacent(i):
            rstd = st_v[1, t]
            for p in range(8):
                x0, uv = _radix9([fc_v[t, blk(b), :] * rstd * mod(1, b) + mod(0, b)
                                  for b in range(p, D // 8, 8)])
                for g in range(4):
                    r_v[t, 128 * g + 16 * p:128 * g + 16 * p + 16, :] = _pair(*uv[g])
                if p % 2:
                    r_v[t, 504 + 8 * p:520 + 8 * p, :] = _pair(prev, x0)
                prev = x0
                yield

    with jax.named_scope("A"):
        skewed([(1, D // 8, lambda i: stage(adjacent(i), 1, squares(x1_v, 0, fc_v), inv_std)),
                (0, D // 8, load_tokens), (2, 16, fwd_butterflies)],
               in_step, NT // 2, first_mod)

    def filt_a(t):
        a = pltpu.bitcast(wr_v[0:DF - 1, lanes(t)], f32)
        b = pltpu.bitcast(wi_v[0:DF - 1, lanes(t)], f32)
        nr = wr_v[DF - 1:DF, lanes(t)].astype(f32)
        ni = wi_v[DF - 1:DF, lanes(t)].astype(f32)
        r = lax.broadcasted_iota(jnp.int32, (8, 128), 0)
        nyq = jnp.where(r == 0, nr, jnp.where(r == 1, ni, 0.0))
        rest = jnp.concatenate([a[128:], b[128:], nyq, jnp.zeros((88, 128), f32)], axis=0)
        for c, tile in enumerate((a[:128].T, b[:128].T, rest.T)):
            for j in range(8):
                lo = (NT + 1) * (8 * t + j)
                wt_v[c, lo:lo + NT, :] = tile[NT * j:NT * (j + 1)]

    def filt_b(k):
        wp_v[k, 0:128, :] = wt_v[0, pl.ds(k, 128, stride=NT + 1), :].T
        wp_v[k, 144:272, :] = wt_v[1, pl.ds(k, 128, stride=NT + 1), :].T
        rest = wt_v[2, pl.ds(k, 128, stride=NT + 1), :].T
        wp_v[k, 128:144, :] = rest[0:16]
        wp_v[k, 272:296, :] = rest[16:40]

    def filt(k, rb, base, nyq_row):
        if rb == NRB - 1:
            return jnp.broadcast_to(wp_v[k, nyq_row:nyq_row + 1, :], (8, 128))
        k0 = _row_runs()[rb // 2]
        w = pltpu.bitcast(wp_v[k, pl.ds(base + k0 // 2 + 72 * (rb % 2), 8, stride=9), :], u32)
        w = (w & np.uint32(0xFFFF0000)) if k0 % 2 else (w << 16)
        return pltpu.bitcast(w, f32)

    groups = [range(8 * g, min(8 * g + 8, NRB)) for g in range(5)]
    rounds = [(q, odd) for q in range(4) for odd in (0, 1)]

    def harmonics(q, odd):
        return q + 4 * odd, q + 4 * odd + 8

    def get(ref, i, rb):
        return ref[i, blk(2 * rb), :], ref[i, blk(2 * rb + 1), :]

    def put(ref, i, rb, z):
        ref[i, blk(2 * rb), :], ref[i, blk(2 * rb + 1), :] = z

    def token_dft(z, m_ref, k, sign):
        lhs = jnp.concatenate([v for pair in z for v in pair], axis=0).astype(bf16)
        p, q = _dot(lhs, m_ref[k, 0]), _dot(lhs, m_ref[k, 1])
        out = []
        for rb in range(NRB):
            re, im = blk(2 * rb), blk(2 * rb + 1)
            out.append((p[re] - q[im], q[re] + p[im]) if sign < 0
                       else (p[re] + q[im], p[im] - q[re]))
        return out

    def fwd_channel(g, t0):
        tiles = range(t0, NT, 4)
        if g < 4:
            outs = [_dot(_halves(chm_v[g]), r_v[t, lanes(g), :]) for t in tiles]
        else:
            pad = jnp.zeros((64, 128), bf16)
            outs = [_dot(_halves(chm_v[4, 0:40, :]),
                         jnp.concatenate([r_v[t, 512:576, :], pad], axis=0)) for t in tiles]
        for i, rb in enumerate(groups[g]):
            y = _radix4([(o[blk(2 * i)], o[blk(2 * i + 1)]) for o in outs], -1)
            for q in range(4):
                put(fa_v, 4 * q + t0, rb, _twiddle16(y[q], t0 * q, -1))

    def fwd_token(q, odd):
        z = []
        for rb in range(NRB):
            a, b, c, d = (get(fa_v, 4 * q + t0, rb) for t0 in range(4))
            if odd:
                z.append(_cross(_csub(a, c), _csub(b, d))[::-1])
            else:
                u, v = _cadd(a, c), _cadd(b, d)
                z.append((_cadd(u, v), _csub(u, v)))
        for k, zk in zip(harmonics(q, odd), zip(*z)):
            for rb, y in enumerate(token_dft(zk, mf_v, k, -1)):
                put(fc_v, k, rb, y)

    def inv_token(q, odd):
        outs = []
        for k in harmonics(q, odd):
            z = [_cmul(get(fc_v, k, rb), (filt(k, rb, 0, 288), filt(k, rb, 144, 289)))
                 for rb in range(NRB)]
            outs.append(token_dft(z, mi_v, k, +1))
        for rb, (a, c) in enumerate(zip(*outs)):
            u, v = _cadd(a, c), _csub(a, c)
            if odd:
                p, m = get(fa_v, q, rb), get(fa_v, 4 + q, rb)
                y1, y3 = _cross(m, v)
                for t0, y in enumerate((_cadd(p, u), y1, _csub(p, u), y3)):
                    put(fa_v, 4 * t0 + q, rb, _twiddle16(y, t0 * q, +1))
            else:
                put(fa_v, q, rb, u)
                put(fa_v, 4 + q, rb, v)

    def inv_channel(g, t0):
        z = [_radix4([get(fa_v, 4 * t0 + q, rb) for q in range(4)], +1) for rb in groups[g]]
        for t, zt in zip(range(t0, NT, 4), zip(*z)):
            parts = [v for pair in zt for v in pair]
            if g < 4:
                fc_v[t, lanes(g), :] = _dot(_halves(chm_v[5 + g]),
                                            jnp.concatenate(parts, axis=0).astype(bf16))
            else:
                parts.append(jnp.zeros((48, 128), f32))
                fc_v[t, 512:576, :] = _dot(_halves(chm_v[9, 0:32, :]),
                                           jnp.concatenate(parts, axis=0).astype(bf16))

    def start(batch):
        for c in batch:
            c.start()

    with jax.named_scope("F"):
        start(cp_mlp[1])
        cp_chm[0].wait()
        for g in range(5):
            for t0 in range(4):
                fwd_channel(g, t0)
        for i, r in enumerate(rounds):
            if i == 2:
                for c in cp_w:
                    c.wait()
            fwd_token(*r)
            if 2 <= i < 6:
                for t in range(4 * i - 8, 4 * i - 4):
                    filt_a(t)
            elif i >= 6:
                for k in harmonics(*rounds[2 * i - 12]) + harmonics(*rounds[2 * i - 11]):
                    filt_b(k)
    with jax.named_scope("I"):
        for i, r in enumerate(rounds):
            if i < 4:
                for k in harmonics(*rounds[i + 4]):
                    filt_b(k)
            inv_token(*r)
        cp_chm[1].wait()
        cp_mod[1].wait()
        lo, hi = MOD_PARTS[1]
        for i in range(20):
            inv_channel(*divmod(i, 4))
            if lo + i < hi:
                store_mod(lo + i)

    def opposite(j):
        return j, j + NT // 2

    def residual(t):
        for p in range(8):
            uv = [(fc_v[t, blk(16 * g + 2 * p), :], fc_v[t, blk(16 * g + 2 * p + 1), :])
                  for g in range(4)]
            for a, y in enumerate(_radix9_t(fc_v[t, blk(64 + p), :], uv)):
                b = 8 * a + p
                x1 = x1_v[t, blk(b), :] + mod(2, b) * y
                x1_v[t, blk(b), :] = x1
                yield x1

    def modulated(t):
        rstd = st_v[1, t]
        for b in range(D // 8):
            h = fa_v[t, blk(b), :] * rstd * mod(4, b) + mod(3, b)
            fc_v[t, blk(b), :] = h
            yield h

    def mlp_operands(j, _):
        stats = [(j + 4 * c, st_v[2, j + 4 * c], st_v[3, j + 4 * c]) for c in range(4)]
        for r0 in range(0, HB, 16):
            h = {(r, c): jnp.concatenate([(fc_v[t, q:q + 8, :] - mean) * rstd
                                          for q in (HB * r + r0, HB * r + r0 + 8)], axis=0)
                 for r in range(4) for c, (t, mean, rstd) in enumerate(stats)}
            for i, a in enumerate(_operands(_LEFT, lambda _, r, c: h[r, c])):
                a_v[i, j, r0:r0 + 16, :] = a

    with jax.named_scope("C"):
        skewed([(1, D // 8, lambda j: stage(opposite(j), 1, squares(x1_v, 0, fa_v), inv_std)),
                (0, D // 8, lambda j: stage(opposite(j), 0, residual))], in_turn, NT // 2)
        skewed([(1, D // 8, lambda j: stage(opposite(j), 3, squares(fc_v, 2), inv_std)),
                (0, D // 8, lambda j: stage(opposite(j), 2, modulated))], in_turn, NT // 2)
        lax.fori_loop(0, 4, mlp_operands, None)

    zero = pl.program_id(0)
    a_words = a_v.bitcast(u32)

    def weights(ref, top, height, left, stride, width, order=range(7)):
        def block(i, r, c):
            rows = pl.ds(pl.multiple_of((top + r * height) // 2 + 8 * i * zero, 8), height // 2)
            first = (left + c * stride) // 128
            words = [ref.bitcast(u32)[t, rows, :] for t in range(first, first + width // 128)]
            return _halves(jnp.concatenate(words, axis=1)).astype(f32)
        return _operands(_RIGHT, block, order)

    def hidden(j):
        lo, n = STARTS[j], CHUNKS[j] // 4
        for c in cp_mlp[j]:
            c.wait()
        for later in cp_mlp[j + 2:j + 3]:
            start(later)
        bias = [jnp.concatenate([b1[t:t + 1, :] for t in range((lo + c * n) // 128,
                                                               (lo + c * n + n) // 128)], axis=1)
                for c in range(4)]
        return {(r, c): _gelu(x + bias[c]) for (r, c), x in _blocks(
            _dot(_halves(jnp.concatenate([a_words[i, t] for t in range(4)], axis=1)), w)
            for i, w in enumerate(weights(w1_v, 0, SB, lo, n, n)))}

    late = range(7)

    def products(j):
        g = hidden(j)
        for a, w in zip(_operands(_LEFT, lambda _, r, c: g[r, c], late),
                        weights(w2_v, STARTS[j], CHUNKS[j] // 4, 0, SB, SB, late)):
            yield _dot(a, w)

    with jax.named_scope("MLP"):
        for c in (cp_b1, cp_b2):
            c.wait()
        b1, b2 = b1_v[...].astype(f32), b2_v[...].astype(f32)
        last = len(CHUNKS) - 1
        for j in range(last):
            for i, m in enumerate(products(j)):
                acc_v[i] = acc_v[i] + m if j else m

        def finish(r, c, y):
            rows = slice(HB * r, HB * (r + 1))
            for j in range(4):
                t = 4 * c + j
                yt = y[:, lanes(j)] + b2[t:t + 1, :]
                o_v[t, rows, :] = (x1_v[t, rows, :] + mod_v[5 * D + HB * r:5 * D + HB * (r + 1), :]
                                   * yt).astype(bf16)
                cp_o.append(pltpu.make_async_copy(
                    o_v.at[t, rows], o_hbm.at[rows, lanes(t)], sem.at[sem_o]))
                cp_o[-1].start()

        cp_o = []
        for (r, c), y in _blocks((acc_v[i] + m for i, m in enumerate(products(last))), late):
            finish(r, c, y)
        for c in cp_o:
            c.wait()


@jax.jit
def pallas_adaLN_cond__spectral_gfnet__mixer_token_mlp__prompt_kernel(
    A_x: jax.Array,
    A_w_r: jax.Array,
    A_w_i: jax.Array,
    B_x: jax.Array,
    B_w1: jax.Array,
    B_b1: jax.Array,
    B_w2: jax.Array,
    B_b2: jax.Array,
    c: jax.Array,
    w_mod: jax.Array,
):
    del B_x
    vmem = pltpu.VMEM
    scratch = [
        vmem((D, S), bf16), vmem((DF, S), bf16), vmem((DF, S), bf16),
        vmem((F // 128, S, 128), bf16), vmem((F // 128, 128), bf16),
        vmem((NT, F, 128), bf16), vmem((S // 128, 128), bf16),
        vmem((1, D), bf16), vmem((D, 6 * D), bf16),
        vmem(_CH_MATS.shape, u32), vmem(_TOK_TAB.shape, f32),
        vmem((6 * D, 128), f32),
        vmem((NT, 2, 128, 128), bf16),
        vmem((NT, 2, 128, 128), bf16),
        vmem((3, S + 128, 128), f32),
        vmem((NT, 296, 128), f32),
        vmem((NT, D, 128), bf16),
        vmem((NT, NRB * 16, 128), f32),
        vmem((NT, NRB * 16, 128), f32),
        vmem((NT, D, 128), f32),
        vmem((49, 4, HB, 128), bf16),
        vmem((49, HB, SB), f32),
        vmem((NT, D, 128), bf16),
        vmem((4, NT, 8, 128), f32),
        pltpu.SemaphoreType.DMA((64,)),
    ]
    out = pl.pallas_call(
        _kernel,
        grid=(1,),
        in_specs=[pl.BlockSpec(memory_space=pl.ANY)] * 11,
        out_specs=pl.BlockSpec(memory_space=pl.ANY),
        out_shape=jax.ShapeDtypeStruct((D, S), bf16),
        scratch_shapes=scratch,
        compiler_params=pltpu.CompilerParams(vmem_limit_bytes=124 * 1024 * 1024),
    )(A_x[0].T, A_w_r.T, A_w_i.T, B_w1, B_b1.reshape(F // 128, 128), B_w2,
      B_b2.reshape(S // 128, 128), c, w_mod, _CH_MATS, _TOK_TAB)
    return out.T[None]
```

```python
import itertools

import jax
import jax.numpy as jnp
import numpy as np
from jax import lax
from jax.experimental import pallas as pl
from jax.experimental.pallas import tpu as pltpu

D, S, F = 576, 2048, 4608
DF = D // 2 + 1
NT = S // 128
NRB = 37
EPS = 1e-5
HB, SB = D // 4, S // 4
CHUNKS = (512, 1024, 1024, 2048)
STARTS = tuple(sum(CHUNKS[:j]) for j in range(len(CHUNKS)))
MOD_PARTS = ((0, 9), (9, 27))

f32, bf16, u32 = jnp.float32, jnp.bfloat16, jnp.uint32

_Q = np.sqrt(3.0) / 2
_C1, _C2, _C4 = (float(np.cos(2 * np.pi * k / 9)) for k in (1, 2, 4))
_S1, _S2, _S4 = (float(np.sin(2 * np.pi * k / 9) / _Q) for k in (1, 2, 4))


def _row_runs():
    runs = []
    for g in (1, 2, 3, 4):
        for r in (g, 9 - g):
            runs += [r, r + 9]
    return runs + [0, 9]


def _pack_rows(m):
    b = m.astype(np.float32).astype(jnp.bfloat16).view(np.uint16).astype(np.uint32)
    return b[..., 0::2, :] | (b[..., 1::2, :] << np.uint32(16))


def _channel_mats():
    kd_all = [k0 + 18 * j for k0 in _row_runs() for j in range(16)] + [D // 2] + [-1] * 7
    kd_all = np.array(kd_all)
    b = np.arange(64)
    mats = np.zeros((10, 128, 128))
    for g in (1, 2, 3, 4):
        kd = kd_all[64 * (g - 1):64 * g]
        sg = np.where(kd % 9 == g, -1.0, 1.0).reshape(8, 8, 1, 1)
        th = (2 * np.pi / D) * ((kd[:, None] * b[None, :]) % D)
        c, s = np.cos(th).reshape(8, 8, 8, 8), np.sin(th).reshape(8, 8, 8, 8)
        m = np.zeros((8, 2, 8, 8, 2, 8))
        m[:, 0, :, :, 0, :] = c
        m[:, 0, :, :, 1, :] = sg * _Q * s
        m[:, 1, :, :, 0, :] = -s
        m[:, 1, :, :, 1, :] = sg * _Q * c
        mats[g - 1] = m.reshape(128, 128)
        mats[5 + g - 1] = m.reshape(128, 128).T
    kd = kd_all[256:]
    valid = (kd >= 0)[:, None]
    th = (2 * np.pi / D) * ((kd[:, None] * b[None, :]) % D)
    m = np.zeros((5, 2, 8, 64))
    m[:, 0] = (np.cos(th) * valid).reshape(5, 8, 64)
    m[:, 1] = (-np.sin(th) * valid * (kd != D // 2)[:, None]).reshape(5, 8, 64)
    half = np.where((kd == 0) | (kd == D // 2), 0.5, 1.0).reshape(5, 1, 8, 1)
    mats[4, :80, :64] = m.reshape(80, 64)
    mats[9, :64, :80] = (m * half).reshape(80, 64).T
    return _pack_rows(mats)


def _token_tables():
    l = np.arange(128)
    ones = np.ones((8, 1))
    angles = [(2 * np.pi / 128) * ((l[:8, None] * l[None, :]) % 128),
              (2 * np.pi / 128) * ((8 * l) % 128) * ones, (2 * np.pi / S) * l * ones]
    return np.concatenate([p for a in angles for p in (np.cos(a), -np.sin(a))]).astype(np.float32)


_CH_MATS = _channel_mats()
_TOK_TAB = _token_tables()


def _dot(a, b):
    return jnp.dot(a, b, preferred_element_type=f32)


def _radix9(x):
    s1, s2, s3, s4 = x[1] + x[8], x[2] + x[7], x[3] + x[6], x[4] + x[5]
    d1, d2, d3, d4 = x[1] - x[8], x[2] - x[7], x[3] - x[6], x[4] - x[5]
    p = x[0] - 0.5 * s3
    a, b = s1 - s4, s2 - s4
    r1 = _C1 * a + _C2 * b
    r2 = _C2 * a + _C4 * b
    e, g = d1 + d2, d2 + d4
    i1 = _S1 * e + _S4 * g
    i2 = _S2 * e - _S1 * g
    t, u = s1 + s2 + s4, x[0] + s3
    return u + t, [(p + r1, i1 + d3), (p + r2, i2 - d3),
                   (u - 0.5 * t, d1 - d2 + d4), ((p - r1) - r2, (i2 - i1) + d3)]


def _radix9_t(x0, uv):
    (u1, v1), (u2, v2), (u3, v3), (u4, v4) = uv
    u, t = x0 + u3, x0 - 0.5 * u3
    p, r1, r2 = u1 + u2 + u4, u1 - u4, u2 - u4
    a = _C1 * r1 + _C2 * r2
    b = _C2 * r1 + _C4 * r2
    s1, s2, s3, s4 = t + a, t + b, u - 0.5 * p, (t - a) - b
    i1, i2, d3 = v1 - v4, v2 + v4, v1 - v2 + v4
    e = _S1 * i1 + _S2 * i2
    g = _S4 * i1 - _S1 * i2
    d1, d2, d4 = e + v3, (e + g) - v3, g + v3
    return [u + p, s1 + d1, s2 + d2, s3 + d3, s4 + d4, s4 - d4, s3 - d3, s2 - d2, s1 - d1]


def _cadd(a, b):
    return a[0] + b[0], a[1] + b[1]


def _csub(a, b):
    return a[0] - b[0], a[1] - b[1]


def _cmul(a, b):
    return a[0] * b[0] - a[1] * b[1], a[0] * b[1] + a[1] * b[0]


def _cross(a, b):
    return (a[0] - b[1], a[1] + b[0]), (a[0] + b[1], a[1] - b[0])


def _radix4(x, sign):
    a, b, c, d = x
    u, v = _cadd(a, c), _cadd(b, d)
    k1, k3 = _cross(_csub(a, c), _csub(b, d))[::sign]
    return [_cadd(u, v), k1, _csub(u, v), k3]


def _twiddle16(z, e, sign):
    re, im = z
    if e == 0:
        return z
    c, s = float(np.cos(2 * np.pi * e / 16)), float(sign * np.sin(2 * np.pi * e / 16))
    if e == 4:
        return (-im, re) if sign > 0 else (im, -re)
    if e % 2 == 0:
        if c * s > 0:
            return c * (re - im), c * (re + im)
        return c * (re + im), c * (im - re)
    return c * re - s * im, s * re + c * im


def _halves(w):
    return pltpu.bitcast(w, bf16)


def _pair(a, b):
    return jnp.concatenate([a, b], axis=0).astype(bf16)


class _RowMean:
    def __init__(self, lanes=2):
        self.acc, self.n = [None] * lanes, 0

    def add(self, v):
        i = self.n % len(self.acc)
        self.acc[i] = v if self.acc[i] is None else self.acc[i] + v
        self.n += 1

    def mean(self):
        acc = self.acc
        while len(acc) > 1:
            acc = [acc[i] + acc[i + 1] for i in range(0, len(acc), 2)]
        return jnp.sum(acc[0], axis=0, keepdims=True) * (1.0 / D)


def _gelu(x):
    inner = x * (0.7978845608028654 + (0.7978845608028654 * 0.044715) * (x * x))
    hx = 0.5 * x
    return hx + hx * jnp.tanh(inner)


_LEFT = (((0, 0), 1, (1, 1)), ((1, 0), 1, (1, 1)), ((0, 0), 0, None), ((1, 1), 0, None),
         ((0, 0), 1, (0, 1)), ((1, 0), -1, (0, 0)), ((0, 1), -1, (1, 1)))
_RIGHT = (((0, 0), 1, (1, 1)), ((0, 0), 0, None), ((0, 1), -1, (1, 1)), ((1, 0), -1, (0, 0)),
          ((1, 1), 0, None), ((0, 0), 1, (0, 1)), ((1, 0), 1, (1, 1)))


def _signed_sum(term, quad):
    a, sign, b = term
    if sign == 0:
        return quad(*a)
    return quad(*a) + quad(*b) if sign > 0 else quad(*a) - quad(*b)


def _operands(table, block, order=range(7)):
    for i in order:
        outer = table[i]
        if outer[1]:
            sums = {(u, v): _signed_sum(outer, lambda r, c: block(i, 2 * r + u, 2 * c + v))
                    for u in range(2) for v in range(2)}
        for j, inner in enumerate(table):
            def quad(u, v):
                if outer[1]:
                    return sums[u, v]
                return block(7 * i + j, 2 * outer[0][0] + u, 2 * outer[0][1] + v)
            yield _signed_sum(inner, quad).astype(bf16)


_RESULT = {(0, 0): {0: 1, 3: 1, 4: -1, 6: 1}, (0, 1): {2: 1, 4: 1},
           (1, 0): {1: 1, 3: 1}, (1, 1): {0: 1, 1: -1, 2: 1, 5: 1}}


def _completed(i, have):
    for quadrant, terms in _RESULT.items():
        if i in terms and all(j in have for j in terms):
            first, *rest = terms
            x = have[first]
            for j in rest:
                x = x + have[j] if terms[j] > 0 else x - have[j]
            yield quadrant, x


def _blocks(products, order=range(7)):
    outer = {quadrant: {} for quadrant in _RESULT}
    for i in order:
        inner = {}
        for j in range(7):
            inner[j] = next(products)
            for (u, v), x in _completed(j, inner):
                outer[u, v][i] = x
                for (r, c), y in _completed(i, outer[u, v]):
                    yield (2 * r + u, 2 * c + v), y


def _kernel(x_hbm, wr_hbm, wi_hbm, w1_hbm, b1_hbm, w2_hbm, b2_hbm, c_hbm, wm_hbm, chm_hbm, tok_hbm,
            o_hbm,
            x_v, wr_v, wi_v, w1_v, b1_v, w2_v, b2_v, c_v, wm_v, chm_v, tok_v,
            mod_v, mf_v, mi_v, wt_v, wp_v, r_v, fa_v, fc_v, x1_v, a_v, acc_v, o_v, st_v,
            sem):
    slots = itertools.count()

    def copy(src, dst):
        return pltpu.make_async_copy(src, dst, sem.at[next(slots)])

    def cols(ref, lo, n):
        return ref.at[:, pl.ds(lo, n)]

    def copy_cols(src, dst, lo, n):
        return copy(cols(src, lo, n), cols(dst, lo, n))

    cp_tok, cp_c = copy(tok_hbm, tok_v), copy(c_hbm, c_v)
    cp_mod = [copy_cols(wm_hbm, wm_v, 128 * lo, 128 * (hi - lo)) for lo, hi in MOD_PARTS]
    cp_chm = [copy(chm_hbm.at[pl.ds(5 * i, 5)], chm_v.at[pl.ds(5 * i, 5)]) for i in range(2)]
    cp_w = [copy(wr_hbm, wr_v), copy(wi_hbm, wi_v)]
    cp_b1, cp_b2 = copy(b1_hbm, b1_v), copy(b2_hbm, b2_v)

    def batch(pairs):
        slot = next(slots)
        return [pltpu.make_async_copy(src, dst, sem.at[slot]) for src, dst in pairs]

    cp_mlp = [batch([(cols(w1_hbm, 128 * t, 128), w1_v.at[t])
                     for t in range(lo // 128, (lo + n) // 128)]
                    + [(w2_hbm.at[pl.ds(lo, n), pl.ds(128 * t, 128)], w2_v.at[t, pl.ds(lo, n)])
                       for t in range(NT)]) for lo, n in zip(STARTS, CHUNKS)]
    sem_o, sem_x = next(slots), next(slots)

    def cp_x(i):
        lo = i * 256 if isinstance(i, int) else pl.multiple_of(i * 256, 256)
        return pltpu.make_async_copy(cols(x_hbm, lo, 256), cols(x_v, lo, 256), sem.at[sem_x + i])

    for c in (cp_tok, cp_c, cp_x(0), cp_x(1), cp_mod[0], *map(cp_x, range(2, NT // 2)), cp_chm[0],
              *cp_w, cp_chm[1], cp_mod[1], cp_b1, cp_b2, *cp_mlp[0]):
        c.start()

    def lanes(t):
        if isinstance(t, int):
            return slice(128 * t, 128 * (t + 1))
        return pl.ds(pl.multiple_of(t * 128, 128), 128)

    def blk(i):
        return slice(8 * i, 8 * i + 8)

    with jax.named_scope("gen"):
        cp_tok.wait()
        rows = [(tok_v[blk(0), :], tok_v[blk(1), :])]
        for _ in range(15):
            rows.append(_cmul(rows[-1], (tok_v[blk(2), :], tok_v[blk(3), :])))
        dft = tuple(jnp.concatenate([r[i] for r in rows], axis=0) for i in range(2))
        along = tuple(jnp.concatenate([tok_v[blk(i), :]] * 16, axis=0) for i in (4, 5))
        down = tuple(a.T for a in along)

        def gen(k, carry):
            for ref, (re, im), order in zip((mf_v, mi_v), carry, ((1, 2), (2, 1))):
                for i, m in zip((0, *order), (re, re + im, re - im)):
                    ref[k, i] = m.astype(bf16)
            return _cmul(carry[0], down), _cmul(carry[1], along)

        lax.fori_loop(0, NT, gen, (dft, dft))

    cp_c.wait()
    cf = c_v[...].astype(f32)
    sc = jnp.broadcast_to(cf * jax.nn.sigmoid(cf), (16, D)).astype(bf16)

    def store_mod(j):
        row = _dot(sc, wm_v[:, lanes(j)])[0:8, :]
        n = 128 * j + lax.broadcasted_iota(jnp.int32, row.shape, 1)
        scale = jnp.logical_or(jnp.logical_and(n >= D, n < 2 * D),
                               jnp.logical_and(n >= 4 * D, n < 5 * D))
        row = jnp.where(scale, row + 1.0, row)
        row = jnp.where(jnp.logical_and(n >= 2 * D, n < 3 * D), row * (2.0 / (S * D)), row)
        mod_v[lanes(j), :] = jnp.concatenate([row] * 16, axis=0).T

    def mod(i, b=None):
        return mod_v[i * D:(i + 1) * D, :] if b is None else mod_v[blk(i * D // 8 + b), :]

    def first_mod():
        cp_mod[0].wait()
        for j in range(*MOD_PARTS[0]):
            store_mod(j)

    def stage(pair, slot, values, finish=lambda m: m):
        means = [_RowMean() for _ in pair]
        for vs in zip(*map(values, pair)):
            for m, v in zip(means, vs):
                m.add(v)
            yield
        for t, m in zip(pair, means):
            st_v[slot, t] = jnp.broadcast_to(finish(m.mean()), (8, 128))

    def in_turn(gens):
        for g, _ in gens:
            for _ in g:
                pass

    def in_step(gens):
        n = D // 8
        for q in range(n):
            for g, cuts in gens:
                for _ in range(cuts * q // n, cuts * (q + 1) // n):
                    next(g)
        in_turn(gens)

    def skewed(stages, emit, n, after_fill=lambda: None):
        depth = len(stages) - 1

        def step(oldest, lo, hi):
            emit([(fn(oldest + (depth - lag)), cuts)
                  for lag, cuts, fn in stages if lo <= lag <= hi])

        for i in range(depth):
            step(i - depth, 0, i)
        after_fill()
        lax.fori_loop(0, n - depth, lambda i, _: step(i, 0, depth), None)
        for i in range(n, n + depth):
            step(i - depth, i - n + 1, depth)

    def inv_std(var):
        return lax.rsqrt(var + EPS)

    def squares(src, slot, dst=None):
        def values(t):
            mean = st_v[slot, t]
            for b in range(D // 8):
                c = src[t, blk(b), :] - mean
                if dst is not None:
                    dst[t, blk(b), :] = c
                yield c * c
        return values

    def adjacent(i):
        return 2 * i, 2 * i + 1

    def tokens(t):
        for i in range(D // 16):
            x = x_v[16 * i:16 * i + 16, lanes(t)].astype(f32)
            for b, half in enumerate((x[:8], x[8:]), 2 * i):
                x1_v[t, blk(b), :] = half
                yield half

    def load_tokens(i):
        cp_x(i).wait()
        return stage(adjacent(i), 0, tokens)

    def fwd_butterflies(i):
        for t in adjacent(i):
            rstd = st_v[1, t]
            for p in range(8):
                x0, uv = _radix9([fc_v[t, blk(b), :] * rstd * mod(1, b) + mod(0, b)
                                  for b in range(p, D // 8, 8)])
                for g in range(4):
                    r_v[t, 128 * g + 16 * p:128 * g + 16 * p + 16, :] = _pair(*uv[g])
                if p % 2:
                    r_v[t, 504 + 8 * p:520 + 8 * p, :] = _pair(prev, x0)
                prev = x0
                yield

    with jax.named_scope("A"):
        skewed([(1, D // 8, lambda i: stage(adjacent(i), 1, squares(x1_v, 0, fc_v), inv_std)),
                (0, D // 8, load_tokens), (2, 16, fwd_butterflies)],
               in_step, NT // 2, first_mod)

    def filt_a(t):
        a = pltpu.bitcast(wr_v[0:DF - 1, lanes(t)], f32)
        b = pltpu.bitcast(wi_v[0:DF - 1, lanes(t)], f32)
        nr = wr_v[DF - 1:DF, lanes(t)].astype(f32)
        ni = wi_v[DF - 1:DF, lanes(t)].astype(f32)
        r = lax.broadcasted_iota(jnp.int32, (8, 128), 0)
        nyq = jnp.where(r == 0, nr, jnp.where(r == 1, ni, 0.0))
        rest = jnp.concatenate([a[128:], b[128:], nyq, jnp.zeros((88, 128), f32)], axis=0)
        for c, tile in enumerate((a[:128].T, b[:128].T, rest.T)):
            for j in range(8):
                lo = (NT + 1) * (8 * t + j)
                wt_v[c, lo:lo + NT, :] = tile[NT * j:NT * (j + 1)]

    def filt_b(k):
        wp_v[k, 0:128, :] = wt_v[0, pl.ds(k, 128, stride=NT + 1), :].T
        wp_v[k, 144:272, :] = wt_v[1, pl.ds(k, 128, stride=NT + 1), :].T
        rest = wt_v[2, pl.ds(k, 128, stride=NT + 1), :].T
        wp_v[k, 128:144, :] = rest[0:16]
        wp_v[k, 272:296, :] = rest[16:40]

    def filt(k, rb, base, nyq_row):
        if rb == NRB - 1:
            return jnp.broadcast_to(wp_v[k, nyq_row:nyq_row + 1, :], (8, 128))
        k0 = _row_runs()[rb // 2]
        w = pltpu.bitcast(wp_v[k, pl.ds(base + k0 // 2 + 72 * (rb % 2), 8, stride=9), :], u32)
        w = (w & np.uint32(0xFFFF0000)) if k0 % 2 else (w << 16)
        return pltpu.bitcast(w, f32)

    groups = [range(8 * g, min(8 * g + 8, NRB)) for g in range(5)]
    rounds = [(q, odd) for q in range(4) for odd in (0, 1)]

    def harmonics(q, odd):
        return q + 4 * odd, q + 4 * odd + 8

    def get(ref, i, rb):
        return ref[i, blk(2 * rb), :], ref[i, blk(2 * rb + 1), :]

    def put(ref, i, rb, z):
        ref[i, blk(2 * rb), :], ref[i, blk(2 * rb + 1), :] = z

    def token_dft(z, m_ref, k):
        def times(parts, i):
            lhs = jnp.concatenate([*parts, jnp.zeros((8, 128), f32)], axis=0).astype(bf16)
            return _dot(lhs, m_ref[k, i])
        s = times([re + im for re, im in z], 0)
        a, b = times([im for _, im in z], 1), times([re for re, _ in z], 2)
        return [(s[blk(rb)] - a[blk(rb)], s[blk(rb)] - b[blk(rb)]) for rb in range(NRB)]

    def fwd_channel(g, t0):
        tiles = range(t0, NT, 4)
        if g < 4:
            outs = [_dot(_halves(chm_v[g]), r_v[t, lanes(g), :]) for t in tiles]
        else:
            pad = jnp.zeros((64, 128), bf16)
            outs = [_dot(_halves(chm_v[4, 0:40, :]),
                         jnp.concatenate([r_v[t, 512:576, :], pad], axis=0)) for t in tiles]
        for i, rb in enumerate(groups[g]):
            y = _radix4([(o[blk(2 * i)], o[blk(2 * i + 1)]) for o in outs], -1)
            for q in range(4):
                put(fa_v, 4 * q + t0, rb, _twiddle16(y[q], t0 * q, -1))

    def fwd_token(q, odd):
        z = []
        for rb in range(NRB):
            a, b, c, d = (get(fa_v, 4 * q + t0, rb) for t0 in range(4))
            if odd:
                z.append(_cross(_csub(a, c), _csub(b, d))[::-1])
            else:
                u, v = _cadd(a, c), _cadd(b, d)
                z.append((_cadd(u, v), _csub(u, v)))
        for k, zk in zip(harmonics(q, odd), zip(*z)):
            for rb, y in enumerate(token_dft(zk, mf_v, k)):
                put(fc_v, k, rb, y)

    def inv_token(q, odd):
        outs = []
        for k in harmonics(q, odd):
            z = [_cmul(get(fc_v, k, rb), (filt(k, rb, 0, 288), filt(k, rb, 144, 289)))
                 for rb in range(NRB)]
            outs.append(token_dft(z, mi_v, k))
        for rb, (a, c) in enumerate(zip(*outs)):
            u, v = _cadd(a, c), _csub(a, c)
            if odd:
                p, m = get(fa_v, q, rb), get(fa_v, 4 + q, rb)
                y1, y3 = _cross(m, v)
                for t0, y in enumerate((_cadd(p, u), y1, _csub(p, u), y3)):
                    put(fa_v, 4 * t0 + q, rb, _twiddle16(y, t0 * q, +1))
            else:
                put(fa_v, q, rb, u)
                put(fa_v, 4 + q, rb, v)

    def inv_channel(g, t0):
        z = [_radix4([get(fa_v, 4 * t0 + q, rb) for q in range(4)], +1) for rb in groups[g]]
        for t, zt in zip(range(t0, NT, 4), zip(*z)):
            parts = [v for pair in zt for v in pair]
            if g < 4:
                fc_v[t, lanes(g), :] = _dot(_halves(chm_v[5 + g]),
                                            jnp.concatenate(parts, axis=0).astype(bf16))
            else:
                parts.append(jnp.zeros((48, 128), f32))
                fc_v[t, 512:576, :] = _dot(_halves(chm_v[9, 0:32, :]),
                                           jnp.concatenate(parts, axis=0).astype(bf16))

    def start(batch):
        for c in batch:
            c.start()

    with jax.named_scope("F"):
        start(cp_mlp[1])
        cp_chm[0].wait()
        for g in range(5):
            for t0 in range(4):
                fwd_channel(g, t0)
        for i, r in enumerate(rounds):
            if i == 2:
                for c in cp_w:
                    c.wait()
            fwd_token(*r)
            if 2 <= i < 6:
                for t in range(4 * i - 8, 4 * i - 4):
                    filt_a(t)
            elif i >= 6:
                for k in harmonics(*rounds[i - 6]):
                    filt_b(k)
    with jax.named_scope("I"):
        for i, r in enumerate(rounds):
            if i < 6:
                for k in harmonics(*rounds[i + 2]):
                    filt_b(k)
            inv_token(*r)
        cp_chm[1].wait()
        cp_mod[1].wait()
        lo, hi = MOD_PARTS[1]
        for i in range(20):
            inv_channel(*divmod(i, 4))
            if lo + i < hi:
                store_mod(lo + i)

    def opposite(j):
        return j, j + NT // 2

    def residual(t):
        for p in range(8):
            uv = [(fc_v[t, blk(16 * g + 2 * p), :], fc_v[t, blk(16 * g + 2 * p + 1), :])
                  for g in range(4)]
            for a, y in enumerate(_radix9_t(fc_v[t, blk(64 + p), :], uv)):
                b = 8 * a + p
                x1 = x1_v[t, blk(b), :] + mod(2, b) * y
                x1_v[t, blk(b), :] = x1
                yield x1

    def modulated(t):
        rstd = st_v[1, t]
        for b in range(D // 8):
            h = fa_v[t, blk(b), :] * rstd * mod(4, b) + mod(3, b)
            fc_v[t, blk(b), :] = h
            yield h

    def mlp_operands(j, _):
        stats = [(j + 4 * c, st_v[2, j + 4 * c], st_v[3, j + 4 * c]) for c in range(4)]
        for r0 in range(0, HB, 16):
            h = {(r, c): jnp.concatenate([(fc_v[t, q:q + 8, :] - mean) * rstd
                                          for q in (HB * r + r0, HB * r + r0 + 8)], axis=0)
                 for r in range(4) for c, (t, mean, rstd) in enumerate(stats)}
            for i, a in enumerate(_operands(_LEFT, lambda _, r, c: h[r, c])):
                a_v[i, j, r0:r0 + 16, :] = a

    with jax.named_scope("C"):
        skewed([(1, D // 8, lambda j: stage(opposite(j), 1, squares(x1_v, 0, fa_v), inv_std)),
                (0, D // 8, lambda j: stage(opposite(j), 0, residual))], in_turn, NT // 2)
        skewed([(1, D // 8, lambda j: stage(opposite(j), 3, squares(fc_v, 2), inv_std)),
                (0, D // 8, lambda j: stage(opposite(j), 2, modulated))], in_turn, NT // 2)
        lax.fori_loop(0, 4, mlp_operands, None)

    zero = pl.program_id(0)
    a_words = a_v.bitcast(u32)

    def weights(ref, top, height, left, stride, width, order=range(7)):
        def block(i, r, c):
            rows = pl.ds(pl.multiple_of((top + r * height) // 2 + 8 * i * zero, 8), height // 2)
            first = (left + c * stride) // 128
            words = [ref.bitcast(u32)[t, rows, :] for t in range(first, first + width // 128)]
            return _halves(jnp.concatenate(words, axis=1)).astype(f32)
        return _operands(_RIGHT, block, order)

    def hidden(j):
        lo, n = STARTS[j], CHUNKS[j] // 4
        for c in cp_mlp[j]:
            c.wait()
        for later in cp_mlp[j + 2:j + 3]:
            start(later)
        bias = [jnp.concatenate([b1[t:t + 1, :] for t in range((lo + c * n) // 128,
                                                               (lo + c * n + n) // 128)], axis=1)
                for c in range(4)]
        return {(r, c): _gelu(x + bias[c]) for (r, c), x in _blocks(
            _dot(_halves(jnp.concatenate([a_words[i, t] for t in range(4)], axis=1)), w)
            for i, w in enumerate(weights(w1_v, 0, SB, lo, n, n)))}

    late = range(7)

    def products(j):
        g = hidden(j)
        for a, w in zip(_operands(_LEFT, lambda _, r, c: g[r, c], late),
                        weights(w2_v, STARTS[j], CHUNKS[j] // 4, 0, SB, SB, late)):
            yield _dot(a, w)

    with jax.named_scope("MLP"):
        for c in (cp_b1, cp_b2):
            c.wait()
        b1, b2 = b1_v[...].astype(f32), b2_v[...].astype(f32)
        last = len(CHUNKS) - 1
        for j in range(last):
            for i, m in enumerate(products(j)):
                acc_v[i] = acc_v[i] + m if j else m

        def finish(r, c, y):
            rows = slice(HB * r, HB * (r + 1))
            for j in range(4):
                t = 4 * c + j
                yt = y[:, lanes(j)] + b2[t:t + 1, :]
                o_v[t, rows, :] = (x1_v[t, rows, :] + mod_v[5 * D + HB * r:5 * D + HB * (r + 1), :]
                                   * yt).astype(bf16)
                cp_o.append(pltpu.make_async_copy(
                    o_v.at[t, rows], o_hbm.at[rows, lanes(t)], sem.at[sem_o]))
                cp_o[-1].start()

        cp_o = []
        for (r, c), y in _blocks((acc_v[i] + m for i, m in enumerate(products(last))), late):
            finish(r, c, y)
        for c in cp_o:
            c.wait()


@jax.jit
def pallas_adaLN_cond__spectral_gfnet__mixer_token_mlp__prompt_kernel(
    A_x: jax.Array,
    A_w_r: jax.Array,
    A_w_i: jax.Array,
    B_x: jax.Array,
    B_w1: jax.Array,
    B_b1: jax.Array,
    B_w2: jax.Array,
    B_b2: jax.Array,
    c: jax.Array,
    w_mod: jax.Array,
):
    del B_x
    vmem = pltpu.VMEM
    scratch = [
        vmem((D, S), bf16), vmem((DF, S), bf16), vmem((DF, S), bf16),
        vmem((F // 128, S, 128), bf16), vmem((F // 128, 128), bf16),
        vmem((NT, F, 128), bf16), vmem((S // 128, 128), bf16),
        vmem((1, D), bf16), vmem((D, 6 * D), bf16),
        vmem(_CH_MATS.shape, u32), vmem(_TOK_TAB.shape, f32),
        vmem((6 * D, 128), f32),
        vmem((NT, 3, 128, 128), bf16),
        vmem((NT, 3, 128, 128), bf16),
        vmem((3, S + 128, 128), f32),
        vmem((NT, 296, 128), f32),
        vmem((NT, D, 128), bf16),
        vmem((NT, NRB * 16, 128), f32),
        vmem((NT, NRB * 16, 128), f32),
        vmem((NT, D, 128), f32),
        vmem((49, 4, HB, 128), bf16),
        vmem((49, HB, SB), f32),
        vmem((NT, D, 128), bf16),
        vmem((4, NT, 8, 128), f32),
        pltpu.SemaphoreType.DMA((64,)),
    ]
    out = pl.pallas_call(
        _kernel,
        grid=(1,),
        in_specs=[pl.BlockSpec(memory_space=pl.ANY)] * 11,
        out_specs=pl.BlockSpec(memory_space=pl.ANY),
        out_shape=jax.ShapeDtypeStruct((D, S), bf16),
        scratch_shapes=scratch,
        compiler_params=pltpu.CompilerParams(vmem_limit_bytes=124 * 1024 * 1024),
    )(A_x[0].T, A_w_r.T, A_w_i.T, B_w1, B_b1.reshape(F // 128, 128), B_w2,
      B_b2.reshape(S // 128, 128), c, w_mod, _CH_MATS, _TOK_TAB)
    return out.T[None]
```

```python
import itertools

import jax
import jax.numpy as jnp
import numpy as np
from jax import lax
from jax.experimental import pallas as pl
from jax.experimental.pallas import tpu as pltpu

D, S, F = 576, 2048, 4608
DF = D // 2 + 1
NT = S // 128
NRB = 37
EPS = 1e-5
HB, SB = D // 4, S // 4
CHUNKS = (1024, 1536, 2048)
STARTS = tuple(sum(CHUNKS[:j]) for j in range(len(CHUNKS)))
MOD_PARTS = ((0, 9), (9, 27))

f32, bf16, u32 = jnp.float32, jnp.bfloat16, jnp.uint32

_Q = np.sqrt(3.0) / 2
_C1, _C2, _C4 = (float(np.cos(2 * np.pi * k / 9)) for k in (1, 2, 4))
_S1, _S2, _S4 = (float(np.sin(2 * np.pi * k / 9) / _Q) for k in (1, 2, 4))


def _row_runs():
    runs = []
    for g in (1, 2, 3, 4):
        for r in (g, 9 - g):
            runs += [r, r + 9]
    return runs + [0, 9]


def _pack_rows(m):
    b = m.astype(np.float32).astype(jnp.bfloat16).view(np.uint16).astype(np.uint32)
    return b[..., 0::2, :] | (b[..., 1::2, :] << np.uint32(16))


def _channel_mats():
    kd_all = [k0 + 18 * j for k0 in _row_runs() for j in range(16)] + [D // 2] + [-1] * 7
    kd_all = np.array(kd_all)
    b = np.arange(64)
    mats = np.zeros((10, 128, 128))
    for g in (1, 2, 3, 4):
        kd = kd_all[64 * (g - 1):64 * g]
        sg = np.where(kd % 9 == g, -1.0, 1.0).reshape(8, 8, 1, 1)
        th = (2 * np.pi / D) * ((kd[:, None] * b[None, :]) % D)
        c, s = np.cos(th).reshape(8, 8, 8, 8), np.sin(th).reshape(8, 8, 8, 8)
        m = np.zeros((8, 2, 8, 8, 2, 8))
        m[:, 0, :, :, 0, :] = c
        m[:, 0, :, :, 1, :] = sg * _Q * s
        m[:, 1, :, :, 0, :] = -s
        m[:, 1, :, :, 1, :] = sg * _Q * c
        mats[g - 1] = m.reshape(128, 128)
        mats[5 + g - 1] = m.reshape(128, 128).T
    kd = kd_all[256:]
    valid = (kd >= 0)[:, None]
    th = (2 * np.pi / D) * ((kd[:, None] * b[None, :]) % D)
    m = np.zeros((5, 2, 8, 64))
    m[:, 0] = (np.cos(th) * valid).reshape(5, 8, 64)
    m[:, 1] = (-np.sin(th) * valid * (kd != D // 2)[:, None]).reshape(5, 8, 64)
    half = np.where((kd == 0) | (kd == D // 2), 0.5, 1.0).reshape(5, 1, 8, 1)
    mats[4, :80, :64] = m.reshape(80, 64)
    mats[9, :64, :80] = (m * half).reshape(80, 64).T
    return _pack_rows(mats)


def _token_tables():
    l = np.arange(128)
    ones = np.ones((8, 1))
    angles = [(2 * np.pi / 128) * ((l[:8, None] * l[None, :]) % 128),
              (2 * np.pi / 128) * ((8 * l) % 128) * ones, (2 * np.pi / S) * l * ones]
    return np.concatenate([p for a in angles for p in (np.cos(a), -np.sin(a))]).astype(np.float32)


_CH_MATS = _channel_mats()
_TOK_TAB = _token_tables()


def _dot(a, b):
    return jnp.dot(a, b, preferred_element_type=f32)


def _radix9(x):
    s1, s2, s3, s4 = x[1] + x[8], x[2] + x[7], x[3] + x[6], x[4] + x[5]
    d1, d2, d3, d4 = x[1] - x[8], x[2] - x[7], x[3] - x[6], x[4] - x[5]
    p = x[0] - 0.5 * s3
    a, b = s1 - s4, s2 - s4
    r1 = _C1 * a + _C2 * b
    r2 = _C2 * a + _C4 * b
    e, g = d1 + d2, d2 + d4
    i1 = _S1 * e + _S4 * g
    i2 = _S2 * e - _S1 * g
    t, u = s1 + s2 + s4, x[0] + s3
    return u + t, [(p + r1, i1 + d3), (p + r2, i2 - d3),
                   (u - 0.5 * t, d1 - d2 + d4), ((p - r1) - r2, (i2 - i1) + d3)]


def _radix9_t(x0, uv):
    (u1, v1), (u2, v2), (u3, v3), (u4, v4) = uv
    u, t = x0 + u3, x0 - 0.5 * u3
    p, r1, r2 = u1 + u2 + u4, u1 - u4, u2 - u4
    a = _C1 * r1 + _C2 * r2
    b = _C2 * r1 + _C4 * r2
    s1, s2, s3, s4 = t + a, t + b, u - 0.5 * p, (t - a) - b
    i1, i2, d3 = v1 - v4, v2 + v4, v1 - v2 + v4
    e = _S1 * i1 + _S2 * i2
    g = _S4 * i1 - _S1 * i2
    d1, d2, d4 = e + v3, (e + g) - v3, g + v3
    return [u + p, s1 + d1, s2 + d2, s3 + d3, s4 + d4, s4 - d4, s3 - d3, s2 - d2, s1 - d1]


def _cadd(a, b):
    return a[0] + b[0], a[1] + b[1]


def _csub(a, b):
    return a[0] - b[0], a[1] - b[1]


def _cmul(a, b):
    return a[0] * b[0] - a[1] * b[1], a[0] * b[1] + a[1] * b[0]


def _cross(a, b):
    return (a[0] - b[1], a[1] + b[0]), (a[0] + b[1], a[1] - b[0])


def _radix4(x, sign):
    a, b, c, d = x
    u, v = _cadd(a, c), _cadd(b, d)
    k1, k3 = _cross(_csub(a, c), _csub(b, d))[::sign]
    return [_cadd(u, v), k1, _csub(u, v), k3]


def _twiddle16(z, e, sign):
    re, im = z
    if e == 0:
        return z
    c, s = float(np.cos(2 * np.pi * e / 16)), float(sign * np.sin(2 * np.pi * e / 16))
    if e == 4:
        return (-im, re) if sign > 0 else (im, -re)
    if e % 2 == 0:
        if c * s > 0:
            return c * (re - im), c * (re + im)
        return c * (re + im), c * (im - re)
    return c * re - s * im, s * re + c * im


def _halves(w):
    return pltpu.bitcast(w, bf16)


def _pair(a, b):
    return jnp.concatenate([a, b], axis=0).astype(bf16)


class _RowMean:
    def __init__(self, lanes=2):
        self.acc, self.n = [None] * lanes, 0

    def add(self, v):
        i = self.n % len(self.acc)
        self.acc[i] = v if self.acc[i] is None else self.acc[i] + v
        self.n += 1

    def mean(self):
        acc = self.acc
        while len(acc) > 1:
            acc = [acc[i] + acc[i + 1] for i in range(0, len(acc), 2)]
        return jnp.sum(acc[0], axis=0, keepdims=True) * (1.0 / D)


def _gelu(x):
    inner = x * (0.7978845608028654 + (0.7978845608028654 * 0.044715) * (x * x))
    hx = 0.5 * x
    return hx + hx * jnp.tanh(inner)


_LEFT = (((0, 0), 1, (1, 1)), ((1, 0), 1, (1, 1)), ((0, 0), 0, None), ((1, 1), 0, None),
         ((0, 0), 1, (0, 1)), ((1, 0), -1, (0, 0)), ((0, 1), -1, (1, 1)))
_RIGHT = (((0, 0), 1, (1, 1)), ((0, 0), 0, None), ((0, 1), -1, (1, 1)), ((1, 0), -1, (0, 0)),
          ((1, 1), 0, None), ((0, 0), 1, (0, 1)), ((1, 0), 1, (1, 1)))


def _signed_sum(term, quad):
    a, sign, b = term
    if sign == 0:
        return quad(*a)
    return quad(*a) + quad(*b) if sign > 0 else quad(*a) - quad(*b)


def _operands(table, block, order=range(7)):
    for i in order:
        outer = table[i]
        if outer[1]:
            sums = {(u, v): _signed_sum(outer, lambda r, c: block(i, 2 * r + u, 2 * c + v))
                    for u in range(2) for v in range(2)}
        for j, inner in enumerate(table):
            def quad(u, v):
                if outer[1]:
                    return sums[u, v]
                return block(7 * i + j, 2 * outer[0][0] + u, 2 * outer[0][1] + v)
            yield _signed_sum(inner, quad).astype(bf16)


_RESULT = {(0, 0): {0: 1, 3: 1, 4: -1, 6: 1}, (0, 1): {2: 1, 4: 1},
           (1, 0): {1: 1, 3: 1}, (1, 1): {0: 1, 1: -1, 2: 1, 5: 1}}


def _completed(i, have):
    for quadrant, terms in _RESULT.items():
        if i in terms and all(j in have for j in terms):
            first, *rest = terms
            x = have[first]
            for j in rest:
                x = x + have[j] if terms[j] > 0 else x - have[j]
            yield quadrant, x


def _blocks(products, order=range(7)):
    outer = {quadrant: {} for quadrant in _RESULT}
    for i in order:
        inner = {}
        for j in range(7):
            inner[j] = next(products)
            for (u, v), x in _completed(j, inner):
                outer[u, v][i] = x
                for (r, c), y in _completed(i, outer[u, v]):
                    yield (2 * r + u, 2 * c + v), y


def _kernel(x_hbm, wr_hbm, wi_hbm, w1_hbm, b1_hbm, w2_hbm, b2_hbm, c_hbm, wm_hbm, chm_hbm, tok_hbm,
            o_hbm,
            x_v, wr_v, wi_v, w1_v, b1_v, w2_v, b2_v, c_v, wm_v, chm_v, tok_v,
            mod_v, mf_v, mi_v, wt_v, wp_v, r_v, fa_v, fc_v, x1_v, a_v, acc_v, o_v, st_v,
            sem):
    slots = itertools.count()

    def copy(src, dst):
        return pltpu.make_async_copy(src, dst, sem.at[next(slots)])

    def cols(ref, lo, n):
        return ref.at[:, pl.ds(lo, n)]

    def copy_cols(src, dst, lo, n):
        return copy(cols(src, lo, n), cols(dst, lo, n))

    cp_tok, cp_c = copy(tok_hbm, tok_v), copy(c_hbm, c_v)
    cp_mod = [copy_cols(wm_hbm, wm_v, 128 * lo, 128 * (hi - lo)) for lo, hi in MOD_PARTS]
    cp_chm = [copy(chm_hbm.at[pl.ds(5 * i, 5)], chm_v.at[pl.ds(5 * i, 5)]) for i in range(2)]
    cp_w = [copy(wr_hbm, wr_v), copy(wi_hbm, wi_v)]
    cp_b1, cp_b2 = copy(b1_hbm, b1_v), copy(b2_hbm, b2_v)

    def batch(pairs):
        slot = next(slots)
        return [pltpu.make_async_copy(src, dst, sem.at[slot]) for src, dst in pairs]

    cp_w1 = [batch((cols(w1_hbm, 128 * t, 128), w1_v.at[t])
                   for t in range(lo // 128, (lo + n) // 128)) for lo, n in zip(STARTS, CHUNKS)]
    cp_w2 = [batch((w2_hbm.at[pl.ds(lo, n), pl.ds(128 * t, 128)], w2_v.at[t, pl.ds(lo, n)])
                   for t in range(NT)) for lo, n in zip(STARTS, CHUNKS)]
    sem_o, sem_x = next(slots), next(slots)

    def cp_x(i):
        lo = i * 256 if isinstance(i, int) else pl.multiple_of(i * 256, 256)
        return pltpu.make_async_copy(cols(x_hbm, lo, 256), cols(x_v, lo, 256), sem.at[sem_x + i])

    for c in (cp_tok, cp_c, cp_x(0), cp_x(1), cp_mod[0], *map(cp_x, range(2, NT // 2)), cp_chm[0],
              *cp_w, cp_chm[1], cp_mod[1], cp_b1, cp_b2, *cp_w1[0]):
        c.start()

    def lanes(t):
        if isinstance(t, int):
            return slice(128 * t, 128 * (t + 1))
        return pl.ds(pl.multiple_of(t * 128, 128), 128)

    def blk(i):
        return slice(8 * i, 8 * i + 8)

    with jax.named_scope("gen"):
        cp_tok.wait()
        rows = [(tok_v[blk(0), :], tok_v[blk(1), :])]
        for _ in range(15):
            rows.append(_cmul(rows[-1], (tok_v[blk(2), :], tok_v[blk(3), :])))
        dft = tuple(jnp.concatenate([r[i] for r in rows], axis=0) for i in range(2))
        along = tuple(jnp.concatenate([tok_v[blk(i), :]] * 16, axis=0) for i in (4, 5))
        down = tuple(a.T for a in along)

        def gen(k, carry):
            for ref, (re, im), order in zip((mf_v, mi_v), carry, ((1, 2), (2, 1))):
                for i, m in zip((0, *order), (re, re + im, re - im)):
                    ref[k, i] = m.astype(bf16)
            return _cmul(carry[0], down), _cmul(carry[1], along)

        lax.fori_loop(0, NT, gen, (dft, dft))

    cp_c.wait()
    cf = c_v[...].astype(f32)
    sc = jnp.broadcast_to(cf * jax.nn.sigmoid(cf), (16, D)).astype(bf16)

    def store_mod(j):
        row = _dot(sc, wm_v[:, lanes(j)])[0:8, :]
        n = 128 * j + lax.broadcasted_iota(jnp.int32, row.shape, 1)
        scale = jnp.logical_or(jnp.logical_and(n >= D, n < 2 * D),
                               jnp.logical_and(n >= 4 * D, n < 5 * D))
        row = jnp.where(scale, row + 1.0, row)
        row = jnp.where(jnp.logical_and(n >= 2 * D, n < 3 * D), row * (2.0 / (S * D)), row)
        mod_v[lanes(j), :] = jnp.concatenate([row] * 16, axis=0).T

    def mod(i, b=None):
        return mod_v[i * D:(i + 1) * D, :] if b is None else mod_v[blk(i * D // 8 + b), :]

    def first_mod():
        cp_mod[0].wait()
        for j in range(*MOD_PARTS[0]):
            store_mod(j)

    def stage(pair, slot, values, finish=lambda m: m):
        means = [_RowMean() for _ in pair]
        for vs in zip(*map(values, pair)):
            for m, v in zip(means, vs):
                m.add(v)
            yield
        for t, m in zip(pair, means):
            st_v[slot, t] = jnp.broadcast_to(finish(m.mean()), (8, 128))

    def in_turn(gens):
        for g, _ in gens:
            for _ in g:
                pass

    def in_step(gens):
        n = D // 8
        for q in range(n):
            for g, cuts in gens:
                for _ in range(cuts * q // n, cuts * (q + 1) // n):
                    next(g)
        in_turn(gens)

    def skewed(stages, emit, n, after_fill=lambda: None):
        depth = len(stages) - 1

        def step(oldest, lo, hi):
            emit([(fn(oldest + (depth - lag)), cuts)
                  for lag, cuts, fn in stages if lo <= lag <= hi])

        for i in range(depth):
            step(i - depth, 0, i)
        after_fill()
        lax.fori_loop(0, n - depth, lambda i, _: step(i, 0, depth), None)
        for i in range(n, n + depth):
            step(i - depth, i - n + 1, depth)

    def inv_std(var):
        return lax.rsqrt(var + EPS)

    def squares(src, slot, dst=None):
        def values(t):
            mean = st_v[slot, t]
            for b in range(D // 8):
                c = src[t, blk(b), :] - mean
                if dst is not None:
                    dst[t, blk(b), :] = c
                yield c * c
        return values

    def adjacent(i):
        return 2 * i, 2 * i + 1

    def tokens(t):
        for i in range(D // 16):
            x = x_v[16 * i:16 * i + 16, lanes(t)].astype(f32)
            for b, half in enumerate((x[:8], x[8:]), 2 * i):
                x1_v[t, blk(b), :] = half
                yield half

    def load_tokens(i):
        cp_x(i).wait()
        return stage(adjacent(i), 0, tokens)

    def fwd_butterflies(i):
        for t in adjacent(i):
            rstd = st_v[1, t]
            for p in range(8):
                x0, uv = _radix9([fc_v[t, blk(b), :] * rstd * mod(1, b) + mod(0, b)
                                  for b in range(p, D // 8, 8)])
                for g in range(4):
                    r_v[t, 128 * g + 16 * p:128 * g + 16 * p + 16, :] = _pair(*uv[g])
                if p % 2:
                    r_v[t, 504 + 8 * p:520 + 8 * p, :] = _pair(prev, x0)
                prev = x0
                yield

    with jax.named_scope("A"):
        skewed([(1, D // 8, lambda i: stage(adjacent(i), 1, squares(x1_v, 0, fc_v), inv_std)),
                (0, D // 8, load_tokens), (2, 16, fwd_butterflies)],
               in_step, NT // 2, first_mod)

    def filt_a(t):
        a = pltpu.bitcast(wr_v[0:DF - 1, lanes(t)], f32)
        b = pltpu.bitcast(wi_v[0:DF - 1, lanes(t)], f32)
        nr = wr_v[DF - 1:DF, lanes(t)].astype(f32)
        ni = wi_v[DF - 1:DF, lanes(t)].astype(f32)
        r = lax.broadcasted_iota(jnp.int32, (8, 128), 0)
        nyq = jnp.where(r == 0, nr, jnp.where(r == 1, ni, 0.0))
        rest = jnp.concatenate([a[128:], b[128:], nyq, jnp.zeros((88, 128), f32)], axis=0)
        for c, tile in enumerate((a[:128].T, b[:128].T, rest.T)):
            for j in range(8):
                lo = (NT + 1) * (8 * t + j)
                wt_v[c, lo:lo + NT, :] = tile[NT * j:NT * (j + 1)]

    def filt_b(k):
        wp_v[k, 0:128, :] = wt_v[0, pl.ds(k, 128, stride=NT + 1), :].T
        wp_v[k, 144:272, :] = wt_v[1, pl.ds(k, 128, stride=NT + 1), :].T
        rest = wt_v[2, pl.ds(k, 128, stride=NT + 1), :].T
        wp_v[k, 128:144, :] = rest[0:16]
        wp_v[k, 272:296, :] = rest[16:40]

    def filt(k, rb, base, nyq_row):
        if rb == NRB - 1:
            return jnp.broadcast_to(wp_v[k, nyq_row:nyq_row + 1, :], (8, 128))
        k0 = _row_runs()[rb // 2]
        w = pltpu.bitcast(wp_v[k, pl.ds(base + k0 // 2 + 72 * (rb % 2), 8, stride=9), :], u32)
        w = (w & np.uint32(0xFFFF0000)) if k0 % 2 else (w << 16)
        return pltpu.bitcast(w, f32)

    groups = [range(8 * g, min(8 * g + 8, NRB)) for g in range(5)]
    rounds = [(q, odd) for q in range(4) for odd in (0, 1)]

    def harmonics(q, odd):
        return q + 4 * odd, q + 4 * odd + 8

    def get(ref, i, rb):
        return ref[i, blk(2 * rb), :], ref[i, blk(2 * rb + 1), :]

    def put(ref, i, rb, z):
        ref[i, blk(2 * rb), :], ref[i, blk(2 * rb + 1), :] = z

    def token_dft(z, m_ref, k):
        def times(parts, i):
            lhs = jnp.concatenate([*parts, jnp.zeros((8, 128), f32)], axis=0).astype(bf16)
            return _dot(lhs, m_ref[k, i])
        s = times([re + im for re, im in z], 0)
        a, b = times([im for _, im in z], 1), times([re for re, _ in z], 2)
        return [(s[blk(rb)] - a[blk(rb)], s[blk(rb)] - b[blk(rb)]) for rb in range(NRB)]

    def fwd_channel(g, t0):
        tiles = range(t0, NT, 4)
        if g < 4:
            outs = [_dot(_halves(chm_v[g]), r_v[t, lanes(g), :]) for t in tiles]
        else:
            pad = jnp.zeros((64, 128), bf16)
            outs = [_dot(_halves(chm_v[4, 0:40, :]),
                         jnp.concatenate([r_v[t, 512:576, :], pad], axis=0)) for t in tiles]
        for i, rb in enumerate(groups[g]):
            y = _radix4([(o[blk(2 * i)], o[blk(2 * i + 1)]) for o in outs], -1)
            for q in range(4):
                put(fa_v, 4 * q + t0, rb, _twiddle16(y[q], t0 * q, -1))

    def fwd_token(q, odd):
        z = []
        for rb in range(NRB):
            a, b, c, d = (get(fa_v, 4 * q + t0, rb) for t0 in range(4))
            if odd:
                z.append(_cross(_csub(a, c), _csub(b, d))[::-1])
            else:
                u, v = _cadd(a, c), _cadd(b, d)
                z.append((_cadd(u, v), _csub(u, v)))
        for k, zk in zip(harmonics(q, odd), zip(*z)):
            for rb, y in enumerate(token_dft(zk, mf_v, k)):
                put(fc_v, k, rb, y)

    def inv_token(q, odd):
        outs = []
        for k in harmonics(q, odd):
            z = [_cmul(get(fc_v, k, rb), (filt(k, rb, 0, 288), filt(k, rb, 144, 289)))
                 for rb in range(NRB)]
            outs.append(token_dft(z, mi_v, k))
        for rb, (a, c) in enumerate(zip(*outs)):
            u, v = _cadd(a, c), _csub(a, c)
            if odd:
                p, m = get(fa_v, q, rb), get(fa_v, 4 + q, rb)
                y1, y3 = _cross(m, v)
                for t0, y in enumerate((_cadd(p, u), y1, _csub(p, u), y3)):
                    put(fa_v, 4 * t0 + q, rb, _twiddle16(y, t0 * q, +1))
            else:
                put(fa_v, q, rb, u)
                put(fa_v, 4 + q, rb, v)

    def inv_channel(g, t0):
        z = [_radix4([get(fa_v, 4 * t0 + q, rb) for q in range(4)], +1) for rb in groups[g]]
        for t, zt in zip(range(t0, NT, 4), zip(*z)):
            parts = [v for pair in zt for v in pair]
            if g < 4:
                fc_v[t, lanes(g), :] = _dot(_halves(chm_v[5 + g]),
                                            jnp.concatenate(parts, axis=0).astype(bf16))
            else:
                parts.append(jnp.zeros((48, 128), f32))
                fc_v[t, 512:576, :] = _dot(_halves(chm_v[9, 0:32, :]),
                                           jnp.concatenate(parts, axis=0).astype(bf16))

    def start(batch):
        for c in batch:
            c.start()

    with jax.named_scope("F"):
        start(cp_w1[1])
        cp_chm[0].wait()
        for g in range(5):
            for t0 in range(4):
                fwd_channel(g, t0)
        for i, r in enumerate(rounds):
            if i == 2:
                for c in cp_w:
                    c.wait()
            fwd_token(*r)
            if 2 <= i < 6:
                for t in range(4 * i - 8, 4 * i - 4):
                    filt_a(t)
            elif i >= 6:
                for k in harmonics(*rounds[i - 6]):
                    filt_b(k)
    with jax.named_scope("I"):
        for i, r in enumerate(rounds):
            if i < 6:
                for k in harmonics(*rounds[i + 2]):
                    filt_b(k)
            inv_token(*r)
        cp_chm[1].wait()
        cp_mod[1].wait()
        lo, hi = MOD_PARTS[1]
        for i in range(20):
            inv_channel(*divmod(i, 4))
            if lo + i < hi:
                store_mod(lo + i)

    def opposite(j):
        return j, j + NT // 2

    def residual(t):
        for p in range(8):
            uv = [(fc_v[t, blk(16 * g + 2 * p), :], fc_v[t, blk(16 * g + 2 * p + 1), :])
                  for g in range(4)]
            for a, y in enumerate(_radix9_t(fc_v[t, blk(64 + p), :], uv)):
                b = 8 * a + p
                x1 = x1_v[t, blk(b), :] + mod(2, b) * y
                x1_v[t, blk(b), :] = x1
                yield x1

    def modulated(t):
        rstd = st_v[1, t]
        for b in range(D // 8):
            h = fa_v[t, blk(b), :] * rstd * mod(4, b) + mod(3, b)
            fc_v[t, blk(b), :] = h
            yield h

    def mlp_operands(j, _):
        stats = [(j + 4 * c, st_v[2, j + 4 * c], st_v[3, j + 4 * c]) for c in range(4)]
        for r0 in range(0, HB, 16):
            h = {(r, c): jnp.concatenate([(fc_v[t, q:q + 8, :] - mean) * rstd
                                          for q in (HB * r + r0, HB * r + r0 + 8)], axis=0)
                 for r in range(4) for c, (t, mean, rstd) in enumerate(stats)}
            for i, a in enumerate(_operands(_LEFT, lambda _, r, c: h[r, c])):
                a_v[i, j, r0:r0 + 16, :] = a

    with jax.named_scope("C"):
        skewed([(1, D // 8, lambda j: stage(opposite(j), 1, squares(x1_v, 0, fa_v), inv_std)),
                (0, D // 8, lambda j: stage(opposite(j), 0, residual))], in_turn, NT // 2)
        skewed([(1, D // 8, lambda j: stage(opposite(j), 3, squares(fc_v, 2), inv_std)),
                (0, D // 8, lambda j: stage(opposite(j), 2, modulated))], in_turn, NT // 2)
        lax.fori_loop(0, 4, mlp_operands, None)

    zero = pl.program_id(0)
    a_words = a_v.bitcast(u32)

    def weights(ref, top, height, left, stride, width, order=range(7)):
        def block(i, r, c):
            rows = pl.ds(pl.multiple_of((top + r * height) // 2 + 8 * i * zero, 8), height // 2)
            first = (left + c * stride) // 128
            words = [ref.bitcast(u32)[t, rows, :] for t in range(first, first + width // 128)]
            return _halves(jnp.concatenate(words, axis=1)).astype(f32)
        return _operands(_RIGHT, block, order)

    def hidden(j):
        lo, n = STARTS[j], CHUNKS[j] // 4
        bias = [jnp.concatenate([b1[t:t + 1, :] for t in range((lo + c * n) // 128,
                                                               (lo + c * n + n) // 128)], axis=1)
                for c in range(4)]
        return {(r, c): _gelu(x + bias[c]) for (r, c), x in _blocks(
            _dot(_halves(jnp.concatenate([a_words[i, t] for t in range(4)], axis=1)), w)
            for i, w in enumerate(weights(w1_v, 0, SB, lo, n, n)))}

    def products(j, g):
        for a, w in zip(_operands(_LEFT, lambda _, r, c: g[r, c]),
                        weights(w2_v, STARTS[j], CHUNKS[j] // 4, 0, SB, SB)):
            yield _dot(a, w)

    def advance(landed, queued):
        for c in landed:
            c.wait()
        start(queued)

    with jax.named_scope("MLP"):
        advance((cp_b1, cp_b2, *cp_w1[0]), (*cp_w2[0], *cp_w1[2]))
        b1, b2 = b1_v[...].astype(f32), b2_v[...].astype(f32)
        g0 = hidden(0)
        advance(cp_w1[1], cp_w2[1])
        g1 = hidden(1)
        advance((*cp_w2[0], *cp_w1[2]), cp_w2[2])
        for i, m in enumerate(products(0, g0)):
            acc_v[i] = m
        g2 = hidden(2)
        advance((*cp_w2[1], *cp_w2[2]), ())
        for i, m in enumerate(products(1, g1)):
            acc_v[i] += m

        def finish(r, c, y):
            rows = slice(HB * r, HB * (r + 1))
            for j in range(4):
                t = 4 * c + j
                yt = y[:, lanes(j)] + b2[t:t + 1, :]
                o_v[t, rows, :] = (x1_v[t, rows, :] + mod_v[5 * D + HB * r:5 * D + HB * (r + 1), :]
                                   * yt).astype(bf16)
                pltpu.make_async_copy(
                    o_v.at[t, rows], o_hbm.at[rows, lanes(t)], sem.at[sem_o]).start()

        for (r, c), y in _blocks((acc_v[i] + m for i, m in enumerate(products(2, g2)))):
            finish(r, c, y)
        pltpu.make_async_copy(o_v, o_v, sem.at[sem_o]).wait()


@jax.jit
def pallas_adaLN_cond__spectral_gfnet__mixer_token_mlp__prompt_kernel(
    A_x: jax.Array,
    A_w_r: jax.Array,
    A_w_i: jax.Array,
    B_x: jax.Array,
    B_w1: jax.Array,
    B_b1: jax.Array,
    B_w2: jax.Array,
    B_b2: jax.Array,
    c: jax.Array,
    w_mod: jax.Array,
):
    del B_x
    vmem = pltpu.VMEM
    scratch = [
        vmem((D, S), bf16), vmem((DF, S), bf16), vmem((DF, S), bf16),
        vmem((F // 128, S, 128), bf16), vmem((F // 128, 128), bf16),
        vmem((NT, F, 128), bf16), vmem((S // 128, 128), bf16),
        vmem((1, D), bf16), vmem((D, 6 * D), bf16),
        vmem(_CH_MATS.shape, u32), vmem(_TOK_TAB.shape, f32),
        vmem((6 * D, 128), f32),
        vmem((NT, 3, 128, 128), bf16),
        vmem((NT, 3, 128, 128), bf16),
        vmem((3, S + 128, 128), f32),
        vmem((NT, 296, 128), f32),
        vmem((NT, D, 128), bf16),
        vmem((NT, NRB * 16, 128), f32),
        vmem((NT, NRB * 16, 128), f32),
        vmem((NT, D, 128), f32),
        vmem((49, 4, HB, 128), bf16),
        vmem((49, HB, SB), f32),
        vmem((NT, D, 128), bf16),
        vmem((4, NT, 8, 128), f32),
        pltpu.SemaphoreType.DMA((64,)),
    ]
    out = pl.pallas_call(
        _kernel,
        grid=(1,),
        in_specs=[pl.BlockSpec(memory_space=pl.ANY)] * 11,
        out_specs=pl.BlockSpec(memory_space=pl.ANY),
        out_shape=jax.ShapeDtypeStruct((D, S), bf16),
        scratch_shapes=scratch,
        compiler_params=pltpu.CompilerParams(vmem_limit_bytes=124 * 1024 * 1024),
    )(A_x[0].T, A_w_r.T, A_w_i.T, B_w1, B_b1.reshape(F // 128, 128), B_w2,
      B_b2.reshape(S // 128, 128), c, w_mod, _CH_MATS, _TOK_TAB)
    return out.T[None]
```

```python
import itertools

import jax
import jax.numpy as jnp
import numpy as np
from jax import lax
from jax.experimental import pallas as pl
from jax.experimental.pallas import tpu as pltpu

D, S, F = 576, 2048, 4608
DF = D // 2 + 1
NT = S // 128
NRB = 37
EPS = 1e-5
HB, SB = D // 4, S // 4
CHUNKS = (1024, 1536, 2048)
STARTS = tuple(sum(CHUNKS[:j]) for j in range(len(CHUNKS)))
MOD_PARTS = ((0, 9), (9, 27))

f32, bf16, u32 = jnp.float32, jnp.bfloat16, jnp.uint32

_Q = np.sqrt(3.0) / 2
_C1, _C2, _C4 = (float(np.cos(2 * np.pi * k / 9)) for k in (1, 2, 4))
_S1, _S2, _S4 = (float(np.sin(2 * np.pi * k / 9) / _Q) for k in (1, 2, 4))


def _row_runs():
    runs = []
    for g in (1, 2, 3, 4):
        for r in (g, 9 - g):
            runs += [r, r + 9]
    return runs + [0, 9]


def _pack_rows(m):
    b = m.astype(np.float32).astype(jnp.bfloat16).view(np.uint16).astype(np.uint32)
    return b[..., 0::2, :] | (b[..., 1::2, :] << np.uint32(16))


def _channel_mats():
    kd_all = [k0 + 18 * j for k0 in _row_runs() for j in range(16)] + [D // 2] + [-1] * 7
    kd_all = np.array(kd_all)
    b = np.arange(64)
    mats = np.zeros((10, 128, 128))
    for g in (1, 2, 3, 4):
        kd = kd_all[64 * (g - 1):64 * g]
        sg = np.where(kd % 9 == g, -1.0, 1.0).reshape(8, 8, 1, 1)
        th = (2 * np.pi / D) * ((kd[:, None] * b[None, :]) % D)
        c, s = np.cos(th).reshape(8, 8, 8, 8), np.sin(th).reshape(8, 8, 8, 8)
        m = np.zeros((8, 2, 8, 8, 2, 8))
        m[:, 0, :, :, 0, :] = c
        m[:, 0, :, :, 1, :] = sg * _Q * s
        m[:, 1, :, :, 0, :] = -s
        m[:, 1, :, :, 1, :] = sg * _Q * c
        mats[g - 1] = m.reshape(128, 128)
        mats[5 + g - 1] = m.reshape(128, 128).T
    kd = kd_all[256:]
    valid = (kd >= 0)[:, None]
    th = (2 * np.pi / D) * ((kd[:, None] * b[None, :]) % D)
    m = np.zeros((5, 2, 8, 64))
    m[:, 0] = (np.cos(th) * valid).reshape(5, 8, 64)
    m[:, 1] = (-np.sin(th) * valid * (kd != D // 2)[:, None]).reshape(5, 8, 64)
    half = np.where((kd == 0) | (kd == D // 2), 0.5, 1.0).reshape(5, 1, 8, 1)
    mats[4, :80, :64] = m.reshape(80, 64)
    mats[9, :64, :80] = (m * half).reshape(80, 64).T
    return _pack_rows(mats)


def _token_tables():
    l = np.arange(128)
    ones = np.ones((8, 1))
    angles = [(2 * np.pi / 128) * ((l[:8, None] * l[None, :]) % 128),
              (2 * np.pi / 128) * ((8 * l) % 128) * ones, (2 * np.pi / S) * l * ones]
    return np.concatenate([p for a in angles for p in (np.cos(a), -np.sin(a))]).astype(np.float32)


_CH_MATS = _channel_mats()
_TOK_TAB = _token_tables()


def _dot(a, b):
    return jnp.dot(a, b, preferred_element_type=f32)


def _radix9(x):
    s1, s2, s3, s4 = x[1] + x[8], x[2] + x[7], x[3] + x[6], x[4] + x[5]
    d1, d2, d3, d4 = x[1] - x[8], x[2] - x[7], x[3] - x[6], x[4] - x[5]
    p = x[0] - 0.5 * s3
    a, b = s1 - s4, s2 - s4
    r1 = _C1 * a + _C2 * b
    r2 = _C2 * a + _C4 * b
    e, g = d1 + d2, d2 + d4
    i1 = _S1 * e + _S4 * g
    i2 = _S2 * e - _S1 * g
    t, u = s1 + s2 + s4, x[0] + s3
    return u + t, [(p + r1, i1 + d3), (p + r2, i2 - d3),
                   (u - 0.5 * t, d1 - d2 + d4), ((p - r1) - r2, (i2 - i1) + d3)]


def _radix9_t(x0, uv):
    (u1, v1), (u2, v2), (u3, v3), (u4, v4) = uv
    u, t = x0 + u3, x0 - 0.5 * u3
    p, r1, r2 = u1 + u2 + u4, u1 - u4, u2 - u4
    a = _C1 * r1 + _C2 * r2
    b = _C2 * r1 + _C4 * r2
    s1, s2, s3, s4 = t + a, t + b, u - 0.5 * p, (t - a) - b
    i1, i2, d3 = v1 - v4, v2 + v4, v1 - v2 + v4
    e = _S1 * i1 + _S2 * i2
    g = _S4 * i1 - _S1 * i2
    d1, d2, d4 = e + v3, (e + g) - v3, g + v3
    return [u + p, s1 + d1, s2 + d2, s3 + d3, s4 + d4, s4 - d4, s3 - d3, s2 - d2, s1 - d1]


def _cadd(a, b):
    return a[0] + b[0], a[1] + b[1]


def _csub(a, b):
    return a[0] - b[0], a[1] - b[1]


def _cmul(a, b):
    return a[0] * b[0] - a[1] * b[1], a[0] * b[1] + a[1] * b[0]


def _cross(a, b):
    return (a[0] - b[1], a[1] + b[0]), (a[0] + b[1], a[1] - b[0])


def _radix4(x, sign):
    a, b, c, d = x
    u, v = _cadd(a, c), _cadd(b, d)
    k1, k3 = _cross(_csub(a, c), _csub(b, d))[::sign]
    return [_cadd(u, v), k1, _csub(u, v), k3]


def _twiddle16(z, e, sign):
    re, im = z
    if e == 0:
        return z
    c, s = float(np.cos(2 * np.pi * e / 16)), float(sign * np.sin(2 * np.pi * e / 16))
    if e == 4:
        return (-im, re) if sign > 0 else (im, -re)
    if e % 2 == 0:
        if c * s > 0:
            return c * (re - im), c * (re + im)
        return c * (re + im), c * (im - re)
    return c * re - s * im, s * re + c * im


def _halves(w):
    return pltpu.bitcast(w, bf16)


def _pair(a, b):
    return jnp.concatenate([a, b], axis=0).astype(bf16)


class _RowMean:
    def __init__(self, lanes=2):
        self.acc, self.n = [None] * lanes, 0

    def add(self, v):
        i = self.n % len(self.acc)
        self.acc[i] = v if self.acc[i] is None else self.acc[i] + v
        self.n += 1

    def mean(self):
        acc = self.acc
        while len(acc) > 1:
            acc = [acc[i] + acc[i + 1] for i in range(0, len(acc), 2)]
        return jnp.sum(acc[0], axis=0, keepdims=True) * (1.0 / D)


def _gelu(x):
    inner = x * (0.7978845608028654 + (0.7978845608028654 * 0.044715) * (x * x))
    hx = 0.5 * x
    return hx + hx * jnp.tanh(inner)


_LEFT = (((0, 0), 1, (1, 1)), ((1, 0), 1, (1, 1)), ((0, 0), 0, None), ((1, 1), 0, None),
         ((0, 0), 1, (0, 1)), ((1, 0), -1, (0, 0)), ((0, 1), -1, (1, 1)))
_RIGHT = (((0, 0), 1, (1, 1)), ((0, 0), 0, None), ((0, 1), -1, (1, 1)), ((1, 0), -1, (0, 0)),
          ((1, 1), 0, None), ((0, 0), 1, (0, 1)), ((1, 0), 1, (1, 1)))


def _signed_sum(term, quad):
    a, sign, b = term
    if sign == 0:
        return quad(*a)
    return quad(*a) + quad(*b) if sign > 0 else quad(*a) - quad(*b)


def _operands(table, block, order=range(7)):
    for i in order:
        outer = table[i]
        if outer[1]:
            sums = {(u, v): _signed_sum(outer, lambda r, c: block(i, 2 * r + u, 2 * c + v))
                    for u in range(2) for v in range(2)}
        for j, inner in enumerate(table):
            def quad(u, v):
                if outer[1]:
                    return sums[u, v]
                return block(7 * i + j, 2 * outer[0][0] + u, 2 * outer[0][1] + v)
            yield _signed_sum(inner, quad).astype(bf16)


_RESULT = {(0, 0): {0: 1, 3: 1, 4: -1, 6: 1}, (0, 1): {2: 1, 4: 1},
           (1, 0): {1: 1, 3: 1}, (1, 1): {0: 1, 1: -1, 2: 1, 5: 1}}


def _completed(i, have):
    for quadrant, terms in _RESULT.items():
        if i in terms and all(j in have for j in terms):
            first, *rest = terms
            x = have[first]
            for j in rest:
                x = x + have[j] if terms[j] > 0 else x - have[j]
            yield quadrant, x


def _blocks(products, order=range(7)):
    outer = {quadrant: {} for quadrant in _RESULT}
    for i in order:
        inner = {}
        for j in range(7):
            inner[j] = next(products)
            for (u, v), x in _completed(j, inner):
                outer[u, v][i] = x
                for (r, c), y in _completed(i, outer[u, v]):
                    yield (2 * r + u, 2 * c + v), y


def _kernel(x_hbm, wr_hbm, wi_hbm, w1_hbm, b1_hbm, w2_hbm, b2_hbm, c_hbm, wm_hbm, chm_hbm, tok_hbm,
            o_hbm,
            x_v, wr_v, wi_v, w1_v, b1_v, w2_v, b2_v, c_v, wm_v, chm_v, tok_v,
            mod_v, mf_v, mi_v, wt_v, wp_v, r_v, fa_v, fc_v, x1_v, a_v, acc_v, o_v, st_v,
            sem):
    slots = itertools.count()

    def copy(src, dst):
        return pltpu.make_async_copy(src, dst, sem.at[next(slots)])

    def cols(ref, lo, n):
        return ref.at[:, pl.ds(lo, n)]

    def copy_cols(src, dst, lo, n):
        return copy(cols(src, lo, n), cols(dst, lo, n))

    cp_tok, cp_c = copy(tok_hbm, tok_v), copy(c_hbm, c_v)
    cp_mod = [copy_cols(wm_hbm, wm_v, 128 * lo, 128 * (hi - lo)) for lo, hi in MOD_PARTS]
    cp_chm = [copy(chm_hbm.at[pl.ds(5 * i, 5)], chm_v.at[pl.ds(5 * i, 5)]) for i in range(2)]
    cp_w = [copy(wr_hbm, wr_v), copy(wi_hbm, wi_v)]
    cp_b1, cp_b2 = copy(b1_hbm, b1_v), copy(b2_hbm, b2_v)

    def batch(pairs):
        slot = next(slots)
        return [pltpu.make_async_copy(src, dst, sem.at[slot]) for src, dst in pairs]

    cp_w1 = [batch((cols(w1_hbm, 128 * t, 128), w1_v.at[t])
                   for t in range(lo // 128, (lo + n) // 128)) for lo, n in zip(STARTS, CHUNKS)]
    cp_w2 = [batch((w2_hbm.at[pl.ds(lo, n), pl.ds(128 * t, 128)], w2_v.at[t, pl.ds(lo, n)])
                   for t in range(NT)) for lo, n in zip(STARTS, CHUNKS)]
    sem_o, sem_x = next(slots), next(slots)

    def cp_x(i):
        lo = i * 256 if isinstance(i, int) else pl.multiple_of(i * 256, 256)
        return pltpu.make_async_copy(cols(x_hbm, lo, 256), cols(x_v, lo, 256), sem.at[sem_x + i])

    for c in (cp_tok, cp_c, cp_x(0), cp_x(1), cp_mod[0], *map(cp_x, range(2, NT // 2)), cp_chm[0],
              *cp_w, cp_chm[1], cp_mod[1], cp_b1, cp_b2, *cp_w1[0]):
        c.start()

    def lanes(t):
        if isinstance(t, int):
            return slice(128 * t, 128 * (t + 1))
        return pl.ds(pl.multiple_of(t * 128, 128), 128)

    def blk(i):
        return slice(8 * i, 8 * i + 8)

    with jax.named_scope("gen"):
        cp_tok.wait()
        rows = [(tok_v[blk(0), :], tok_v[blk(1), :])]
        for _ in range(15):
            rows.append(_cmul(rows[-1], (tok_v[blk(2), :], tok_v[blk(3), :])))
        dft = tuple(jnp.concatenate([r[i] for r in rows], axis=0) for i in range(2))
        along = tuple(jnp.concatenate([tok_v[blk(i), :]] * 16, axis=0) for i in (4, 5))
        down = tuple(a.T for a in along)

        def gen(k, carry):
            for ref, (re, im), order in zip((mf_v, mi_v), carry, ((1, 2), (2, 1))):
                for i, m in zip((0, *order), (re, re + im, re - im)):
                    ref[k, i] = m.astype(bf16)
            return _cmul(carry[0], down), _cmul(carry[1], along)

        lax.fori_loop(0, NT, gen, (dft, dft))

    cp_c.wait()
    cf = c_v[...].astype(f32)
    sc = jnp.broadcast_to(cf * jax.nn.sigmoid(cf), (16, D)).astype(bf16)

    def store_mod(j):
        row = _dot(sc, wm_v[:, lanes(j)])[0:8, :]
        n = 128 * j + lax.broadcasted_iota(jnp.int32, row.shape, 1)
        scale = jnp.logical_or(jnp.logical_and(n >= D, n < 2 * D),
                               jnp.logical_and(n >= 4 * D, n < 5 * D))
        row = jnp.where(scale, row + 1.0, row)
        row = jnp.where(jnp.logical_and(n >= 2 * D, n < 3 * D), row * (2.0 / (S * D)), row)
        mod_v[lanes(j), :] = jnp.concatenate([row] * 16, axis=0).T

    def mod(i, b=None):
        return mod_v[i * D:(i + 1) * D, :] if b is None else mod_v[blk(i * D // 8 + b), :]

    def first_mod():
        cp_mod[0].wait()
        for j in range(*MOD_PARTS[0]):
            store_mod(j)

    def stage(pair, slot, values, finish=lambda m: m):
        means = [_RowMean() for _ in pair]
        for vs in zip(*map(values, pair)):
            for m, v in zip(means, vs):
                m.add(v)
            yield
        for t, m in zip(pair, means):
            st_v[slot, t] = jnp.broadcast_to(finish(m.mean()), (8, 128))

    def in_turn(gens):
        for g, _ in gens:
            for _ in g:
                pass

    def in_step(gens):
        n = D // 8
        for q in range(n):
            for g, cuts in gens:
                for _ in range(cuts * q // n, cuts * (q + 1) // n):
                    next(g)
        in_turn(gens)

    def skewed(stages, emit, n, after_fill=lambda: None):
        depth = len(stages) - 1

        def step(oldest, lo, hi):
            emit([(fn(oldest + (depth - lag)), cuts)
                  for lag, cuts, fn in stages if lo <= lag <= hi])

        for i in range(depth):
            step(i - depth, 0, i)
        after_fill()
        lax.fori_loop(0, n - depth, lambda i, _: step(i, 0, depth), None)
        for i in range(n, n + depth):
            step(i - depth, i - n + 1, depth)

    def inv_std(var):
        return lax.rsqrt(var + EPS)

    def squares(src, slot, dst=None):
        def values(t):
            mean = st_v[slot, t]
            for b in range(D // 8):
                c = src[t, blk(b), :] - mean
                if dst is not None:
                    dst[t, blk(b), :] = c
                yield c * c
        return values

    def adjacent(i):
        return 2 * i, 2 * i + 1

    def tokens(t):
        for i in range(D // 16):
            x = x_v[16 * i:16 * i + 16, lanes(t)].astype(f32)
            for b, half in enumerate((x[:8], x[8:]), 2 * i):
                x1_v[t, blk(b), :] = half
                yield half

    def load_tokens(i):
        cp_x(i).wait()
        return stage(adjacent(i), 0, tokens)

    def fwd_butterflies(i):
        for t in adjacent(i):
            rstd = st_v[1, t]
            for p in range(8):
                x0, uv = _radix9([fc_v[t, blk(b), :] * rstd * mod(1, b) + mod(0, b)
                                  for b in range(p, D // 8, 8)])
                for g in range(4):
                    r_v[t, 128 * g + 16 * p:128 * g + 16 * p + 16, :] = _pair(*uv[g])
                if p % 2:
                    r_v[t, 504 + 8 * p:520 + 8 * p, :] = _pair(prev, x0)
                prev = x0
                yield

    with jax.named_scope("A"):
        skewed([(1, D // 8, lambda i: stage(adjacent(i), 1, squares(x1_v, 0, fc_v), inv_std)),
                (0, D // 8, load_tokens), (2, 16, fwd_butterflies)],
               in_step, NT // 2, first_mod)

    def filt_a(t):
        a = pltpu.bitcast(wr_v[0:DF - 1, lanes(t)], u32)
        b = pltpu.bitcast(wi_v[0:DF - 1, lanes(t)], u32)
        nr = wr_v[DF - 1:DF, lanes(t)].astype(f32)
        ni = wi_v[DF - 1:DF, lanes(t)].astype(f32)
        r = lax.broadcasted_iota(jnp.int32, (8, 128), 0)
        nyq = pltpu.bitcast(jnp.where(r == 0, nr, jnp.where(r == 1, ni, 0.0)), u32)
        rest = jnp.concatenate([a[128:], b[128:], nyq, jnp.zeros((88, 128), u32)], axis=0)
        for c, tile in enumerate((a[:128].T, b[:128].T, rest.T)):
            for j in range(8):
                lo = (NT + 1) * (8 * t + j)
                wt_v[c, lo:lo + NT, :] = tile[NT * j:NT * (j + 1)]

    def filt_b(k):
        wp_v[k, 0:128, :] = wt_v[0, pl.ds(k, 128, stride=NT + 1), :].T
        wp_v[k, 144:272, :] = wt_v[1, pl.ds(k, 128, stride=NT + 1), :].T
        rest = wt_v[2, pl.ds(k, 128, stride=NT + 1), :].T
        wp_v[k, 128:144, :] = rest[0:16]
        wp_v[k, 272:296, :] = rest[16:40]

    def filt(k, rb, base, nyq_row):
        if rb == NRB - 1:
            w = jnp.broadcast_to(wp_v[k, nyq_row:nyq_row + 1, :], (8, 128))
        else:
            k0 = _row_runs()[rb // 2]
            w = wp_v[k, pl.ds(base + k0 // 2 + 72 * (rb % 2), 8, stride=9), :]
            w = (w & np.uint32(0xFFFF0000)) if k0 % 2 else (w << 16)
        return pltpu.bitcast(w, f32)

    groups = [range(8 * g, min(8 * g + 8, NRB)) for g in range(5)]
    rounds = [(q, odd) for q in range(4) for odd in (0, 1)]

    def harmonics(q, odd):
        return q + 4 * odd, q + 4 * odd + 8

    def get(ref, i, rb):
        return ref[i, blk(2 * rb), :], ref[i, blk(2 * rb + 1), :]

    def put(ref, i, rb, z):
        ref[i, blk(2 * rb), :], ref[i, blk(2 * rb + 1), :] = z

    def token_dft(z, m_ref, k):
        def times(parts, i):
            lhs = jnp.concatenate([*parts, jnp.zeros((8, 128), f32)], axis=0).astype(bf16)
            return _dot(lhs, m_ref[k, i])
        s = times([re + im for re, im in z], 0)
        a, b = times([im for _, im in z], 1), times([re for re, _ in z], 2)
        return [(s[blk(rb)] - a[blk(rb)], s[blk(rb)] - b[blk(rb)]) for rb in range(NRB)]

    def fwd_channel(g, t0):
        tiles = range(t0, NT, 4)
        if g < 4:
            outs = [_dot(_halves(chm_v[g]), r_v[t, lanes(g), :]) for t in tiles]
        else:
            pad = jnp.zeros((64, 128), bf16)
            outs = [_dot(_halves(chm_v[4, 0:40, :]),
                         jnp.concatenate([r_v[t, 512:576, :], pad], axis=0)) for t in tiles]
        for i, rb in enumerate(groups[g]):
            y = _radix4([(o[blk(2 * i)], o[blk(2 * i + 1)]) for o in outs], -1)
            for q in range(4):
                put(fa_v, 4 * q + t0, rb, _twiddle16(y[q], t0 * q, -1))

    def fwd_token(q, odd):
        z = []
        for rb in range(NRB):
            a, b, c, d = (get(fa_v, 4 * q + t0, rb) for t0 in range(4))
            if odd:
                z.append(_cross(_csub(a, c), _csub(b, d))[::-1])
            else:
                u, v = _cadd(a, c), _cadd(b, d)
                z.append((_cadd(u, v), _csub(u, v)))
        for k, zk in zip(harmonics(q, odd), zip(*z)):
            for rb, y in enumerate(token_dft(zk, mf_v, k)):
                put(fc_v, k, rb, y)

    def inv_token(q, odd):
        outs = []
        for k in harmonics(q, odd):
            z = [_cmul(get(fc_v, k, rb), (filt(k, rb, 0, 288), filt(k, rb, 144, 289)))
                 for rb in range(NRB)]
            outs.append(token_dft(z, mi_v, k))
        for rb, (a, c) in enumerate(zip(*outs)):
            u, v = _cadd(a, c), _csub(a, c)
            if odd:
                p, m = get(fa_v, q, rb), get(fa_v, 4 + q, rb)
                y1, y3 = _cross(m, v)
                for t0, y in enumerate((_cadd(p, u), y1, _csub(p, u), y3)):
                    put(fa_v, 4 * t0 + q, rb, _twiddle16(y, t0 * q, +1))
            else:
                put(fa_v, q, rb, u)
                put(fa_v, 4 + q, rb, v)

    def inv_channel(g, t0):
        z = [_radix4([get(fa_v, 4 * t0 + q, rb) for q in range(4)], +1) for rb in groups[g]]
        for t, zt in zip(range(t0, NT, 4), zip(*z)):
            parts = [v for pair in zt for v in pair]
            if g < 4:
                fc_v[t, lanes(g), :] = _dot(_halves(chm_v[5 + g]),
                                            jnp.concatenate(parts, axis=0).astype(bf16))
            else:
                parts.append(jnp.zeros((48, 128), f32))
                fc_v[t, 512:576, :] = _dot(_halves(chm_v[9, 0:32, :]),
                                           jnp.concatenate(parts, axis=0).astype(bf16))

    def start(batch):
        for c in batch:
            c.start()

    with jax.named_scope("F"):
        start(cp_w1[1])
        cp_chm[0].wait()
        for g in range(5):
            for t0 in range(4):
                fwd_channel(g, t0)
        for i, r in enumerate(rounds):
            if i == 2:
                for c in cp_w:
                    c.wait()
            fwd_token(*r)
            if 2 <= i < 6:
                for t in range(4 * i - 8, 4 * i - 4):
                    filt_a(t)
            elif i >= 6:
                for k in harmonics(*rounds[i - 6]):
                    filt_b(k)
    with jax.named_scope("I"):
        for i, r in enumerate(rounds):
            if i < 6:
                for k in harmonics(*rounds[i + 2]):
                    filt_b(k)
            inv_token(*r)
        cp_chm[1].wait()
        cp_mod[1].wait()
        lo, hi = MOD_PARTS[1]
        for i in range(20):
            inv_channel(*divmod(i, 4))
            if lo + i < hi:
                store_mod(lo + i)

    def opposite(j):
        return j, j + NT // 2

    def residual(t):
        for p in range(8):
            uv = [(fc_v[t, blk(16 * g + 2 * p), :], fc_v[t, blk(16 * g + 2 * p + 1), :])
                  for g in range(4)]
            for a, y in enumerate(_radix9_t(fc_v[t, blk(64 + p), :], uv)):
                b = 8 * a + p
                x1 = x1_v[t, blk(b), :] + mod(2, b) * y
                x1_v[t, blk(b), :] = x1
                yield x1

    def modulated(t):
        rstd = st_v[1, t]
        for b in range(D // 8):
            h = fa_v[t, blk(b), :] * rstd * mod(4, b) + mod(3, b)
            fc_v[t, blk(b), :] = h
            yield h

    def mlp_operands(j, _):
        stats = [(j + 4 * c, st_v[2, j + 4 * c], st_v[3, j + 4 * c]) for c in range(4)]
        for r0 in range(0, HB, 16):
            h = {(r, c): jnp.concatenate([(fc_v[t, q:q + 8, :] - mean) * rstd
                                          for q in (HB * r + r0, HB * r + r0 + 8)], axis=0)
                 for r in range(4) for c, (t, mean, rstd) in enumerate(stats)}
            for i, a in enumerate(_operands(_LEFT, lambda _, r, c: h[r, c])):
                a_v[i, j, r0:r0 + 16, :] = a

    with jax.named_scope("C"):
        skewed([(1, D // 8, lambda j: stage(opposite(j), 1, squares(x1_v, 0, fa_v), inv_std)),
                (0, D // 8, lambda j: stage(opposite(j), 0, residual))], in_turn, NT // 2)
        skewed([(1, D // 8, lambda j: stage(opposite(j), 3, squares(fc_v, 2), inv_std)),
                (0, D // 8, lambda j: stage(opposite(j), 2, modulated))], in_turn, NT // 2)
        lax.fori_loop(0, 4, mlp_operands, None)

    zero = pl.program_id(0)
    a_words = a_v.bitcast(u32)

    def weights(ref, top, height, left, stride, width, order=range(7)):
        def block(i, r, c):
            rows = pl.ds(pl.multiple_of((top + r * height) // 2 + 8 * i * zero, 8), height // 2)
            first = (left + c * stride) // 128
            words = [ref.bitcast(u32)[t, rows, :] for t in range(first, first + width // 128)]
            return _halves(jnp.concatenate(words, axis=1)).astype(f32)
        return _operands(_RIGHT, block, order)

    def hidden(j):
        lo, n = STARTS[j], CHUNKS[j] // 4
        bias = [jnp.concatenate([b1[t:t + 1, :] for t in range((lo + c * n) // 128,
                                                               (lo + c * n + n) // 128)], axis=1)
                for c in range(4)]
        return {(r, c): _gelu(x + bias[c]) for (r, c), x in _blocks(
            _dot(_halves(jnp.concatenate([a_words[i, t] for t in range(4)], axis=1)), w)
            for i, w in enumerate(weights(w1_v, 0, SB, lo, n, n)))}

    def products(j, g):
        for a, w in zip(_operands(_LEFT, lambda _, r, c: g[r, c]),
                        weights(w2_v, STARTS[j], CHUNKS[j] // 4, 0, SB, SB)):
            yield _dot(a, w)

    def advance(landed, queued):
        for c in landed:
            c.wait()
        start(queued)

    with jax.named_scope("MLP"):
        advance((cp_b1, cp_b2, *cp_w1[0]), (*cp_w2[0], *cp_w1[2]))
        b1, b2 = b1_v[...].astype(f32), b2_v[...].astype(f32)
        g0 = hidden(0)
        advance(cp_w1[1], cp_w2[1])
        g1 = hidden(1)
        advance((*cp_w2[0], *cp_w1[2]), cp_w2[2])
        for i, m in enumerate(products(0, g0)):
            acc_v[i] = m
        g2 = hidden(2)
        advance((*cp_w2[1], *cp_w2[2]), ())
        for i, m in enumerate(products(1, g1)):
            acc_v[i] += m

        def finish(r, c, y):
            rows = slice(HB * r, HB * (r + 1))
            for j in range(4):
                t = 4 * c + j
                yt = y[:, lanes(j)] + b2[t:t + 1, :]
                o_v[t, rows, :] = (x1_v[t, rows, :] + mod_v[5 * D + HB * r:5 * D + HB * (r + 1), :]
                                   * yt).astype(bf16)
                pltpu.make_async_copy(
                    o_v.at[t, rows], o_hbm.at[rows, lanes(t)], sem.at[sem_o]).start()

        for (r, c), y in _blocks((acc_v[i] + m for i, m in enumerate(products(2, g2)))):
            finish(r, c, y)
        pltpu.make_async_copy(o_hbm, o_hbm, sem.at[sem_o]).wait()


@jax.jit
def pallas_adaLN_cond__spectral_gfnet__mixer_token_mlp__prompt_kernel(
    A_x: jax.Array,
    A_w_r: jax.Array,
    A_w_i: jax.Array,
    B_x: jax.Array,
    B_w1: jax.Array,
    B_b1: jax.Array,
    B_w2: jax.Array,
    B_b2: jax.Array,
    c: jax.Array,
    w_mod: jax.Array,
):
    del B_x
    vmem = pltpu.VMEM
    scratch = [
        vmem((D, S), bf16), vmem((DF, S), bf16), vmem((DF, S), bf16),
        vmem((F // 128, S, 128), bf16), vmem((F // 128, 128), bf16),
        vmem((NT, F, 128), bf16), vmem((S // 128, 128), bf16),
        vmem((1, D), bf16), vmem((D, 6 * D), bf16),
        vmem(_CH_MATS.shape, u32), vmem(_TOK_TAB.shape, f32),
        vmem((6 * D, 128), f32),
        vmem((NT, 3, 128, 128), bf16),
        vmem((NT, 3, 128, 128), bf16),
        vmem((3, S + 128, 128), u32),
        vmem((NT, 296, 128), u32),
        vmem((NT, D, 128), bf16),
        vmem((NT, NRB * 16, 128), f32),
        vmem((NT, NRB * 16, 128), f32),
        vmem((NT, D, 128), f32),
        vmem((49, 4, HB, 128), bf16),
        vmem((49, HB, SB), f32),
        vmem((NT, D, 128), bf16),
        vmem((4, NT, 8, 128), f32),
        pltpu.SemaphoreType.DMA((64,)),
    ]
    out = pl.pallas_call(
        _kernel,
        grid=(1,),
        in_specs=[pl.BlockSpec(memory_space=pl.ANY)] * 11,
        out_specs=pl.BlockSpec(memory_space=pl.ANY),
        out_shape=jax.ShapeDtypeStruct((D, S), bf16),
        scratch_shapes=scratch,
        compiler_params=pltpu.CompilerParams(vmem_limit_bytes=124 * 1024 * 1024),
    )(A_x.reshape(S, D).T, A_w_r.T, A_w_i.T, B_w1, B_b1.reshape(F // 128, 128), B_w2,
      B_b2.reshape(S // 128, 128), c, w_mod, _CH_MATS, _TOK_TAB)
    return out.T.reshape(1, S, D)
```

```python
import jax
import jax.numpy as jnp
import numpy as np
from jax import lax
from jax.experimental import pallas as pl
from jax.experimental.pallas import tpu as pltpu

D, S, F = 576, 2048, 4608
DF = D // 2 + 1
NT = S // 128
NRB = 37
EPS = 1e-5
HB, SB = D // 4, S // 4
CHUNKS = (1024, 1536, 2048)
STARTS = tuple(sum(CHUNKS[:j]) for j in range(len(CHUNKS)))
MOD_PARTS = ((0, 9), (9, 27))

f32, bf16, u32 = jnp.float32, jnp.bfloat16, jnp.uint32

_Q = np.sqrt(3.0) / 2
_C1, _C2, _C4 = (float(np.cos(2 * np.pi * k / 9)) for k in (1, 2, 4))
_S1, _S2, _S4 = (float(np.sin(2 * np.pi * k / 9) / _Q) for k in (1, 2, 4))


def _row_runs():
    runs = []
    for g in (1, 2, 3, 4):
        for r in (g, 9 - g):
            runs += [r, r + 9]
    return runs + [0, 9]


def _pack_rows(m):
    b = m.astype(np.float32).astype(jnp.bfloat16).view(np.uint16).astype(np.uint32)
    return b[..., 0::2, :] | (b[..., 1::2, :] << np.uint32(16))


def _channel_mats():
    kd_all = [k0 + 18 * j for k0 in _row_runs() for j in range(16)] + [D // 2] + [-1] * 7
    kd_all = np.array(kd_all)
    b = np.arange(64)
    mats = np.zeros((10, 128, 128))
    for g in (1, 2, 3, 4):
        kd = kd_all[64 * (g - 1):64 * g]
        sg = np.where(kd % 9 == g, -1.0, 1.0).reshape(8, 8, 1, 1)
        th = (2 * np.pi / D) * ((kd[:, None] * b[None, :]) % D)
        c, s = np.cos(th).reshape(8, 8, 8, 8), np.sin(th).reshape(8, 8, 8, 8)
        m = np.zeros((8, 2, 8, 8, 2, 8))
        m[:, 0, :, :, 0, :] = c
        m[:, 0, :, :, 1, :] = sg * _Q * s
        m[:, 1, :, :, 0, :] = -s
        m[:, 1, :, :, 1, :] = sg * _Q * c
        mats[g - 1] = m.reshape(128, 128)
        mats[5 + g - 1] = m.reshape(128, 128).T
    kd = kd_all[256:]
    valid = (kd >= 0)[:, None]
    th = (2 * np.pi / D) * ((kd[:, None] * b[None, :]) % D)
    m = np.zeros((5, 2, 8, 64))
    m[:, 0] = (np.cos(th) * valid).reshape(5, 8, 64)
    m[:, 1] = (-np.sin(th) * valid * (kd != D // 2)[:, None]).reshape(5, 8, 64)
    half = np.where((kd == 0) | (kd == D // 2), 0.5, 1.0).reshape(5, 1, 8, 1)
    mats[4, :80, :64] = m.reshape(80, 64)
    mats[9, :64, :80] = (m * half).reshape(80, 64).T
    return _pack_rows(mats)


def _token_tables():
    l = np.arange(128)
    ones = np.ones((8, 1))
    angles = [(2 * np.pi / 128) * ((l[:8, None] * l[None, :]) % 128),
              (2 * np.pi / 128) * ((8 * l) % 128) * ones, (2 * np.pi / S) * l * ones]
    return np.concatenate([p for a in angles for p in (np.cos(a), -np.sin(a))]).astype(np.float32)


_CH_MATS = _channel_mats()
_TOK_TAB = _token_tables()


def _dot(a, b):
    return jnp.dot(a, b, preferred_element_type=f32)


def _radix9(x):
    s1, s2, s3, s4 = x[1] + x[8], x[2] + x[7], x[3] + x[6], x[4] + x[5]
    d1, d2, d3, d4 = x[1] - x[8], x[2] - x[7], x[3] - x[6], x[4] - x[5]
    p = x[0] - 0.5 * s3
    a, b = s1 - s4, s2 - s4
    r1 = _C1 * a + _C2 * b
    r2 = _C2 * a + _C4 * b
    e, g = d1 + d2, d2 + d4
    i1 = _S1 * e + _S4 * g
    i2 = _S2 * e - _S1 * g
    t, u = s1 + s2 + s4, x[0] + s3
    return u + t, [(p + r1, i1 + d3), (p + r2, i2 - d3),
                   (u - 0.5 * t, d1 - d2 + d4), ((p - r1) - r2, (i2 - i1) + d3)]


def _radix9_t(x0, uv):
    (u1, v1), (u2, v2), (u3, v3), (u4, v4) = uv
    u, t = x0 + u3, x0 - 0.5 * u3
    p, r1, r2 = u1 + u2 + u4, u1 - u4, u2 - u4
    a = _C1 * r1 + _C2 * r2
    b = _C2 * r1 + _C4 * r2
    s1, s2, s3, s4 = t + a, t + b, u - 0.5 * p, (t - a) - b
    i1, i2, d3 = v1 - v4, v2 + v4, v1 - v2 + v4
    e = _S1 * i1 + _S2 * i2
    g = _S4 * i1 - _S1 * i2
    d1, d2, d4 = e + v3, (e + g) - v3, g + v3
    return [u + p, s1 + d1, s2 + d2, s3 + d3, s4 + d4, s4 - d4, s3 - d3, s2 - d2, s1 - d1]


def _cadd(a, b):
    return a[0] + b[0], a[1] + b[1]


def _csub(a, b):
    return a[0] - b[0], a[1] - b[1]


def _cmul(a, b):
    return a[0] * b[0] - a[1] * b[1], a[0] * b[1] + a[1] * b[0]


def _cross(a, b):
    return (a[0] - b[1], a[1] + b[0]), (a[0] + b[1], a[1] - b[0])


def _radix4(x, sign):
    a, b, c, d = x
    u, v = _cadd(a, c), _cadd(b, d)
    k1, k3 = _cross(_csub(a, c), _csub(b, d))[::sign]
    return [_cadd(u, v), k1, _csub(u, v), k3]


def _twiddle16(z, e, sign):
    re, im = z
    if e == 0:
        return z
    c, s = float(np.cos(2 * np.pi * e / 16)), float(sign * np.sin(2 * np.pi * e / 16))
    if e == 4:
        return (-im, re) if sign > 0 else (im, -re)
    if e % 2 == 0:
        if c * s > 0:
            return c * (re - im), c * (re + im)
        return c * (re + im), c * (im - re)
    return c * re - s * im, s * re + c * im


def _halves(w):
    return pltpu.bitcast(w, bf16)


def _pair(a, b):
    return jnp.concatenate([a, b], axis=0).astype(bf16)


class _RowMean:
    def __init__(self, lanes=2):
        self.acc, self.n = [None] * lanes, 0

    def add(self, v):
        i = self.n % len(self.acc)
        self.acc[i] = v if self.acc[i] is None else self.acc[i] + v
        self.n += 1

    def mean(self):
        acc = self.acc
        while len(acc) > 1:
            acc = [acc[i] + acc[i + 1] for i in range(0, len(acc), 2)]
        return jnp.sum(acc[0], axis=0, keepdims=True) * (1.0 / D)


def _gelu(x):
    inner = x * (0.7978845608028654 + (0.7978845608028654 * 0.044715) * (x * x))
    hx = 0.5 * x
    return hx + hx * jnp.tanh(inner)


_LEFT = (((0, 0), 1, (1, 1)), ((1, 0), 1, (1, 1)), ((0, 0), 0, None), ((1, 1), 0, None),
         ((0, 0), 1, (0, 1)), ((1, 0), -1, (0, 0)), ((0, 1), -1, (1, 1)))
_RIGHT = (((0, 0), 1, (1, 1)), ((0, 0), 0, None), ((0, 1), -1, (1, 1)), ((1, 0), -1, (0, 0)),
          ((1, 1), 0, None), ((0, 0), 1, (0, 1)), ((1, 0), 1, (1, 1)))


def _signed_sum(term, quad):
    a, sign, b = term
    if sign == 0:
        return quad(*a)
    return quad(*a) + quad(*b) if sign > 0 else quad(*a) - quad(*b)


def _operands(table, block, order=range(7)):
    for i in order:
        outer = table[i]
        if outer[1]:
            sums = {(u, v): _signed_sum(outer, lambda r, c: block(i, 2 * r + u, 2 * c + v))
                    for u in range(2) for v in range(2)}
        for j, inner in enumerate(table):
            def quad(u, v):
                if outer[1]:
                    return sums[u, v]
                return block(7 * i + j, 2 * outer[0][0] + u, 2 * outer[0][1] + v)
            yield _signed_sum(inner, quad).astype(bf16)


_RESULT = {(0, 0): {0: 1, 3: 1, 4: -1, 6: 1}, (0, 1): {2: 1, 4: 1},
           (1, 0): {1: 1, 3: 1}, (1, 1): {0: 1, 1: -1, 2: 1, 5: 1}}


def _completed(i, have):
    for quadrant, terms in _RESULT.items():
        if i in terms and all(j in have for j in terms):
            first, *rest = terms
            x = have[first]
            for j in rest:
                x = x + have[j] if terms[j] > 0 else x - have[j]
            yield quadrant, x


def _blocks(products, order=range(7)):
    outer = {quadrant: {} for quadrant in _RESULT}
    for i in order:
        inner = {}
        for j in range(7):
            inner[j] = next(products)
            for (u, v), x in _completed(j, inner):
                outer[u, v][i] = x
                for (r, c), y in _completed(i, outer[u, v]):
                    yield (2 * r + u, 2 * c + v), y


def _kernel(x_hbm, wr_hbm, wi_hbm, w1_hbm, b1_hbm, w2_hbm, b2_hbm, c_hbm, wm_hbm, chm_hbm, tok_hbm,
            o_hbm,
            x_v, wr_v, wi_v, w1_v, b1_v, w2_v, b2_v, c_v, wm_v, chm_v, tok_v,
            mod_v, mf_v, mi_v, wt_v, wp_v, r_v, fa_v, fc_v, x1_v, a_v, acc_v, o_v, st_v,
            sem):
    def batch(slot, pairs):
        return [pltpu.make_async_copy(src, dst, sem.at[slot]) for src, dst in pairs]

    def start(copies):
        for c in copies:
            c.start()

    def wait(copies):
        for c in copies:
            c.wait()

    def cols(lo, n, *refs):
        return tuple(ref.at[:, pl.ds(lo, n)] for ref in refs)

    def mod_cols(part):
        lo, hi = MOD_PARTS[part]
        return cols(128 * lo, 128 * (hi - lo), wm_hbm, wm_v)

    def chm_half(i):
        return chm_hbm.at[pl.ds(5 * i, 5)], chm_v.at[pl.ds(5 * i, 5)]

    def w1_tiles(j):
        first = STARTS[j] // 128
        return [(*cols(128 * t, 128, w1_hbm), w1_v.at[t])
                for t in range(first, first + CHUNKS[j] // 128)]

    def w2_tiles(j):
        rows = pl.ds(STARTS[j], CHUNKS[j])
        return [(w2_hbm.at[rows, pl.ds(128 * t, 128)], w2_v.at[t, rows]) for t in range(NT)]

    def cp_x(i):
        lo = i * 256 if isinstance(i, int) else pl.multiple_of(i * 256, 256)
        return batch(i, [cols(lo, 256, x_hbm, x_v)])

    cp_tables = batch(8, [(tok_hbm, tok_v), (c_hbm, c_v)])
    cp_mod = batch(9, [mod_cols(0)])
    cp_forward = batch(10, [chm_half(0)])
    cp_filter = batch(11, [(wr_hbm, wr_v), (wi_hbm, wi_v)])
    cp_inverse = batch(12, [chm_half(1), mod_cols(1)])
    cp_mlp = [batch(13, [(b1_hbm, b1_v), (b2_hbm, b2_v), *w1_tiles(0)]),
              batch(0, w1_tiles(1)),
              batch(8, w2_tiles(0) + w1_tiles(2)),
              batch(9, w2_tiles(1)), batch(10, w2_tiles(2))]
    sem_o = sem.at[11]

    for copies in (cp_tables, cp_x(0), cp_x(1), cp_mod, *map(cp_x, range(2, NT // 2)),
                   cp_forward, cp_filter, cp_inverse, cp_mlp[0]):
        start(copies)

    def lanes(t):
        if isinstance(t, int):
            return slice(128 * t, 128 * (t + 1))
        return pl.ds(pl.multiple_of(t * 128, 128), 128)

    def blk(i):
        return slice(8 * i, 8 * i + 8)

    with jax.named_scope("gen"):
        wait(cp_tables)
        rows = [(tok_v[blk(0), :], tok_v[blk(1), :])]
        for _ in range(15):
            rows.append(_cmul(rows[-1], (tok_v[blk(2), :], tok_v[blk(3), :])))
        dft = tuple(jnp.concatenate([r[i] for r in rows], axis=0) for i in range(2))
        along = tuple(jnp.concatenate([tok_v[blk(i), :]] * 16, axis=0) for i in (4, 5))
        down = tuple(a.T for a in along)

        def gen(k, carry):
            for ref, (re, im), order in zip((mf_v, mi_v), carry, ((1, 2), (2, 1))):
                for i, m in zip((0, *order), (re, re + im, re - im)):
                    ref[k, i] = m.astype(bf16)
            return _cmul(carry[0], down), _cmul(carry[1], along)

        lax.fori_loop(0, NT, gen, (dft, dft))

    cf = c_v[...].astype(f32)
    sc = jnp.broadcast_to(cf * jax.nn.sigmoid(cf), (16, D)).astype(bf16)

    def store_mod(j):
        row = _dot(sc, wm_v[:, lanes(j)])[0:8, :]
        n = 128 * j + lax.broadcasted_iota(jnp.int32, row.shape, 1)
        scale = jnp.logical_or(jnp.logical_and(n >= D, n < 2 * D),
                               jnp.logical_and(n >= 4 * D, n < 5 * D))
        row = jnp.where(scale, row + 1.0, row)
        row = jnp.where(jnp.logical_and(n >= 2 * D, n < 3 * D), row * (2.0 / (S * D)), row)
        mod_v[lanes(j), :] = jnp.concatenate([row] * 16, axis=0).T

    def mod(i, b=None):
        return mod_v[i * D:(i + 1) * D, :] if b is None else mod_v[blk(i * D // 8 + b), :]

    def first_mod():
        wait(cp_mod)
        for j in range(*MOD_PARTS[0]):
            store_mod(j)

    def stage(pair, slot, values, finish=lambda m: m):
        means = [_RowMean() for _ in pair]
        for vs in zip(*map(values, pair)):
            for m, v in zip(means, vs):
                m.add(v)
            yield
        for t, m in zip(pair, means):
            st_v[slot, t] = jnp.broadcast_to(finish(m.mean()), (8, 128))

    def in_turn(gens):
        for g, _ in gens:
            for _ in g:
                pass

    def in_step(gens):
        n = D // 8
        for q in range(n):
            for g, cuts in gens:
                for _ in range(cuts * q // n, cuts * (q + 1) // n):
                    next(g)
        in_turn(gens)

    def skewed(stages, emit, n, after_fill=lambda: None):
        depth = len(stages) - 1

        def step(oldest, lo, hi):
            emit([(fn(oldest + (depth - lag)), cuts)
                  for lag, cuts, fn in stages if lo <= lag <= hi])

        for i in range(depth):
            step(i - depth, 0, i)
        after_fill()
        lax.fori_loop(0, n - depth, lambda i, _: step(i, 0, depth), None)
        for i in range(n, n + depth):
            step(i - depth, i - n + 1, depth)

    def inv_std(var):
        return lax.rsqrt(var + EPS)

    def squares(src, slot, dst=None):
        def values(t):
            mean = st_v[slot, t]
            for b in range(D // 8):
                c = src[t, blk(b), :] - mean
                if dst is not None:
                    dst[t, blk(b), :] = c
                yield c * c
        return values

    def adjacent(i):
        return 2 * i, 2 * i + 1

    def tokens(t):
        for i in range(D // 16):
            x = x_v[16 * i:16 * i + 16, lanes(t)].astype(f32)
            for b, half in enumerate((x[:8], x[8:]), 2 * i):
                x1_v[t, blk(b), :] = half
                yield half

    def load_tokens(i):
        wait(cp_x(i))
        return stage(adjacent(i), 0, tokens)

    def fwd_butterflies(i):
        for t in adjacent(i):
            rstd = st_v[1, t]
            for p in range(8):
                x0, uv = _radix9([fc_v[t, blk(b), :] * rstd * mod(1, b) + mod(0, b)
                                  for b in range(p, D // 8, 8)])
                for g in range(4):
                    r_v[t, 128 * g + 16 * p:128 * g + 16 * p + 16, :] = _pair(*uv[g])
                if p % 2:
                    r_v[t, 504 + 8 * p:520 + 8 * p, :] = _pair(prev, x0)
                prev = x0
                yield

    with jax.named_scope("A"):
        skewed([(1, D // 8, lambda i: stage(adjacent(i), 1, squares(x1_v, 0, fc_v), inv_std)),
                (0, D // 8, load_tokens), (2, 16, fwd_butterflies)],
               in_step, NT // 2, first_mod)

    def filt_a(t):
        a = pltpu.bitcast(wr_v[0:DF - 1, lanes(t)], u32)
        b = pltpu.bitcast(wi_v[0:DF - 1, lanes(t)], u32)
        nr = wr_v[DF - 1:DF, lanes(t)].astype(f32)
        ni = wi_v[DF - 1:DF, lanes(t)].astype(f32)
        r = lax.broadcasted_iota(jnp.int32, (8, 128), 0)
        nyq = pltpu.bitcast(jnp.where(r == 0, nr, jnp.where(r == 1, ni, 0.0)), u32)
        rest = jnp.concatenate([a[128:], b[128:], nyq, jnp.zeros((88, 128), u32)], axis=0)
        for c, tile in enumerate((a[:128].T, b[:128].T, rest.T)):
            for j in range(8):
                lo = (NT + 1) * (8 * t + j)
                wt_v[c, lo:lo + NT, :] = tile[NT * j:NT * (j + 1)]

    def filt_b(k):
        wp_v[k, 0:128, :] = wt_v[0, pl.ds(k, 128, stride=NT + 1), :].T
        wp_v[k, 144:272, :] = wt_v[1, pl.ds(k, 128, stride=NT + 1), :].T
        rest = wt_v[2, pl.ds(k, 128, stride=NT + 1), :].T
        wp_v[k, 128:144, :] = rest[0:16]
        wp_v[k, 272:296, :] = rest[16:40]

    def filt(k, rb, base, nyq_row):
        if rb == NRB - 1:
            w = jnp.broadcast_to(wp_v[k, nyq_row:nyq_row + 1, :], (8, 128))
        else:
            k0 = _row_runs()[rb // 2]
            w = wp_v[k, pl.ds(base + k0 // 2 + 72 * (rb % 2), 8, stride=9), :]
            w = (w & np.uint32(0xFFFF0000)) if k0 % 2 else (w << 16)
        return pltpu.bitcast(w, f32)

    groups = [range(8 * g, min(8 * g + 8, NRB)) for g in range(5)]
    rounds = [(q, odd) for q in range(4) for odd in (0, 1)]

    def harmonics(q, odd):
        return q + 4 * odd, q + 4 * odd + 8

    def get(ref, i, rb):
        return ref[i, blk(2 * rb), :], ref[i, blk(2 * rb + 1), :]

    def put(ref, i, rb, z):
        ref[i, blk(2 * rb), :], ref[i, blk(2 * rb + 1), :] = z

    def token_dft(z, m_ref, k):
        def times(parts, i):
            lhs = jnp.concatenate([*parts, jnp.zeros((8, 128), f32)], axis=0).astype(bf16)
            return _dot(lhs, m_ref[k, i])
        s = times([re + im for re, im in z], 0)
        a, b = times([im for _, im in z], 1), times([re for re, _ in z], 2)
        return [(s[blk(rb)] - a[blk(rb)], s[blk(rb)] - b[blk(rb)]) for rb in range(NRB)]

    def fwd_channel(g, t0):
        tiles = range(t0, NT, 4)
        if g < 4:
            outs = [_dot(_halves(chm_v[g]), r_v[t, lanes(g), :]) for t in tiles]
        else:
            pad = jnp.zeros((64, 128), bf16)
            outs = [_dot(_halves(chm_v[4, 0:40, :]),
                         jnp.concatenate([r_v[t, 512:576, :], pad], axis=0)) for t in tiles]
        for i, rb in enumerate(groups[g]):
            y = _radix4([(o[blk(2 * i)], o[blk(2 * i + 1)]) for o in outs], -1)
            for q in range(4):
                put(fa_v, 4 * q + t0, rb, _twiddle16(y[q], t0 * q, -1))

    def fwd_token(q, odd):
        z = []
        for rb in range(NRB):
            a, b, c, d = (get(fa_v, 4 * q + t0, rb) for t0 in range(4))
            if odd:
                z.append(_cross(_csub(a, c), _csub(b, d))[::-1])
            else:
                u, v = _cadd(a, c), _cadd(b, d)
                z.append((_cadd(u, v), _csub(u, v)))
        for k, zk in zip(harmonics(q, odd), zip(*z)):
            for rb, y in enumerate(token_dft(zk, mf_v, k)):
                put(fc_v, k, rb, y)

    def inv_token(q, odd):
        outs = []
        for k in harmonics(q, odd):
            z = [_cmul(get(fc_v, k, rb), (filt(k, rb, 0, 288), filt(k, rb, 144, 289)))
                 for rb in range(NRB)]
            outs.append(token_dft(z, mi_v, k))
        for rb, (a, c) in enumerate(zip(*outs)):
            u, v = _cadd(a, c), _csub(a, c)
            if odd:
                p, m = get(fa_v, q, rb), get(fa_v, 4 + q, rb)
                y1, y3 = _cross(m, v)
                for t0, y in enumerate((_cadd(p, u), y1, _csub(p, u), y3)):
                    put(fa_v, 4 * t0 + q, rb, _twiddle16(y, t0 * q, +1))
            else:
                put(fa_v, q, rb, u)
                put(fa_v, 4 + q, rb, v)

    def inv_channel(g, t0):
        z = [_radix4([get(fa_v, 4 * t0 + q, rb) for q in range(4)], +1) for rb in groups[g]]
        for t, zt in zip(range(t0, NT, 4), zip(*z)):
            parts = [v for pair in zt for v in pair]
            if g < 4:
                fc_v[t, lanes(g), :] = _dot(_halves(chm_v[5 + g]),
                                            jnp.concatenate(parts, axis=0).astype(bf16))
            else:
                parts.append(jnp.zeros((48, 128), f32))
                fc_v[t, 512:576, :] = _dot(_halves(chm_v[9, 0:32, :]),
                                           jnp.concatenate(parts, axis=0).astype(bf16))

    with jax.named_scope("F"):
        start(cp_mlp[1])
        wait(cp_forward)
        for g in range(5):
            for t0 in range(4):
                fwd_channel(g, t0)
        for i, r in enumerate(rounds):
            if i == 2:
                wait(cp_filter)
            fwd_token(*r)
            if 2 <= i < 6:
                for t in range(4 * i - 8, 4 * i - 4):
                    filt_a(t)
            elif i >= 6:
                for k in harmonics(*rounds[i - 6]):
                    filt_b(k)
    with jax.named_scope("I"):
        for i, r in enumerate(rounds):
            if i < 6:
                for k in harmonics(*rounds[i + 2]):
                    filt_b(k)
            inv_token(*r)
        wait(cp_inverse)
        lo, hi = MOD_PARTS[1]
        for i in range(20):
            inv_channel(*divmod(i, 4))
            if lo + i < hi:
                store_mod(lo + i)

    def opposite(j):
        return j, j + NT // 2

    def residual(t):
        for p in range(8):
            uv = [(fc_v[t, blk(16 * g + 2 * p), :], fc_v[t, blk(16 * g + 2 * p + 1), :])
                  for g in range(4)]
            for a, y in enumerate(_radix9_t(fc_v[t, blk(64 + p), :], uv)):
                b = 8 * a + p
                x1 = x1_v[t, blk(b), :] + mod(2, b) * y
                x1_v[t, blk(b), :] = x1
                yield x1

    def modulated(t):
        rstd = st_v[1, t]
        for b in range(D // 8):
            h = fa_v[t, blk(b), :] * rstd * mod(4, b) + mod(3, b)
            fc_v[t, blk(b), :] = h
            yield h

    def mlp_operands(j, _):
        stats = [(j + 4 * c, st_v[2, j + 4 * c], st_v[3, j + 4 * c]) for c in range(4)]
        for r0 in range(0, HB, 16):
            h = {(r, c): jnp.concatenate([(fc_v[t, q:q + 8, :] - mean) * rstd
                                          for q in (HB * r + r0, HB * r + r0 + 8)], axis=0)
                 for r in range(4) for c, (t, mean, rstd) in enumerate(stats)}
            for i, a in enumerate(_operands(_LEFT, lambda _, r, c: h[r, c])):
                a_v[i, j, r0:r0 + 16, :] = a

    with jax.named_scope("C"):
        skewed([(1, D // 8, lambda j: stage(opposite(j), 1, squares(x1_v, 0, fa_v), inv_std)),
                (0, D // 8, lambda j: stage(opposite(j), 0, residual))], in_turn, NT // 2)
        skewed([(1, D // 8, lambda j: stage(opposite(j), 3, squares(fc_v, 2), inv_std)),
                (0, D // 8, lambda j: stage(opposite(j), 2, modulated))], in_turn, NT // 2)
        lax.fori_loop(0, 4, mlp_operands, None)

    zero = pl.program_id(0)
    a_words = a_v.bitcast(u32)

    def weights(ref, top, height, left, stride, width, order=range(7)):
        def block(i, r, c):
            rows = pl.ds(pl.multiple_of((top + r * height) // 2 + 8 * i * zero, 8), height // 2)
            first = (left + c * stride) // 128
            words = [ref.bitcast(u32)[t, rows, :] for t in range(first, first + width // 128)]
            return _halves(jnp.concatenate(words, axis=1)).astype(f32)
        return _operands(_RIGHT, block, order)

    def hidden(j):
        lo, n = STARTS[j], CHUNKS[j] // 4
        bias = [jnp.concatenate([b1[t:t + 1, :] for t in range((lo + c * n) // 128,
                                                               (lo + c * n + n) // 128)], axis=1)
                for c in range(4)]
        return {(r, c): _gelu(x + bias[c]) for (r, c), x in _blocks(
            _dot(_halves(jnp.concatenate([a_words[i, t] for t in range(4)], axis=1)), w)
            for i, w in enumerate(weights(w1_v, 0, SB, lo, n, n)))}

    def products(j, g):
        for a, w in zip(_operands(_LEFT, lambda _, r, c: g[r, c]),
                        weights(w2_v, STARTS[j], CHUNKS[j] // 4, 0, SB, SB)):
            yield _dot(a, w)

    with jax.named_scope("MLP"):
        wait(cp_mlp[0])
        start(cp_mlp[2])
        b1, b2 = b1_v[...].astype(f32), b2_v[...].astype(f32)
        g0 = hidden(0)
        wait(cp_mlp[1])
        start(cp_mlp[3])
        g1 = hidden(1)
        wait(cp_mlp[2])
        start(cp_mlp[4])
        for i, m in enumerate(products(0, g0)):
            acc_v[i] = m
        g2 = hidden(2)
        wait(cp_mlp[3] + cp_mlp[4])
        for i, m in enumerate(products(1, g1)):
            acc_v[i] += m

        def finish(r, c, y):
            rows = slice(HB * r, HB * (r + 1))
            for j in range(4):
                t = 4 * c + j
                yt = y[:, lanes(j)] + b2[t:t + 1, :]
                o_v[t, rows, :] = (x1_v[t, rows, :] + mod_v[5 * D + HB * r:5 * D + HB * (r + 1), :]
                                   * yt).astype(bf16)
                pltpu.make_async_copy(
                    o_v.at[t, rows], o_hbm.at[rows, lanes(t)], sem_o).start()

        for (r, c), y in _blocks((acc_v[i] + m for i, m in enumerate(products(2, g2)))):
            finish(r, c, y)
        pltpu.make_async_copy(o_hbm, o_hbm, sem_o).wait()


@jax.jit
def pallas_adaLN_cond__spectral_gfnet__mixer_token_mlp__prompt_kernel(
    A_x: jax.Array,
    A_w_r: jax.Array,
    A_w_i: jax.Array,
    B_x: jax.Array,
    B_w1: jax.Array,
    B_b1: jax.Array,
    B_w2: jax.Array,
    B_b2: jax.Array,
    c: jax.Array,
    w_mod: jax.Array,
):
    del B_x
    vmem = pltpu.VMEM
    scratch = [
        vmem((D, S), bf16), vmem((DF, S), bf16), vmem((DF, S), bf16),
        vmem((F // 128, S, 128), bf16), vmem((F // 128, 128), bf16),
        vmem((NT, F, 128), bf16), vmem((S // 128, 128), bf16),
        vmem((1, D), bf16), vmem((D, 6 * D), bf16),
        vmem(_CH_MATS.shape, u32), vmem(_TOK_TAB.shape, f32),
        vmem((6 * D, 128), f32),
        vmem((NT, 3, 128, 128), bf16),
        vmem((NT, 3, 128, 128), bf16),
        vmem((3, S + 128, 128), u32),
        vmem((NT, 296, 128), u32),
        vmem((NT, D, 128), bf16),
        vmem((NT, NRB * 16, 128), f32),
        vmem((NT, NRB * 16, 128), f32),
        vmem((NT, D, 128), f32),
        vmem((49, 4, HB, 128), bf16),
        vmem((49, HB, SB), f32),
        vmem((NT, D, 128), bf16),
        vmem((4, NT, 8, 128), f32),
        pltpu.SemaphoreType.DMA((14,)),
    ]
    out = pl.pallas_call(
        _kernel,
        grid=(1,),
        in_specs=[pl.BlockSpec(memory_space=pl.ANY)] * 11,
        out_specs=pl.BlockSpec(memory_space=pl.ANY),
        out_shape=jax.ShapeDtypeStruct((D, S), bf16),
        scratch_shapes=scratch,
        compiler_params=pltpu.CompilerParams(vmem_limit_bytes=124 * 1024 * 1024),
    )(A_x.reshape(S, D).T, A_w_r.T, A_w_i.T, B_w1, B_b1.reshape(F // 128, 128), B_w2,
      B_b2.reshape(S // 128, 128), c, w_mod, _CH_MATS, _TOK_TAB)
    return out.T.reshape(1, S, D)
```

```python
import jax
import jax.numpy as jnp
import numpy as np
from jax import lax
from jax.experimental import pallas as pl
from jax.experimental.pallas import tpu as pltpu

D, S, F = 576, 2048, 4608
DF = D // 2 + 1
NT = S // 128
NRB = 37
EPS = 1e-5
HB, SB = D // 4, S // 4
CHUNKS = (1024, 1536, 2048)
STARTS = tuple(sum(CHUNKS[:j]) for j in range(len(CHUNKS)))
MOD_PARTS = ((0, 9), (9, 27))

f32, bf16, u32 = jnp.float32, jnp.bfloat16, jnp.uint32

_Q = np.sqrt(3.0) / 2
_C1, _C2, _C4 = (float(np.cos(2 * np.pi * k / 9)) for k in (1, 2, 4))
_S1, _S2, _S4 = (float(np.sin(2 * np.pi * k / 9) / _Q) for k in (1, 2, 4))


def _row_runs():
    runs = []
    for g in (1, 2, 3, 4):
        for r in (g, 9 - g):
            runs += [r, r + 9]
    return runs + [0, 9]


def _pack_rows(m):
    b = m.astype(np.float32).astype(jnp.bfloat16).view(np.uint16).astype(np.uint32)
    return b[..., 0::2, :] | (b[..., 1::2, :] << np.uint32(16))


def _channel_mats():
    kd_all = [k0 + 18 * j for k0 in _row_runs() for j in range(16)] + [D // 2] + [-1] * 7
    kd_all = np.array(kd_all)
    b = np.arange(64)
    mats = np.zeros((10, 128, 128))
    for g in (1, 2, 3, 4):
        kd = kd_all[64 * (g - 1):64 * g]
        sg = np.where(kd % 9 == g, -1.0, 1.0).reshape(8, 8, 1, 1)
        th = (2 * np.pi / D) * ((kd[:, None] * b[None, :]) % D)
        c, s = np.cos(th).reshape(8, 8, 8, 8), np.sin(th).reshape(8, 8, 8, 8)
        m = np.zeros((8, 2, 8, 8, 2, 8))
        m[:, 0, :, :, 0, :] = c
        m[:, 0, :, :, 1, :] = sg * _Q * s
        m[:, 1, :, :, 0, :] = -s
        m[:, 1, :, :, 1, :] = sg * _Q * c
        mats[g - 1] = m.reshape(128, 128)
        mats[5 + g - 1] = m.reshape(128, 128).T
    kd = kd_all[256:]
    valid = (kd >= 0)[:, None]
    th = (2 * np.pi / D) * ((kd[:, None] * b[None, :]) % D)
    m = np.zeros((5, 2, 8, 64))
    m[:, 0] = (np.cos(th) * valid).reshape(5, 8, 64)
    m[:, 1] = (-np.sin(th) * valid * (kd != D // 2)[:, None]).reshape(5, 8, 64)
    half = np.where((kd == 0) | (kd == D // 2), 0.5, 1.0).reshape(5, 1, 8, 1)
    mats[4, :80, :64] = m.reshape(80, 64)
    mats[9, :64, :80] = (m * half).reshape(80, 64).T
    return _pack_rows(mats)


def _token_tables():
    l = np.arange(128)
    ones = np.ones((8, 1))
    angles = [(2 * np.pi / 128) * ((l[:8, None] * l[None, :]) % 128),
              (2 * np.pi / 128) * ((8 * l) % 128) * ones, (2 * np.pi / S) * l * ones]
    return np.concatenate([p for a in angles for p in (np.cos(a), -np.sin(a))]).astype(np.float32)


_CH_MATS = _channel_mats()
_TOK_TAB = _token_tables()


def _dot(a, b):
    return jnp.dot(a, b, preferred_element_type=f32)


def _radix9(x):
    s1, s2, s3, s4 = x[1] + x[8], x[2] + x[7], x[3] + x[6], x[4] + x[5]
    d1, d2, d3, d4 = x[1] - x[8], x[2] - x[7], x[3] - x[6], x[4] - x[5]
    p = x[0] - 0.5 * s3
    a, b = s1 - s4, s2 - s4
    r1 = _C1 * a + _C2 * b
    r2 = _C2 * a + _C4 * b
    e, g = d1 + d2, d2 + d4
    i1 = _S1 * e + _S4 * g
    i2 = _S2 * e - _S1 * g
    t, u = s1 + s2 + s4, x[0] + s3
    return u + t, [(p + r1, i1 + d3), (p + r2, i2 - d3),
                   (u - 0.5 * t, d1 - d2 + d4), ((p - r1) - r2, (i2 - i1) + d3)]


def _radix9_t(x0, uv):
    (u1, v1), (u2, v2), (u3, v3), (u4, v4) = uv
    u, t = x0 + u3, x0 - 0.5 * u3
    p, r1, r2 = u1 + u2 + u4, u1 - u4, u2 - u4
    a = _C1 * r1 + _C2 * r2
    b = _C2 * r1 + _C4 * r2
    s1, s2, s3, s4 = t + a, t + b, u - 0.5 * p, (t - a) - b
    i1, i2, d3 = v1 - v4, v2 + v4, v1 - v2 + v4
    e = _S1 * i1 + _S2 * i2
    g = _S4 * i1 - _S1 * i2
    d1, d2, d4 = e + v3, (e + g) - v3, g + v3
    return [u + p, s1 + d1, s2 + d2, s3 + d3, s4 + d4, s4 - d4, s3 - d3, s2 - d2, s1 - d1]


def _cadd(a, b):
    return a[0] + b[0], a[1] + b[1]


def _csub(a, b):
    return a[0] - b[0], a[1] - b[1]


def _cmul(a, b):
    return a[0] * b[0] - a[1] * b[1], a[0] * b[1] + a[1] * b[0]


def _cross(a, b):
    return (a[0] - b[1], a[1] + b[0]), (a[0] + b[1], a[1] - b[0])


def _radix4(x, sign):
    a, b, c, d = x
    u, v = _cadd(a, c), _cadd(b, d)
    k1, k3 = _cross(_csub(a, c), _csub(b, d))[::sign]
    return [_cadd(u, v), k1, _csub(u, v), k3]


def _twiddle16(z, e, sign):
    re, im = z
    if e == 0:
        return z
    c, s = float(np.cos(2 * np.pi * e / 16)), float(sign * np.sin(2 * np.pi * e / 16))
    if e == 4:
        return (-im, re) if sign > 0 else (im, -re)
    if e % 2 == 0:
        if c * s > 0:
            return c * (re - im), c * (re + im)
        return c * (re + im), c * (im - re)
    return c * re - s * im, s * re + c * im


def _halves(w):
    return pltpu.bitcast(w, bf16)


def _pair(a, b):
    return jnp.concatenate([a, b], axis=0).astype(bf16)


class _RowMean:
    def __init__(self, lanes=2):
        self.acc, self.n = [None] * lanes, 0

    def add(self, v):
        i = self.n % len(self.acc)
        self.acc[i] = v if self.acc[i] is None else self.acc[i] + v
        self.n += 1

    def mean(self):
        acc = self.acc
        while len(acc) > 1:
            acc = [acc[i] + acc[i + 1] for i in range(0, len(acc), 2)]
        return jnp.sum(acc[0], axis=0, keepdims=True) * (1.0 / D)


def _gelu(x):
    inner = x * (0.7978845608028654 + (0.7978845608028654 * 0.044715) * (x * x))
    hx = 0.5 * x
    return hx + hx * jnp.tanh(inner)


_LEFT = (((0, 0), 1, (1, 1)), ((1, 0), 1, (1, 1)), ((0, 0), 0, None), ((1, 1), 0, None),
         ((0, 0), 1, (0, 1)), ((1, 0), -1, (0, 0)), ((0, 1), -1, (1, 1)))
_RIGHT = (((0, 0), 1, (1, 1)), ((0, 0), 0, None), ((0, 1), -1, (1, 1)), ((1, 0), -1, (0, 0)),
          ((1, 1), 0, None), ((0, 0), 1, (0, 1)), ((1, 0), 1, (1, 1)))


def _signed_sum(term, quad):
    a, sign, b = term
    if sign == 0:
        return quad(*a)
    return quad(*a) + quad(*b) if sign > 0 else quad(*a) - quad(*b)


def _operands(table, block, order=range(7)):
    for i in order:
        outer = table[i]
        if outer[1]:
            sums = {(u, v): _signed_sum(outer, lambda r, c: block(i, 2 * r + u, 2 * c + v))
                    for u in range(2) for v in range(2)}
        for j, inner in enumerate(table):
            def quad(u, v):
                if outer[1]:
                    return sums[u, v]
                return block(7 * i + j, 2 * outer[0][0] + u, 2 * outer[0][1] + v)
            yield _signed_sum(inner, quad).astype(bf16)


_RESULT = {(0, 0): {0: 1, 3: 1, 4: -1, 6: 1}, (0, 1): {2: 1, 4: 1},
           (1, 0): {1: 1, 3: 1}, (1, 1): {0: 1, 1: -1, 2: 1, 5: 1}}


def _completed(i, have):
    for quadrant, terms in _RESULT.items():
        if i in terms and all(j in have for j in terms):
            first, *rest = terms
            x = have[first]
            for j in rest:
                x = x + have[j] if terms[j] > 0 else x - have[j]
            yield quadrant, x


def _blocks(products, order=range(7)):
    outer = {quadrant: {} for quadrant in _RESULT}
    for i in order:
        inner = {}
        for j in range(7):
            inner[j] = next(products)
            for (u, v), x in _completed(j, inner):
                outer[u, v][i] = x
                for (r, c), y in _completed(i, outer[u, v]):
                    yield (2 * r + u, 2 * c + v), y


def _kernel(x_hbm, wr_hbm, wi_hbm, w1_hbm, b1_hbm, w2_hbm, b2_hbm, c_hbm, wm_hbm, chm_hbm, tok_hbm,
            o_hbm,
            x_v, wr_v, wi_v, w1_v, b1_v, w2_v, b2_v, c_v, wm_v, chm_v, tok_v,
            mod_v, mf_v, mi_v, wt_v, wp_v, r_v, fa_v, fc_v, x1_v, a_v, acc_v, o_v, st_v,
            sem):
    def batch(slot, pairs):
        return [pltpu.make_async_copy(src, dst, sem.at[slot]) for src, dst in pairs]

    def start(copies):
        for c in copies:
            c.start()

    def wait(copies):
        for c in copies:
            c.wait()

    def cols(lo, n, *refs):
        return tuple(ref.at[:, pl.ds(lo, n)] for ref in refs)

    def mod_cols(part):
        lo, hi = MOD_PARTS[part]
        return cols(128 * lo, 128 * (hi - lo), wm_hbm, wm_v)

    def chm_half(i):
        return chm_hbm.at[pl.ds(5 * i, 5)], chm_v.at[pl.ds(5 * i, 5)]

    def w1_tiles(j):
        first = STARTS[j] // 128
        return [(*cols(128 * t, 128, w1_hbm), w1_v.at[t])
                for t in range(first, first + CHUNKS[j] // 128)]

    def w2_tiles(j):
        rows = pl.ds(STARTS[j], CHUNKS[j])
        return [(w2_hbm.at[rows, pl.ds(128 * t, 128)], w2_v.at[t, rows]) for t in range(NT)]

    def cp_x(i):
        lo = i * 256 if isinstance(i, int) else pl.multiple_of(i * 256, 256)
        return batch(i, [cols(lo, 256, x_hbm, x_v)])

    cp_tables = batch(8, [(tok_hbm, tok_v), (c_hbm, c_v)])
    cp_mod = batch(9, [mod_cols(0)])
    cp_forward = batch(10, [chm_half(0)])
    cp_filter = batch(11, [(wr_hbm, wr_v), (wi_hbm, wi_v)])
    cp_inverse = batch(12, [chm_half(1), mod_cols(1)])
    cp_mlp = [batch(13, [(b1_hbm, b1_v), (b2_hbm, b2_v), *w1_tiles(0)]),
              batch(0, w1_tiles(1)),
              batch(8, w2_tiles(0) + w1_tiles(2)),
              batch(9, w2_tiles(1)), batch(10, w2_tiles(2))]
    sem_o = sem.at[11]

    for copies in (cp_tables, cp_x(0), cp_x(1), cp_mod, *map(cp_x, range(2, NT // 2)),
                   cp_forward, cp_filter, cp_inverse, cp_mlp[0]):
        start(copies)

    def lanes(t):
        if isinstance(t, int):
            return slice(128 * t, 128 * (t + 1))
        return pl.ds(pl.multiple_of(t * 128, 128), 128)

    def blk(i):
        return slice(8 * i, 8 * i + 8)

    with jax.named_scope("gen"):
        wait(cp_tables)
        rows = [(tok_v[blk(0), :], tok_v[blk(1), :])]
        for _ in range(15):
            rows.append(_cmul(rows[-1], (tok_v[blk(2), :], tok_v[blk(3), :])))
        dft = tuple(jnp.concatenate([r[i] for r in rows], axis=0) for i in range(2))
        along = tuple(jnp.concatenate([tok_v[blk(i), :]] * 16, axis=0) for i in (4, 5))
        down = tuple(a.T for a in along)

        def gen(k, carry):
            for ref, (re, im), order in zip((mf_v, mi_v), carry, ((1, 2), (2, 1))):
                for i, m in zip((0, *order), (re, re + im, re - im)):
                    ref[k, i] = m.astype(bf16)
            return _cmul(carry[0], down), _cmul(carry[1], along)

        lax.fori_loop(0, NT, gen, (dft, dft))

    cf = c_v[...].astype(f32)
    sc = jnp.broadcast_to(cf * jax.nn.sigmoid(cf), (16, D)).astype(bf16)

    def store_mod(j):
        row = _dot(sc, wm_v[:, lanes(j)])[0:8, :]
        n = 128 * j + lax.broadcasted_iota(jnp.int32, row.shape, 1)
        scale = jnp.logical_or(jnp.logical_and(n >= D, n < 2 * D),
                               jnp.logical_and(n >= 4 * D, n < 5 * D))
        row = jnp.where(scale, row + 1.0, row)
        row = jnp.where(jnp.logical_and(n >= 2 * D, n < 3 * D), row * (2.0 / (S * D)), row)
        mod_v[lanes(j), :] = jnp.concatenate([row] * 16, axis=0).T

    def mod(i, b=None):
        return mod_v[i * D:(i + 1) * D, :] if b is None else mod_v[blk(i * D // 8 + b), :]

    def first_mod():
        wait(cp_mod)
        for j in range(*MOD_PARTS[0]):
            store_mod(j)

    def stage(pair, slot, values, finish=lambda m: m):
        means = [_RowMean() for _ in pair]
        for vs in zip(*map(values, pair)):
            for m, v in zip(means, vs):
                m.add(v)
            yield
        for t, m in zip(pair, means):
            st_v[slot, t] = jnp.broadcast_to(finish(m.mean()), (8, 128))

    def in_turn(gens):
        for g, _ in gens:
            for _ in g:
                pass

    def in_step(gens):
        n = D // 8
        for q in range(n):
            for g, cuts in gens:
                for _ in range(cuts * q // n, cuts * (q + 1) // n):
                    next(g)
        in_turn(gens)

    def skewed(stages, emit, n, after_fill=lambda: None):
        depth = len(stages) - 1

        def step(oldest, lo, hi):
            emit([(fn(oldest + (depth - lag)), cuts)
                  for lag, cuts, fn in stages if lo <= lag <= hi])

        for i in range(depth):
            step(i - depth, 0, i)
        after_fill()
        lax.fori_loop(0, n - depth, lambda i, _: step(i, 0, depth), None)
        for i in range(n, n + depth):
            step(i - depth, i - n + 1, depth)

    def inv_std(var):
        return lax.rsqrt(var + EPS)

    def squares(src, slot, dst=None):
        def values(t):
            mean = st_v[slot, t]
            for b in range(D // 8):
                c = src[t, blk(b), :] - mean
                if dst is not None:
                    dst[t, blk(b), :] = c
                yield c * c
        return values

    def adjacent(i):
        return 2 * i, 2 * i + 1

    def tokens(t):
        for i in range(D // 16):
            x = x_v[16 * i:16 * i + 16, lanes(t)].astype(f32)
            for b, half in enumerate((x[:8], x[8:]), 2 * i):
                x1_v[t, blk(b), :] = half
                yield half

    def load_tokens(i):
        wait(cp_x(i))
        return stage(adjacent(i), 0, tokens)

    def fwd_butterflies(i):
        for t in adjacent(i):
            rstd = st_v[1, t]
            for p in range(8):
                x0, uv = _radix9([fc_v[t, blk(b), :] * rstd * mod(1, b) + mod(0, b)
                                  for b in range(p, D // 8, 8)])
                for g in range(4):
                    r_v[t, 128 * g + 16 * p:128 * g + 16 * p + 16, :] = _pair(*uv[g])
                if p % 2:
                    r_v[t, 504 + 8 * p:520 + 8 * p, :] = _pair(prev, x0)
                prev = x0
                yield

    with jax.named_scope("A"):
        skewed([(1, D // 8, lambda i: stage(adjacent(i), 1, squares(x1_v, 0, fc_v), inv_std)),
                (0, D // 8, load_tokens), (2, 16, fwd_butterflies)],
               in_step, NT // 2, first_mod)

    def filt_a(t):
        a = pltpu.bitcast(wr_v[0:DF - 1, lanes(t)], u32)
        b = pltpu.bitcast(wi_v[0:DF - 1, lanes(t)], u32)
        nr = wr_v[DF - 1:DF, lanes(t)].astype(f32)
        ni = wi_v[DF - 1:DF, lanes(t)].astype(f32)
        r = lax.broadcasted_iota(jnp.int32, (8, 128), 0)
        nyq = pltpu.bitcast(jnp.where(r == 0, nr, jnp.where(r == 1, ni, 0.0)), u32)
        rest = jnp.concatenate([a[128:], b[128:], nyq, jnp.zeros((88, 128), u32)], axis=0)
        for c, tile in enumerate((a[:128].T, b[:128].T, rest.T)):
            for j in range(8):
                lo = (NT + 1) * (8 * t + j)
                wt_v[c, lo:lo + NT, :] = tile[NT * j:NT * (j + 1)]

    def filt_b(k):
        wp_v[k, 0:128, :] = wt_v[0, pl.ds(k, 128, stride=NT + 1), :].T
        wp_v[k, 144:272, :] = wt_v[1, pl.ds(k, 128, stride=NT + 1), :].T
        rest = wt_v[2, pl.ds(k, 128, stride=NT + 1), :].T
        wp_v[k, 128:144, :] = rest[0:16]
        wp_v[k, 272:296, :] = rest[16:40]

    def filt(k, rb, base, nyq_row):
        if rb == NRB - 1:
            w = jnp.broadcast_to(wp_v[k, nyq_row:nyq_row + 1, :], (8, 128))
        else:
            k0 = _row_runs()[rb // 2]
            w = wp_v[k, pl.ds(base + k0 // 2 + 72 * (rb % 2), 8, stride=9), :]
            w = (w & np.uint32(0xFFFF0000)) if k0 % 2 else (w << 16)
        return pltpu.bitcast(w, f32)

    groups = [range(8 * g, min(8 * g + 8, NRB)) for g in range(5)]
    rounds = [(q, odd) for q in range(4) for odd in (0, 1)]

    def harmonics(q, odd):
        return q + 4 * odd, q + 4 * odd + 8

    def get(ref, i, rb):
        return ref[i, blk(2 * rb), :], ref[i, blk(2 * rb + 1), :]

    def put(ref, i, rb, z):
        ref[i, blk(2 * rb), :], ref[i, blk(2 * rb + 1), :] = z

    def token_dft(z, m_ref, k):
        def times(parts, i):
            lhs = jnp.concatenate([*parts, jnp.zeros((8, 128), f32)], axis=0).astype(bf16)
            return _dot(lhs, m_ref[k, i])
        s = times([re + im for re, im in z], 0)
        a, b = times([im for _, im in z], 1), times([re for re, _ in z], 2)
        return [(s[blk(rb)] - a[blk(rb)], s[blk(rb)] - b[blk(rb)]) for rb in range(NRB)]

    def fwd_channel(g, t0):
        tiles = range(t0, NT, 4)
        if g < 4:
            outs = [_dot(_halves(chm_v[g]), r_v[t, lanes(g), :]) for t in tiles]
        else:
            pad = jnp.zeros((64, 128), bf16)
            outs = [_dot(_halves(chm_v[4, 0:40, :]),
                         jnp.concatenate([r_v[t, 512:576, :], pad], axis=0)) for t in tiles]
        for i, rb in enumerate(groups[g]):
            y = _radix4([(o[blk(2 * i)], o[blk(2 * i + 1)]) for o in outs], -1)
            for q in range(4):
                put(fa_v, 4 * q + t0, rb, _twiddle16(y[q], t0 * q, -1))

    def fwd_token(q, odd):
        z = []
        for rb in range(NRB):
            a, b, c, d = (get(fa_v, 4 * q + t0, rb) for t0 in range(4))
            if odd:
                z.append(_cross(_csub(a, c), _csub(b, d))[::-1])
            else:
                u, v = _cadd(a, c), _cadd(b, d)
                z.append((_cadd(u, v), _csub(u, v)))
        for k, zk in zip(harmonics(q, odd), zip(*z)):
            for rb, y in enumerate(token_dft(zk, mf_v, k)):
                put(fc_v, k, rb, y)

    def inv_token(q, odd):
        outs = []
        for k in harmonics(q, odd):
            z = [_cmul(get(fc_v, k, rb), (filt(k, rb, 0, 288), filt(k, rb, 144, 289)))
                 for rb in range(NRB)]
            outs.append(token_dft(z, mi_v, k))
        for rb, (a, c) in enumerate(zip(*outs)):
            u, v = _cadd(a, c), _csub(a, c)
            if odd:
                p, m = get(fa_v, q, rb), get(fa_v, 4 + q, rb)
                y1, y3 = _cross(m, v)
                for t0, y in enumerate((_cadd(p, u), y1, _csub(p, u), y3)):
                    put(fa_v, 4 * t0 + q, rb, _twiddle16(y, t0 * q, +1))
            else:
                put(fa_v, q, rb, u)
                put(fa_v, 4 + q, rb, v)

    def inv_channel(g, t0):
        z = [_radix4([get(fa_v, 4 * t0 + q, rb) for q in range(4)], +1) for rb in groups[g]]
        for t, zt in zip(range(t0, NT, 4), zip(*z)):
            parts = [v for pair in zt for v in pair]
            if g < 4:
                fc_v[t, lanes(g), :] = _dot(_halves(chm_v[5 + g]),
                                            jnp.concatenate(parts, axis=0).astype(bf16))
            else:
                parts.append(jnp.zeros((48, 128), f32))
                fc_v[t, 512:576, :] = _dot(_halves(chm_v[9, 0:32, :]),
                                           jnp.concatenate(parts, axis=0).astype(bf16))

    with jax.named_scope("F"):
        start(cp_mlp[1])
        wait(cp_forward)
        for g in range(5):
            for t0 in range(4):
                fwd_channel(g, t0)
        for i, r in enumerate(rounds):
            if i == 2:
                wait(cp_filter)
            fwd_token(*r)
            if 2 <= i < 6:
                for t in range(4 * i - 8, 4 * i - 4):
                    filt_a(t)
            elif i >= 6:
                for k in harmonics(*rounds[i - 6]):
                    filt_b(k)
    with jax.named_scope("I"):
        for i, r in enumerate(rounds):
            if i < 6:
                for k in harmonics(*rounds[i + 2]):
                    filt_b(k)
            inv_token(*r)
        wait(cp_inverse)
        lo, hi = MOD_PARTS[1]
        for i in range(20):
            inv_channel(*divmod(i, 4))
            if lo + i < hi:
                store_mod(lo + i)

    def opposite(j):
        return j, j + NT // 2

    def residual(t):
        for p in range(8):
            uv = [(fc_v[t, blk(16 * g + 2 * p), :], fc_v[t, blk(16 * g + 2 * p + 1), :])
                  for g in range(4)]
            for a, y in enumerate(_radix9_t(fc_v[t, blk(64 + p), :], uv)):
                b = 8 * a + p
                x1 = x1_v[t, blk(b), :] + mod(2, b) * y
                x1_v[t, blk(b), :] = x1
                yield x1

    def modulated(t):
        rstd = st_v[1, t]
        for b in range(D // 8):
            h = fa_v[t, blk(b), :] * rstd * mod(4, b) + mod(3, b)
            fc_v[t, blk(b), :] = h
            yield h

    def mlp_operands(j, _):
        stats = [(j + 4 * c, st_v[2, j + 4 * c], st_v[3, j + 4 * c]) for c in range(4)]
        for r0 in range(0, HB, 16):
            h = {(r, c): jnp.concatenate([(fc_v[t, q:q + 8, :] - mean) * rstd
                                          for q in (HB * r + r0, HB * r + r0 + 8)], axis=0)
                 for r in range(4) for c, (t, mean, rstd) in enumerate(stats)}
            for i, a in enumerate(_operands(_LEFT, lambda _, r, c: h[r, c])):
                a_v[i, j, r0:r0 + 16, :] = a

    with jax.named_scope("C"):
        skewed([(1, D // 8, lambda j: stage(opposite(j), 1, squares(x1_v, 0, fa_v), inv_std)),
                (0, D // 8, lambda j: stage(opposite(j), 0, residual))], in_turn, NT // 2)
        skewed([(1, D // 8, lambda j: stage(opposite(j), 3, squares(fc_v, 2), inv_std)),
                (0, D // 8, lambda j: stage(opposite(j), 2, modulated))], in_turn, NT // 2)
        lax.fori_loop(0, 4, mlp_operands, None)

    zero = pl.program_id(0)

    def weights(ref, top, height, left, stride, width, order=range(7)):
        def block(i, r, c):
            rows = pl.ds(pl.multiple_of(top + r * height + 16 * i * zero, 16), height)
            first = (left + c * stride) // 128
            return jnp.concatenate([ref[t, rows, :].astype(f32)
                                    for t in range(first, first + width // 128)], axis=1)
        return _operands(_RIGHT, block, order)

    def hidden(j):
        lo, n = STARTS[j], CHUNKS[j] // 4
        bias = [jnp.concatenate([b1[t:t + 1, :] for t in range((lo + c * n) // 128,
                                                               (lo + c * n + n) // 128)], axis=1)
                for c in range(4)]
        return {(r, c): _gelu(x + bias[c]) for (r, c), x in _blocks(
            _dot(jnp.concatenate([a_v[i, t] for t in range(4)], axis=1), w)
            for i, w in enumerate(weights(w1_v, 0, SB, lo, n, n)))}

    def products(j, g):
        for a, w in zip(_operands(_LEFT, lambda _, r, c: g[r, c]),
                        weights(w2_v, STARTS[j], CHUNKS[j] // 4, 0, SB, SB)):
            yield _dot(a, w)

    with jax.named_scope("MLP"):
        wait(cp_mlp[0])
        start(cp_mlp[2])
        b1, b2 = b1_v[...].astype(f32), b2_v[...].astype(f32)
        g0 = hidden(0)
        wait(cp_mlp[1])
        start(cp_mlp[3])
        g1 = hidden(1)
        wait(cp_mlp[2])
        start(cp_mlp[4])
        for i, m in enumerate(products(0, g0)):
            acc_v[i] = m
        g2 = hidden(2)
        wait(cp_mlp[3] + cp_mlp[4])
        for i, m in enumerate(products(1, g1)):
            acc_v[i] += m

        def finish(r, c, y):
            rows = slice(HB * r, HB * (r + 1))
            for j in range(4):
                t = 4 * c + j
                yt = y[:, lanes(j)] + b2[t:t + 1, :]
                o_v[t, rows, :] = (x1_v[t, rows, :] + mod_v[5 * D + HB * r:5 * D + HB * (r + 1), :]
                                   * yt).astype(bf16)
                pltpu.make_async_copy(
                    o_v.at[t, rows], o_hbm.at[rows, lanes(t)], sem_o).start()

        for (r, c), y in _blocks((acc_v[i] + m for i, m in enumerate(products(2, g2)))):
            finish(r, c, y)
        pltpu.make_async_copy(o_hbm, o_hbm, sem_o).wait()


@jax.jit
def pallas_adaLN_cond__spectral_gfnet__mixer_token_mlp__prompt_kernel(
    A_x: jax.Array,
    A_w_r: jax.Array,
    A_w_i: jax.Array,
    B_x: jax.Array,
    B_w1: jax.Array,
    B_b1: jax.Array,
    B_w2: jax.Array,
    B_b2: jax.Array,
    c: jax.Array,
    w_mod: jax.Array,
):
    del B_x
    vmem = pltpu.VMEM
    scratch = [
        vmem((D, S), bf16), vmem((DF, S), bf16), vmem((DF, S), bf16),
        vmem((F // 128, S, 128), bf16), vmem((F // 128, 128), bf16),
        vmem((NT, F, 128), bf16), vmem((S // 128, 128), bf16),
        vmem((1, D), bf16), vmem((D, 6 * D), bf16),
        vmem(_CH_MATS.shape, u32), vmem(_TOK_TAB.shape, f32),
        vmem((6 * D, 128), f32),
        vmem((NT, 3, 128, 128), bf16),
        vmem((NT, 3, 128, 128), bf16),
        vmem((3, S + 128, 128), u32),
        vmem((NT, 296, 128), u32),
        vmem((NT, D, 128), bf16),
        vmem((NT, NRB * 16, 128), f32),
        vmem((NT, NRB * 16, 128), f32),
        vmem((NT, D, 128), f32),
        vmem((49, 4, HB, 128), bf16),
        vmem((49, HB, SB), f32),
        vmem((NT, D, 128), bf16),
        vmem((4, NT, 8, 128), f32),
        pltpu.SemaphoreType.DMA((14,)),
    ]
    out = pl.pallas_call(
        _kernel,
        grid=(1,),
        in_specs=[pl.BlockSpec(memory_space=pl.ANY)] * 11,
        out_specs=pl.BlockSpec(memory_space=pl.ANY),
        out_shape=jax.ShapeDtypeStruct((D, S), bf16),
        scratch_shapes=scratch,
        compiler_params=pltpu.CompilerParams(vmem_limit_bytes=124 * 1024 * 1024),
    )(A_x.reshape(S, D).T, A_w_r.T, A_w_i.T, B_w1, B_b1.reshape(F // 128, 128), B_w2,
      B_b2.reshape(S // 128, 128), c, w_mod, _CH_MATS, _TOK_TAB)
    return out.T.reshape(1, S, D)
```

```python
import jax
import jax.numpy as jnp
import numpy as np
from jax import lax
from jax.experimental import pallas as pl
from jax.experimental.pallas import tpu as pltpu

D, S, F = 576, 2048, 4608
DF = D // 2 + 1
NT = S // 128
NB = D // 8
NRB = 37
HB, SB = D // 4, S // 4
CHUNKS = (1024, 1536, 2048)
STARTS = tuple(sum(CHUNKS[:j]) for j in range(len(CHUNKS)))
MOD_PARTS = ((0, 9), (9, 27))
EPS = 1e-5

f32, bf16, u32 = jnp.float32, jnp.bfloat16, jnp.uint32

_Q = np.sqrt(3.0) / 2
_C1, _C2, _C4 = (float(np.cos(2 * np.pi * k / 9)) for k in (1, 2, 4))
_S1, _S2, _S4 = (float(np.sin(2 * np.pi * k / 9) / _Q) for k in (1, 2, 4))

_RUNS = [r + e for g in (1, 2, 3, 4) for r in (g, 9 - g) for e in (0, 9)] + [0, 9]


def _channel_matrices():
    kd_all = np.array([k0 + 18 * j for k0 in _RUNS for j in range(16)] + [D // 2] + [-1] * 7)
    b = np.arange(64)
    mats = np.zeros((10, 128, 128))
    for g in (1, 2, 3, 4):
        kd = kd_all[64 * (g - 1):64 * g]
        sign = np.where(kd % 9 == g, -1.0, 1.0).reshape(8, 8, 1, 1)
        angle = (2 * np.pi / D) * ((kd[:, None] * b[None, :]) % D)
        c, s = np.cos(angle).reshape(8, 8, 8, 8), np.sin(angle).reshape(8, 8, 8, 8)
        m = np.zeros((8, 2, 8, 8, 2, 8))
        m[:, 0, :, :, 0, :] = c
        m[:, 0, :, :, 1, :] = sign * _Q * s
        m[:, 1, :, :, 0, :] = -s
        m[:, 1, :, :, 1, :] = sign * _Q * c
        mats[g - 1] = m.reshape(128, 128)
        mats[g + 4] = m.reshape(128, 128).T
    kd = kd_all[256:]
    valid = (kd >= 0)[:, None]
    angle = (2 * np.pi / D) * ((kd[:, None] * b[None, :]) % D)
    m = np.zeros((5, 2, 8, 64))
    m[:, 0] = (np.cos(angle) * valid).reshape(5, 8, 64)
    m[:, 1] = (-np.sin(angle) * valid * (kd != D // 2)[:, None]).reshape(5, 8, 64)
    half = np.where((kd == 0) | (kd == D // 2), 0.5, 1.0).reshape(5, 1, 8, 1)
    mats[4, :80, :64] = m.reshape(80, 64)
    mats[9, :64, :80] = (m * half).reshape(80, 64).T
    bits = mats.astype(np.float32).astype(jnp.bfloat16).view(np.uint16).astype(np.uint32)
    return bits[:, 0::2, :] | (bits[:, 1::2, :] << np.uint32(16))


def _token_seeds():
    l = np.arange(128)
    ones = np.ones((8, 1))
    angles = [(2 * np.pi / 128) * ((l[:8, None] * l[None, :]) % 128),
              (2 * np.pi / 128) * ((8 * l) % 128) * ones, (2 * np.pi / S) * l * ones]
    return np.concatenate([p for a in angles for p in (np.cos(a), -np.sin(a))]).astype(np.float32)


_CHANNEL_MATRICES = _channel_matrices()
_TOKEN_SEEDS = _token_seeds()


def _dot(a, b):
    return jnp.dot(a, b, preferred_element_type=f32)


def _stack_bf16(parts):
    return jnp.concatenate(parts, axis=0).astype(bf16)


def _radix9(x):
    s1, s2, s3, s4 = x[1] + x[8], x[2] + x[7], x[3] + x[6], x[4] + x[5]
    d1, d2, d3, d4 = x[1] - x[8], x[2] - x[7], x[3] - x[6], x[4] - x[5]
    p = x[0] - 0.5 * s3
    a, b = s1 - s4, s2 - s4
    r1 = _C1 * a + _C2 * b
    r2 = _C2 * a + _C4 * b
    e, g = d1 + d2, d2 + d4
    i1 = _S1 * e + _S4 * g
    i2 = _S2 * e - _S1 * g
    t, u = s1 + s2 + s4, x[0] + s3
    return u + t, [(p + r1, i1 + d3), (p + r2, i2 - d3),
                   (u - 0.5 * t, d1 - d2 + d4), ((p - r1) - r2, (i2 - i1) + d3)]


def _radix9_transposed(x0, uv):
    (u1, v1), (u2, v2), (u3, v3), (u4, v4) = uv
    u, t = x0 + u3, x0 - 0.5 * u3
    p, r1, r2 = u1 + u2 + u4, u1 - u4, u2 - u4
    a = _C1 * r1 + _C2 * r2
    b = _C2 * r1 + _C4 * r2
    s1, s2, s3, s4 = t + a, t + b, u - 0.5 * p, (t - a) - b
    i1, i2, d3 = v1 - v4, v2 + v4, v1 - v2 + v4
    e = _S1 * i1 + _S2 * i2
    g = _S4 * i1 - _S1 * i2
    d1, d2, d4 = e + v3, (e + g) - v3, g + v3
    return [u + p, s1 + d1, s2 + d2, s3 + d3, s4 + d4, s4 - d4, s3 - d3, s2 - d2, s1 - d1]


def _cadd(a, b):
    return a[0] + b[0], a[1] + b[1]


def _csub(a, b):
    return a[0] - b[0], a[1] - b[1]


def _cmul(a, b):
    return a[0] * b[0] - a[1] * b[1], a[0] * b[1] + a[1] * b[0]


def _cross(a, b):
    return (a[0] - b[1], a[1] + b[0]), (a[0] + b[1], a[1] - b[0])


def _radix4(x, sign):
    a, b, c, d = x
    u, v = _cadd(a, c), _cadd(b, d)
    k1, k3 = _cross(_csub(a, c), _csub(b, d))[::sign]
    return [_cadd(u, v), k1, _csub(u, v), k3]


def _twiddle16(z, e, sign):
    re, im = z
    if e == 0:
        return z
    if e == 4:
        return (-im, re) if sign > 0 else (im, -re)
    c, s = float(np.cos(2 * np.pi * e / 16)), float(sign * np.sin(2 * np.pi * e / 16))
    if e % 2:
        return c * re - s * im, s * re + c * im
    return (c * (re - im), c * (re + im)) if c * s > 0 else (c * (re + im), c * (im - re))


class _RowMean:
    def __init__(self):
        self.sums, self.count = [None, None], 0

    def add(self, v):
        i = self.count % 2
        self.sums[i] = v if self.sums[i] is None else self.sums[i] + v
        self.count += 1

    def mean(self):
        return jnp.sum(self.sums[0] + self.sums[1], axis=0, keepdims=True) * (1.0 / D)


def _gelu(x):
    inner = x * (0.7978845608028654 + (0.7978845608028654 * 0.044715) * (x * x))
    half = 0.5 * x
    return half + half * jnp.tanh(inner)


_LEFT = (((0, 0), 1, (1, 1)), ((1, 0), 1, (1, 1)), ((0, 0), 0, None), ((1, 1), 0, None),
         ((0, 0), 1, (0, 1)), ((1, 0), -1, (0, 0)), ((0, 1), -1, (1, 1)))
_RIGHT = (((0, 0), 1, (1, 1)), ((0, 0), 0, None), ((0, 1), -1, (1, 1)), ((1, 0), -1, (0, 0)),
          ((1, 1), 0, None), ((0, 0), 1, (0, 1)), ((1, 0), 1, (1, 1)))
_RESULT = {(0, 0): {0: 1, 3: 1, 4: -1, 6: 1}, (0, 1): {2: 1, 4: 1},
           (1, 0): {1: 1, 3: 1}, (1, 1): {0: 1, 1: -1, 2: 1, 5: 1}}


def _signed_sum(term, quadrant):
    a, sign, b = term
    if sign == 0:
        return quadrant(*a)
    return quadrant(*a) + quadrant(*b) if sign > 0 else quadrant(*a) - quadrant(*b)


def _operands(table, block):
    for i, outer in enumerate(table):
        if outer[1]:
            sums = {(u, v): _signed_sum(outer, lambda r, c: block(i, 2 * r + u, 2 * c + v))
                    for u in range(2) for v in range(2)}
        for j, inner in enumerate(table):
            def quadrant(u, v):
                if outer[1]:
                    return sums[u, v]
                return block(7 * i + j, 2 * outer[0][0] + u, 2 * outer[0][1] + v)
            yield _signed_sum(inner, quadrant).astype(bf16)


def _completed(i, have):
    for quadrant, terms in _RESULT.items():
        if i in terms and all(j in have for j in terms):
            first, *rest = terms
            x = have[first]
            for j in rest:
                x = x + have[j] if terms[j] > 0 else x - have[j]
            yield quadrant, x


def _blocks(products):
    outer = {quadrant: {} for quadrant in _RESULT}
    for i in range(7):
        inner = {}
        for j in range(7):
            inner[j] = next(products)
            for (u, v), x in _completed(j, inner):
                outer[u, v][i] = x
                for (r, c), y in _completed(i, outer[u, v]):
                    yield (2 * r + u, 2 * c + v), y


def _in_turn(stages):
    for stage, _ in stages:
        for _ in stage:
            pass


def _in_step(stages):
    for q in range(NB):
        for stage, cuts in stages:
            for _ in range(cuts * q // NB, cuts * (q + 1) // NB):
                next(stage)
    _in_turn(stages)


def _skewed(stages, emit, n, after_fill=lambda: None):
    depth = len(stages) - 1

    def step(oldest, lo, hi):
        emit([(fn(oldest + (depth - lag)), cuts) for lag, cuts, fn in stages if lo <= lag <= hi])

    for i in range(depth):
        step(i - depth, 0, i)
    after_fill()
    lax.fori_loop(0, n - depth, lambda i, _: step(i, 0, depth), None)
    for i in range(n, n + depth):
        step(i - depth, i - n + 1, depth)


def _tile(t):
    if isinstance(t, int):
        return slice(128 * t, 128 * (t + 1))
    return pl.ds(pl.multiple_of(t * 128, 128), 128)


def _blk(i):
    return slice(8 * i, 8 * i + 8)


def _kernel(x_hbm, wr_hbm, wi_hbm, w1_hbm, b1_hbm, w2_hbm, b2_hbm, c_hbm, wm_hbm, chm_hbm, tok_hbm,
            out_hbm,
            x_v, wr_v, wi_v, w1_v, b1_v, w2_v, b2_v, c_v, wm_v, chm_v, tok_v,
            mod_v, fwd_v, inv_v, wt_v, wp_v, half_v, fa_v, fb_v, res_v, stat_v, a_v, acc_v,
            sem):
    def batch(slot, pairs):
        return [pltpu.make_async_copy(src, dst, sem.at[slot]) for src, dst in pairs]

    def start(copies):
        for c in copies:
            c.start()

    def wait(copies):
        for c in copies:
            c.wait()

    def cols(lo, n, *refs):
        return tuple(ref.at[:, pl.ds(lo, n)] for ref in refs)

    def mod_cols(part):
        lo, hi = MOD_PARTS[part]
        return cols(128 * lo, 128 * (hi - lo), wm_hbm, wm_v)

    def chm_half(i):
        return chm_hbm.at[pl.ds(5 * i, 5)], chm_v.at[pl.ds(5 * i, 5)]

    def w1_tiles(j):
        first = STARTS[j] // 128
        return [(*cols(128 * t, 128, w1_hbm), w1_v.at[t])
                for t in range(first, first + CHUNKS[j] // 128)]

    def w2_tiles(j):
        rows = pl.ds(STARTS[j], CHUNKS[j])
        return [(w2_hbm.at[rows, pl.ds(128 * t, 128)], w2_v.at[t, rows]) for t in range(NT)]

    def cp_x(i):
        lo = i * 256 if isinstance(i, int) else pl.multiple_of(i * 256, 256)
        return batch(i, [cols(lo, 256, x_hbm, x_v)])

    cp_tables = batch(8, [(tok_hbm, tok_v), (c_hbm, c_v)])
    cp_mod = batch(9, [mod_cols(0)])
    cp_forward = batch(10, [chm_half(0)])
    cp_filter = batch(11, [(wr_hbm, wr_v), (wi_hbm, wi_v)])
    cp_inverse = batch(12, [chm_half(1), mod_cols(1)])
    cp_mlp = [batch(13, [(b1_hbm, b1_v), (b2_hbm, b2_v), *w1_tiles(0)]),
              batch(0, w1_tiles(1)),
              batch(8, w2_tiles(0) + w1_tiles(2)),
              batch(9, w2_tiles(1)),
              batch(10, w2_tiles(2))]
    sem_out = sem.at[11]

    for copies in (cp_tables, cp_x(0), cp_x(1), cp_mod, *map(cp_x, range(2, NT // 2)),
                   cp_forward, cp_filter, cp_inverse, cp_mlp[0]):
        start(copies)

    wait(cp_tables)
    seed = [(tok_v[_blk(2 * i), :], tok_v[_blk(2 * i + 1), :]) for i in range(3)]
    dft = [seed[0]]
    for _ in range(15):
        dft.append(_cmul(dft[-1], seed[1]))
    dft = tuple(jnp.concatenate(part, axis=0) for part in zip(*dft))
    along = tuple(jnp.concatenate([part] * 16, axis=0) for part in seed[2])
    down = tuple(part.T for part in along)

    def token_factors(k, carry):
        for ref, (re, im), order in zip((fwd_v, inv_v), carry, ((0, 1, 2), (0, 2, 1))):
            for i, m in zip(order, (re, re + im, re - im)):
                ref[k, i] = m.astype(bf16)
        return _cmul(carry[0], down), _cmul(carry[1], along)

    lax.fori_loop(0, NT, token_factors, (dft, dft))

    c = c_v[...].astype(f32)
    silu_c = jnp.broadcast_to(c * jax.nn.sigmoid(c), (16, D)).astype(bf16)

    def store_mod(j):
        row = _dot(silu_c, wm_v[:, _tile(j)])[0:8, :]
        n = 128 * j + lax.broadcasted_iota(jnp.int32, row.shape, 1)
        scale = jnp.logical_or(jnp.logical_and(n >= D, n < 2 * D),
                               jnp.logical_and(n >= 4 * D, n < 5 * D))
        row = jnp.where(scale, row + 1.0, row)
        row = jnp.where(jnp.logical_and(n >= 2 * D, n < 3 * D), row * (2.0 / (S * D)), row)
        mod_v[_tile(j), :] = jnp.concatenate([row] * 16, axis=0).T

    def mod(i, b):
        return mod_v[_blk(i * NB + b), :]

    def first_mod():
        wait(cp_mod)
        for j in range(*MOD_PARTS[0]):
            store_mod(j)

    def statistic(tiles, slot, values, finish=lambda m: m):
        means = [_RowMean() for _ in tiles]
        for vs in zip(*map(values, tiles)):
            for m, v in zip(means, vs):
                m.add(v)
            yield
        for t, m in zip(tiles, means):
            stat_v[slot, t] = jnp.broadcast_to(finish(m.mean()), (8, 128))

    def inv_std(tiles, slot, src, dst=None):
        def squares(t):
            mean = stat_v[slot - 1, t]
            for b in range(NB):
                centred = src[t, _blk(b), :] - mean
                if dst is not None:
                    dst[t, _blk(b), :] = centred
                yield centred * centred
        return statistic(tiles, slot, squares, lambda var: lax.rsqrt(var + EPS))

    def adjacent(i):
        return 2 * i, 2 * i + 1

    def tokens(t):
        for i in range(D // 16):
            x = x_v[16 * i:16 * i + 16, _tile(t)].astype(f32)
            for b, half in enumerate((x[:8], x[8:]), 2 * i):
                res_v[t, _blk(b), :] = half
                yield half

    def load_tokens(i):
        wait(cp_x(i))
        return statistic(adjacent(i), 0, tokens)

    def fwd_butterflies(i):
        for t in adjacent(i):
            rstd = stat_v[1, t]
            for p in range(8):
                x0, uv = _radix9([fb_v[t, _blk(b), :] * rstd * mod(1, b) + mod(0, b)
                                  for b in range(p, NB, 8)])
                for g in range(4):
                    half_v[t, 128 * g + 16 * p:128 * g + 16 * p + 16, :] = _stack_bf16(uv[g])
                if p % 2:
                    half_v[t, 504 + 8 * p:520 + 8 * p, :] = _stack_bf16([previous, x0])
                previous = x0
                yield

    _skewed([(1, NB, lambda i: inv_std(adjacent(i), 1, res_v, fb_v)),
             (0, NB, load_tokens), (2, 16, fwd_butterflies)], _in_step, NT // 2, first_mod)

    def filter_out(t):
        re = pltpu.bitcast(wr_v[0:DF - 1, _tile(t)], u32)
        im = pltpu.bitcast(wi_v[0:DF - 1, _tile(t)], u32)
        row = lax.broadcasted_iota(jnp.int32, (8, 128), 0)
        nyquist = jnp.where(row == 0, wr_v[DF - 1:DF, _tile(t)].astype(f32),
                            jnp.where(row == 1, wi_v[DF - 1:DF, _tile(t)].astype(f32), 0.0))
        rest = jnp.concatenate([re[128:], im[128:], pltpu.bitcast(nyquist, u32),
                                jnp.zeros((88, 128), u32)], axis=0)
        for i, words in enumerate((re[:128].T, im[:128].T, rest.T)):
            for j in range(8):
                lo = (NT + 1) * (8 * t + j)
                wt_v[i, lo:lo + NT, :] = words[NT * j:NT * (j + 1)]

    def filter_back(k):
        re, im, rest = (wt_v[i, pl.ds(k, 128, stride=NT + 1), :].T for i in range(3))
        wp_v[k, 0:128, :], wp_v[k, 128:144, :] = re, rest[0:16]
        wp_v[k, 144:272, :], wp_v[k, 272:296, :] = im, rest[16:40]

    def filter_rows(k, rb, part):
        if rb == NRB - 1:
            w = jnp.broadcast_to(wp_v[k, 288 + part:289 + part, :], (8, 128))
        else:
            k0 = _RUNS[rb // 2]
            w = wp_v[k, pl.ds(144 * part + k0 // 2 + 72 * (rb % 2), 8, stride=9), :]
            w = (w & np.uint32(0xFFFF0000)) if k0 % 2 else (w << 16)
        return pltpu.bitcast(w, f32)

    groups = [range(8 * g, min(8 * g + 8, NRB)) for g in range(5)]
    rounds = [(q, odd) for q in range(4) for odd in (0, 1)]

    def harmonics(q, odd):
        return q + 4 * odd, q + 4 * odd + 8

    def get(ref, i, rb):
        return ref[i, _blk(2 * rb), :], ref[i, _blk(2 * rb + 1), :]

    def put(ref, i, rb, z):
        ref[i, _blk(2 * rb), :], ref[i, _blk(2 * rb + 1), :] = z

    def channel_matrix(i, rows=128):
        return pltpu.bitcast(chm_v[i, 0:rows // 2, :], bf16)

    def token_dft(z, factors, k):
        def times(parts, i):
            return _dot(_stack_bf16([*parts, jnp.zeros((8, 128), f32)]), factors[k, i])
        s = times([re + im for re, im in z], 0)
        a, b = times([im for _, im in z], 1), times([re for re, _ in z], 2)
        return [(s[_blk(rb)] - a[_blk(rb)], s[_blk(rb)] - b[_blk(rb)]) for rb in range(NRB)]

    def fwd_channel(g, t0):
        tiles = range(t0, NT, 4)
        if g < 4:
            outs = [_dot(channel_matrix(g), half_v[t, _tile(g), :]) for t in tiles]
        else:
            pad = jnp.zeros((64, 128), bf16)
            outs = [_dot(channel_matrix(4, 80),
                         jnp.concatenate([half_v[t, 512:576, :], pad], axis=0)) for t in tiles]
        for i, rb in enumerate(groups[g]):
            y = _radix4([(o[_blk(2 * i)], o[_blk(2 * i + 1)]) for o in outs], -1)
            for q in range(4):
                put(fa_v, 4 * q + t0, rb, _twiddle16(y[q], t0 * q, -1))

    def fwd_token(q, odd):
        z = []
        for rb in range(NRB):
            a, b, c, d = (get(fa_v, 4 * q + t0, rb) for t0 in range(4))
            if odd:
                z.append(_cross(_csub(a, c), _csub(b, d))[::-1])
            else:
                u, v = _cadd(a, c), _cadd(b, d)
                z.append((_cadd(u, v), _csub(u, v)))
        for k, zk in zip(harmonics(q, odd), zip(*z)):
            for rb, y in enumerate(token_dft(zk, fwd_v, k)):
                put(fb_v, k, rb, y)

    def inv_token(q, odd):
        outs = []
        for k in harmonics(q, odd):
            z = [_cmul(get(fb_v, k, rb), (filter_rows(k, rb, 0), filter_rows(k, rb, 1)))
                 for rb in range(NRB)]
            outs.append(token_dft(z, inv_v, k))
        for rb, (a, c) in enumerate(zip(*outs)):
            u, v = _cadd(a, c), _csub(a, c)
            if odd:
                p, m = get(fa_v, q, rb), get(fa_v, 4 + q, rb)
                y1, y3 = _cross(m, v)
                for t0, y in enumerate((_cadd(p, u), y1, _csub(p, u), y3)):
                    put(fa_v, 4 * t0 + q, rb, _twiddle16(y, t0 * q, +1))
            else:
                put(fa_v, q, rb, u)
                put(fa_v, 4 + q, rb, v)

    def inv_channel(g, t0):
        z = [_radix4([get(fa_v, 4 * t0 + q, rb) for q in range(4)], +1) for rb in groups[g]]
        for t, zt in zip(range(t0, NT, 4), zip(*z)):
            parts = [v for pair in zt for v in pair]
            if g < 4:
                fb_v[t, _tile(g), :] = _dot(channel_matrix(5 + g), _stack_bf16(parts))
            else:
                fb_v[t, 512:576, :] = _dot(channel_matrix(9, 64),
                                           _stack_bf16([*parts, jnp.zeros((48, 128), f32)]))

    start(cp_mlp[1])
    wait(cp_forward)
    for i in range(20):
        fwd_channel(*divmod(i, 4))
    for i, r in enumerate(rounds):
        if i == 2:
            wait(cp_filter)
        fwd_token(*r)
        if 2 <= i < 6:
            for t in range(4 * i - 8, 4 * i - 4):
                filter_out(t)
        elif i >= 6:
            for k in harmonics(*rounds[i - 6]):
                filter_back(k)
    for i, r in enumerate(rounds):
        if i < 6:
            for k in harmonics(*rounds[i + 2]):
                filter_back(k)
        inv_token(*r)
    wait(cp_inverse)
    for i in range(20):
        inv_channel(*divmod(i, 4))
        if MOD_PARTS[1][0] + i < MOD_PARTS[1][1]:
            store_mod(MOD_PARTS[1][0] + i)

    def opposite(j):
        return j, j + NT // 2

    def residual(t):
        for p in range(8):
            uv = [(fb_v[t, _blk(16 * g + 2 * p), :], fb_v[t, _blk(16 * g + 2 * p + 1), :])
                  for g in range(4)]
            for a, y in enumerate(_radix9_transposed(fb_v[t, _blk(64 + p), :], uv)):
                b = 8 * a + p
                x = res_v[t, _blk(b), :] + mod(2, b) * y
                res_v[t, _blk(b), :] = x
                yield x

    def modulated(t):
        rstd = stat_v[1, t]
        for b in range(NB):
            h = fa_v[t, _blk(b), :] * rstd * mod(4, b) + mod(3, b)
            fb_v[t, _blk(b), :] = h
            yield h

    def mlp_operands(j, _):
        stats = [(t, stat_v[2, t], stat_v[3, t]) for t in (j + 4 * c for c in range(4))]
        for r0 in range(0, HB, 16):
            h = {(r, c): jnp.concatenate([(fb_v[t, q:q + 8, :] - mean) * rstd
                                          for q in (HB * r + r0, HB * r + r0 + 8)], axis=0)
                 for r in range(4) for c, (t, mean, rstd) in enumerate(stats)}
            for i, a in enumerate(_operands(_LEFT, lambda _, r, c: h[r, c])):
                a_v[i, j, r0:r0 + 16, :] = a

    _skewed([(1, NB, lambda j: inv_std(opposite(j), 1, res_v, fa_v)),
             (0, NB, lambda j: statistic(opposite(j), 0, residual))], _in_turn, NT // 2)
    _skewed([(1, NB, lambda j: inv_std(opposite(j), 3, fb_v)),
             (0, NB, lambda j: statistic(opposite(j), 2, modulated))], _in_turn, NT // 2)
    lax.fori_loop(0, 4, mlp_operands, None)

    zero = pl.program_id(0)

    def weights(ref, top, height, left, width):
        def block(tag, r, c):
            rows = pl.ds(pl.multiple_of(top + r * height + 16 * tag * zero, 16), height)
            first = (left + c * width) // 128
            return jnp.concatenate([ref[t, rows, :].astype(f32)
                                    for t in range(first, first + width // 128)], axis=1)
        return _operands(_RIGHT, block)

    def hidden(j):
        lo, n = STARTS[j], CHUNKS[j] // 4
        bias = [jnp.concatenate([b1[t:t + 1, :] for t in range((lo + c * n) // 128,
                                                               (lo + c * n + n) // 128)], axis=1)
                for c in range(4)]
        return {(r, c): _gelu(u + bias[c]) for (r, c), u in _blocks(
            _dot(jnp.concatenate([a_v[i, t] for t in range(4)], axis=1), w)
            for i, w in enumerate(weights(w1_v, 0, SB, lo, n)))}

    def products(j, g):
        return enumerate(map(_dot, _operands(_LEFT, lambda _, r, c: g[r, c]),
                             weights(w2_v, STARTS[j], CHUNKS[j] // 4, 0, SB)))

    wait(cp_mlp[0])
    start(cp_mlp[2])
    b1, b2 = b1_v[...].astype(f32), b2_v[...].astype(f32)
    g0 = hidden(0)
    wait(cp_mlp[1])
    start(cp_mlp[3])
    g1 = hidden(1)
    wait(cp_mlp[2])
    start(cp_mlp[4])
    for i, m in products(0, g0):
        acc_v[i] = m
    g2 = hidden(2)
    wait(cp_mlp[3] + cp_mlp[4])
    for i, m in products(1, g1):
        acc_v[i] += m
    for (r, c), y in _blocks(acc_v[i] + m for i, m in products(2, g2)):
        rows = slice(HB * r, HB * (r + 1))
        gate = mod_v[5 * D + HB * r:5 * D + HB * (r + 1), :]
        for t in range(4 * c, 4 * c + 4):
            branch = y[:, _tile(t - 4 * c)] + b2[t:t + 1, :]
            half_v[t, rows, :] = (res_v[t, rows, :] + gate * branch).astype(bf16)
            pltpu.make_async_copy(
                half_v.at[t, rows], out_hbm.at[rows, _tile(t)], sem_out).start()
    pltpu.make_async_copy(out_hbm, out_hbm, sem_out).wait()


@jax.jit
def pallas_adaLN_cond__spectral_gfnet__mixer_token_mlp__prompt_kernel(
    A_x: jax.Array,
    A_w_r: jax.Array,
    A_w_i: jax.Array,
    B_x: jax.Array,
    B_w1: jax.Array,
    B_b1: jax.Array,
    B_w2: jax.Array,
    B_b2: jax.Array,
    c: jax.Array,
    w_mod: jax.Array,
):
    del B_x
    vmem = pltpu.VMEM
    scratch = [
        vmem((D, S), bf16), vmem((DF, S), bf16), vmem((DF, S), bf16),
        vmem((F // 128, S, 128), bf16), vmem((F // 128, 128), bf16),
        vmem((NT, F, 128), bf16), vmem((NT, 128), bf16),
        vmem((1, D), bf16), vmem((D, 6 * D), bf16),
        vmem(_CHANNEL_MATRICES.shape, u32), vmem(_TOKEN_SEEDS.shape, f32),
        vmem((6 * D, 128), f32),
        vmem((NT, 3, 128, 128), bf16),
        vmem((NT, 3, 128, 128), bf16),
        vmem((3, S + 128, 128), u32),
        vmem((NT, 8 * NRB, 128), u32),
        vmem((NT, D, 128), bf16),
        vmem((NT, 16 * NRB, 128), f32),
        vmem((NT, 16 * NRB, 128), f32),
        vmem((NT, D, 128), f32),
        vmem((4, NT, 8, 128), f32),
        vmem((49, 4, HB, 128), bf16),
        vmem((49, HB, SB), f32),
        pltpu.SemaphoreType.DMA((14,)),
    ]
    out = pl.pallas_call(
        _kernel,
        grid=(1,),
        in_specs=[pl.BlockSpec(memory_space=pl.ANY)] * 11,
        out_specs=pl.BlockSpec(memory_space=pl.ANY),
        out_shape=jax.ShapeDtypeStruct((D, S), bf16),
        scratch_shapes=scratch,
        compiler_params=pltpu.CompilerParams(vmem_limit_bytes=124 * 1024 * 1024),
    )(A_x.reshape(S, D).T, A_w_r.T, A_w_i.T, B_w1, B_b1.reshape(F // 128, 128), B_w2,
      B_b2.reshape(NT, 128), c, w_mod, _CHANNEL_MATRICES, _TOKEN_SEEDS)
    return out.T.reshape(1, S, D)
```

```python
import jax
import jax.numpy as jnp
import numpy as np
from jax import lax
from jax.experimental import pallas as pl
from jax.experimental.pallas import tpu as pltpu

D, S, F = 576, 2048, 4608
DF = D // 2 + 1
NT = S // 128
NB = D // 8
NRB = 37
HB, SB = D // 4, S // 4
CHUNKS = (1024, 1024, 2560)
STARTS = tuple(sum(CHUNKS[:j]) for j in range(len(CHUNKS)))
MOD_PARTS = ((0, 9), (9, 27))
EPS = 1e-5

f32, bf16, u32 = jnp.float32, jnp.bfloat16, jnp.uint32

_Q = np.sqrt(3.0) / 2
_C1, _C2, _C4 = (float(np.cos(2 * np.pi * k / 9)) for k in (1, 2, 4))
_S1, _S2, _S4 = (float(np.sin(2 * np.pi * k / 9) / _Q) for k in (1, 2, 4))

_RUNS = [r + e for g in (1, 2, 3, 4) for r in (g, 9 - g) for e in (0, 9)] + [0, 9]


def _channel_matrices():
    kd_all = np.array([k0 + 18 * j for k0 in _RUNS for j in range(16)] + [D // 2] + [-1] * 7)
    b = np.arange(64)
    mats = np.zeros((10, 128, 128))
    for g in (1, 2, 3, 4):
        kd = kd_all[64 * (g - 1):64 * g]
        sign = np.where(kd % 9 == g, -1.0, 1.0).reshape(8, 8, 1, 1)
        angle = (2 * np.pi / D) * ((kd[:, None] * b[None, :]) % D)
        c, s = np.cos(angle).reshape(8, 8, 8, 8), np.sin(angle).reshape(8, 8, 8, 8)
        m = np.zeros((8, 2, 8, 8, 2, 8))
        m[:, 0, :, :, 0, :] = c
        m[:, 0, :, :, 1, :] = sign * _Q * s
        m[:, 1, :, :, 0, :] = -s
        m[:, 1, :, :, 1, :] = sign * _Q * c
        mats[g - 1] = m.reshape(128, 128)
        mats[g + 4] = m.reshape(128, 128).T
    kd = kd_all[256:]
    valid = (kd >= 0)[:, None]
    angle = (2 * np.pi / D) * ((kd[:, None] * b[None, :]) % D)
    m = np.zeros((5, 2, 8, 64))
    m[:, 0] = (np.cos(angle) * valid).reshape(5, 8, 64)
    m[:, 1] = (-np.sin(angle) * valid * (kd != D // 2)[:, None]).reshape(5, 8, 64)
    half = np.where((kd == 0) | (kd == D // 2), 0.5, 1.0).reshape(5, 1, 8, 1)
    mats[4, :80, :64] = m.reshape(80, 64)
    mats[9, :64, :80] = (m * half).reshape(80, 64).T
    bits = mats.astype(np.float32).astype(jnp.bfloat16).view(np.uint16).astype(np.uint32)
    return bits[:, 0::2, :] | (bits[:, 1::2, :] << np.uint32(16))


def _token_seeds():
    l = np.arange(128)
    ones = np.ones((8, 1))
    angles = [(2 * np.pi / 128) * ((l[:8, None] * l[None, :]) % 128),
              (2 * np.pi / 128) * ((8 * l) % 128) * ones, (2 * np.pi / S) * l * ones]
    return np.concatenate([p for a in angles for p in (np.cos(a), -np.sin(a))]).astype(np.float32)


_CHANNEL_MATRICES = _channel_matrices()
_TOKEN_SEEDS = _token_seeds()


def _dot(a, b):
    return jnp.dot(a, b, preferred_element_type=f32)


def _stack_bf16(parts):
    return jnp.concatenate(parts, axis=0).astype(bf16)


def _radix9(x):
    s1, s2, s3, s4 = x[1] + x[8], x[2] + x[7], x[3] + x[6], x[4] + x[5]
    d1, d2, d3, d4 = x[1] - x[8], x[2] - x[7], x[3] - x[6], x[4] - x[5]
    p = x[0] - 0.5 * s3
    a, b = s1 - s4, s2 - s4
    r1 = _C1 * a + _C2 * b
    r2 = _C2 * a + _C4 * b
    e, g = d1 + d2, d2 + d4
    i1 = _S1 * e + _S4 * g
    i2 = _S2 * e - _S1 * g
    t, u = s1 + s2 + s4, x[0] + s3
    return u + t, [(p + r1, i1 + d3), (p + r2, i2 - d3),
                   (u - 0.5 * t, d1 - d2 + d4), ((p - r1) - r2, (i2 - i1) + d3)]


def _radix9_transposed(x0, uv):
    (u1, v1), (u2, v2), (u3, v3), (u4, v4) = uv
    u, t = x0 + u3, x0 - 0.5 * u3
    p, r1, r2 = u1 + u2 + u4, u1 - u4, u2 - u4
    a = _C1 * r1 + _C2 * r2
    b = _C2 * r1 + _C4 * r2
    s1, s2, s3, s4 = t + a, t + b, u - 0.5 * p, (t - a) - b
    i1, i2, d3 = v1 - v4, v2 + v4, v1 - v2 + v4
    e = _S1 * i1 + _S2 * i2
    g = _S4 * i1 - _S1 * i2
    d1, d2, d4 = e + v3, (e + g) - v3, g + v3
    return [u + p, s1 + d1, s2 + d2, s3 + d3, s4 + d4, s4 - d4, s3 - d3, s2 - d2, s1 - d1]


def _cadd(a, b):
    return a[0] + b[0], a[1] + b[1]


def _csub(a, b):
    return a[0] - b[0], a[1] - b[1]


def _cmul(a, b):
    return a[0] * b[0] - a[1] * b[1], a[0] * b[1] + a[1] * b[0]


def _cross(a, b):
    return (a[0] - b[1], a[1] + b[0]), (a[0] + b[1], a[1] - b[0])


def _radix4(x, sign):
    a, b, c, d = x
    u, v = _cadd(a, c), _cadd(b, d)
    k1, k3 = _cross(_csub(a, c), _csub(b, d))[::sign]
    return [_cadd(u, v), k1, _csub(u, v), k3]


def _twiddle16(z, e, sign):
    re, im = z
    if e == 0:
        return z
    if e == 4:
        return (-im, re) if sign > 0 else (im, -re)
    c, s = float(np.cos(2 * np.pi * e / 16)), float(sign * np.sin(2 * np.pi * e / 16))
    if e % 2:
        return c * re - s * im, s * re + c * im
    return (c * (re - im), c * (re + im)) if c * s > 0 else (c * (re + im), c * (im - re))


class _RowMean:
    def __init__(self):
        self.sums, self.count = [None, None], 0

    def add(self, v):
        i = self.count % 2
        self.sums[i] = v if self.sums[i] is None else self.sums[i] + v
        self.count += 1

    def mean(self):
        return jnp.sum(self.sums[0] + self.sums[1], axis=0, keepdims=True) * (1.0 / D)


def _gelu(x):
    inner = x * (0.7978845608028654 + (0.7978845608028654 * 0.044715) * (x * x))
    half = 0.5 * x
    return half + half * jnp.tanh(inner)


_LEFT = (((0, 0), 1, (1, 1)), ((1, 0), 1, (1, 1)), ((0, 0), 0, None), ((1, 1), 0, None),
         ((0, 0), 1, (0, 1)), ((1, 0), -1, (0, 0)), ((0, 1), -1, (1, 1)))
_RIGHT = (((0, 0), 1, (1, 1)), ((0, 0), 0, None), ((0, 1), -1, (1, 1)), ((1, 0), -1, (0, 0)),
          ((1, 1), 0, None), ((0, 0), 1, (0, 1)), ((1, 0), 1, (1, 1)))
_RESULT = {(0, 0): {0: 1, 3: 1, 4: -1, 6: 1}, (0, 1): {2: 1, 4: 1},
           (1, 0): {1: 1, 3: 1}, (1, 1): {0: 1, 1: -1, 2: 1, 5: 1}}
_ORDER = (1, 0, 4, 2, 5, 3, 6)


def _signed_sum(term, quadrant):
    a, sign, b = term
    if sign == 0:
        return quadrant(*a)
    return quadrant(*a) + quadrant(*b) if sign > 0 else quadrant(*a) - quadrant(*b)


def _operands(table, block):
    for i in _ORDER:
        outer = table[i]
        if outer[1]:
            sums = {(u, v): _signed_sum(outer, lambda r, c: block(i, 2 * r + u, 2 * c + v))
                    for u in range(2) for v in range(2)}
        for j in _ORDER:
            def quadrant(u, v):
                if outer[1]:
                    return sums[u, v]
                return block(7 * i + j, 2 * outer[0][0] + u, 2 * outer[0][1] + v)
            yield _signed_sum(table[j], quadrant).astype(bf16)


def _completed(i, have):
    for quadrant, terms in _RESULT.items():
        if i in terms and all(j in have for j in terms):
            first, *rest = terms
            x = have[first]
            for j in rest:
                x = x + have[j] if terms[j] > 0 else x - have[j]
            yield quadrant, x


def _blocks(products):
    outer = {quadrant: {} for quadrant in _RESULT}
    for i in _ORDER:
        inner = {}
        for j in _ORDER:
            inner[j] = next(products)
            for (u, v), x in _completed(j, inner):
                outer[u, v][i] = x
                for (r, c), y in _completed(i, outer[u, v]):
                    yield (2 * r + u, 2 * c + v), y


def _in_turn(stages):
    for stage, _ in stages:
        for _ in stage:
            pass


def _in_step(stages):
    for q in range(NB):
        for stage, cuts in stages:
            for _ in range(cuts * q // NB, cuts * (q + 1) // NB):
                next(stage)
    _in_turn(stages)


def _skewed(stages, emit, n, after_fill=lambda: None):
    depth = len(stages) - 1

    def step(oldest, lo, hi):
        emit([(fn(oldest + (depth - lag)), cuts) for lag, cuts, fn in stages if lo <= lag <= hi])

    for i in range(depth):
        step(i - depth, 0, i)
    after_fill()
    lax.fori_loop(0, n - depth, lambda i, _: step(i, 0, depth), None)
    for i in range(n, n + depth):
        step(i - depth, i - n + 1, depth)


def _tile(t):
    if isinstance(t, int):
        return slice(128 * t, 128 * (t + 1))
    return pl.ds(pl.multiple_of(t * 128, 128), 128)


def _blk(i):
    return slice(8 * i, 8 * i + 8)


def _kernel(x_hbm, wr_hbm, wi_hbm, w1_hbm, b1_hbm, w2_hbm, b2_hbm, c_hbm, wm_hbm, chm_hbm, tok_hbm,
            out_hbm,
            x_v, wr_v, wi_v, w1_v, b1_v, w2_v, b2_v, c_v, wm_v, chm_v, tok_v,
            mod_v, fwd_v, inv_v, wt_v, wp_v, half_v, fa_v, fb_v, res_v, stat_v, a_v, acc_v,
            sem):
    def batch(slot, pairs):
        return [pltpu.make_async_copy(src, dst, sem.at[slot]) for src, dst in pairs]

    def start(copies):
        for c in copies:
            c.start()

    def wait(copies):
        for c in copies:
            c.wait()

    def cols(lo, n, *refs):
        return tuple(ref.at[:, pl.ds(lo, n)] for ref in refs)

    def mod_cols(part):
        lo, hi = MOD_PARTS[part]
        return cols(128 * lo, 128 * (hi - lo), wm_hbm, wm_v)

    def chm_half(i):
        return chm_hbm.at[pl.ds(5 * i, 5)], chm_v.at[pl.ds(5 * i, 5)]

    def w1_tiles(j):
        first = STARTS[j] // 128
        return [(*cols(128 * t, 128, w1_hbm), w1_v.at[t])
                for t in range(first, first + CHUNKS[j] // 128)]

    def w2_tiles(j):
        rows = pl.ds(STARTS[j], CHUNKS[j])
        return [(w2_hbm.at[rows, pl.ds(128 * t, 128)], w2_v.at[t, rows]) for t in range(NT)]

    def cp_x(i):
        lo = i * 256 if isinstance(i, int) else pl.multiple_of(i * 256, 256)
        return batch(i, [cols(lo, 256, x_hbm, x_v)])

    cp_tables = batch(8, [(tok_hbm, tok_v), (c_hbm, c_v)])
    cp_mod = batch(9, [mod_cols(0)])
    cp_forward = batch(10, [chm_half(0)])
    cp_filter = batch(11, [(wr_hbm, wr_v), (wi_hbm, wi_v)])
    cp_inverse = batch(12, [chm_half(1), mod_cols(1)])
    cp_mlp = [batch(13, [(b1_hbm, b1_v), (b2_hbm, b2_v), *w1_tiles(0)]),
              batch(0, w1_tiles(1) + w2_tiles(0)),
              batch(8, w1_tiles(2)),
              batch(9, w2_tiles(1)),
              batch(10, w2_tiles(2))]
    sem_out = sem.at[11]

    for copies in (cp_tables, cp_x(0), cp_x(1), cp_mod, *map(cp_x, range(2, NT // 2)),
                   cp_forward, cp_filter, cp_inverse, cp_mlp[0]):
        start(copies)

    wait(cp_tables)
    seed = [(tok_v[_blk(2 * i), :], tok_v[_blk(2 * i + 1), :]) for i in range(3)]
    dft = [seed[0]]
    for _ in range(15):
        dft.append(_cmul(dft[-1], seed[1]))
    dft = tuple(jnp.concatenate(part, axis=0) for part in zip(*dft))
    along = tuple(jnp.concatenate([part] * 16, axis=0) for part in seed[2])
    down = tuple(part.T for part in along)

    def token_factors(k, carry):
        for ref, (re, im), order in zip((fwd_v, inv_v), carry, ((0, 1, 2), (0, 2, 1))):
            for i, m in zip(order, (re, re + im, re - im)):
                ref[k, i] = m.astype(bf16)
        return _cmul(carry[0], down), _cmul(carry[1], along)

    lax.fori_loop(0, NT, token_factors, (dft, dft))

    c = c_v[...].astype(f32)
    silu_c = jnp.broadcast_to(c * jax.nn.sigmoid(c), (16, D)).astype(bf16)

    def store_mod(j):
        row = _dot(silu_c, wm_v[:, _tile(j)])[0:8, :]
        n = 128 * j + lax.broadcasted_iota(jnp.int32, row.shape, 1)
        scale = jnp.logical_or(jnp.logical_and(n >= D, n < 2 * D),
                               jnp.logical_and(n >= 4 * D, n < 5 * D))
        row = jnp.where(scale, row + 1.0, row)
        row = jnp.where(jnp.logical_and(n >= 2 * D, n < 3 * D), row * (2.0 / (S * D)), row)
        mod_v[_tile(j), :] = jnp.concatenate([row] * 16, axis=0).T

    def mod(i, b):
        return mod_v[_blk(i * NB + b), :]

    def first_mod():
        wait(cp_mod)
        for j in range(*MOD_PARTS[0]):
            store_mod(j)

    def statistic(tiles, slot, values, finish=lambda m: m):
        means = [_RowMean() for _ in tiles]
        for vs in zip(*map(values, tiles)):
            for m, v in zip(means, vs):
                m.add(v)
            yield
        for t, m in zip(tiles, means):
            stat_v[slot, t] = jnp.broadcast_to(finish(m.mean()), (8, 128))

    def inv_std(tiles, slot, src, dst=None):
        def squares(t):
            mean = stat_v[slot - 1, t]
            for b in range(NB):
                centred = src[t, _blk(b), :] - mean
                if dst is not None:
                    dst[t, _blk(b), :] = centred
                yield centred * centred
        return statistic(tiles, slot, squares, lambda var: lax.rsqrt(var + EPS))

    def adjacent(i):
        return 2 * i, 2 * i + 1

    def tokens(t):
        for i in range(D // 16):
            x = x_v[16 * i:16 * i + 16, _tile(t)].astype(f32)
            for b, half in enumerate((x[:8], x[8:]), 2 * i):
                res_v[t, _blk(b), :] = half
                yield half

    def load_tokens(i):
        wait(cp_x(i))
        return statistic(adjacent(i), 0, tokens)

    def fwd_butterflies(i):
        for t in adjacent(i):
            rstd = stat_v[1, t]
            for p in range(8):
                x0, uv = _radix9([fb_v[t, _blk(b), :] * rstd * mod(1, b) + mod(0, b)
                                  for b in range(p, NB, 8)])
                for g in range(4):
                    half_v[t, 128 * g + 16 * p:128 * g + 16 * p + 16, :] = _stack_bf16(uv[g])
                if p % 2:
                    half_v[t, 504 + 8 * p:520 + 8 * p, :] = _stack_bf16([previous, x0])
                previous = x0
                yield

    _skewed([(1, NB, lambda i: inv_std(adjacent(i), 1, res_v, fb_v)),
             (0, NB, load_tokens), (2, 16, fwd_butterflies)], _in_step, NT // 2, first_mod)

    def filter_out(t):
        re = pltpu.bitcast(wr_v[0:DF - 1, _tile(t)], u32)
        im = pltpu.bitcast(wi_v[0:DF - 1, _tile(t)], u32)
        row = lax.broadcasted_iota(jnp.int32, (8, 128), 0)
        nyquist = jnp.where(row == 0, wr_v[DF - 1:DF, _tile(t)].astype(f32),
                            jnp.where(row == 1, wi_v[DF - 1:DF, _tile(t)].astype(f32), 0.0))
        rest = jnp.concatenate([re[128:], im[128:], pltpu.bitcast(nyquist, u32),
                                jnp.zeros((88, 128), u32)], axis=0)
        for i, words in enumerate((re[:128].T, im[:128].T, rest.T)):
            for j in range(8):
                lo = (NT + 1) * (8 * t + j)
                wt_v[i, lo:lo + NT, :] = words[NT * j:NT * (j + 1)]

    def filter_back(k):
        re, im, rest = (wt_v[i, pl.ds(k, 128, stride=NT + 1), :].T for i in range(3))
        wp_v[k, 0:128, :], wp_v[k, 128:144, :] = re, rest[0:16]
        wp_v[k, 144:272, :], wp_v[k, 272:296, :] = im, rest[16:40]

    def filter_rows(k, rb, part):
        if rb == NRB - 1:
            w = jnp.broadcast_to(wp_v[k, 288 + part:289 + part, :], (8, 128))
        else:
            k0 = _RUNS[rb // 2]
            w = wp_v[k, pl.ds(144 * part + k0 // 2 + 72 * (rb % 2), 8, stride=9), :]
            w = (w & np.uint32(0xFFFF0000)) if k0 % 2 else (w << 16)
        return pltpu.bitcast(w, f32)

    groups = [range(8 * g, min(8 * g + 8, NRB)) for g in range(5)]
    rounds = [(q, odd) for q in range(4) for odd in (0, 1)]

    def harmonics(q, odd):
        return q + 4 * odd, q + 4 * odd + 8

    def get(ref, i, rb):
        return ref[i, _blk(2 * rb), :], ref[i, _blk(2 * rb + 1), :]

    def put(ref, i, rb, z):
        ref[i, _blk(2 * rb), :], ref[i, _blk(2 * rb + 1), :] = z

    def channel_matrix(i, rows=128):
        return pltpu.bitcast(chm_v[i, 0:rows // 2, :], bf16)

    def token_dft(z, factors, k):
        def times(parts, i):
            return _dot(_stack_bf16([*parts, jnp.zeros((8, 128), f32)]), factors[k, i])
        s = times([re + im for re, im in z], 0)
        a, b = times([im for _, im in z], 1), times([re for re, _ in z], 2)
        return [(s[_blk(rb)] - a[_blk(rb)], s[_blk(rb)] - b[_blk(rb)]) for rb in range(NRB)]

    def fwd_channel(g, t0):
        tiles = range(t0, NT, 4)
        if g < 4:
            outs = [_dot(channel_matrix(g), half_v[t, _tile(g), :]) for t in tiles]
        else:
            pad = jnp.zeros((64, 128), bf16)
            outs = [_dot(channel_matrix(4, 80),
                         jnp.concatenate([half_v[t, 512:576, :], pad], axis=0)) for t in tiles]
        for i, rb in enumerate(groups[g]):
            y = _radix4([(o[_blk(2 * i)], o[_blk(2 * i + 1)]) for o in outs], -1)
            for q in range(4):
                put(fa_v, 4 * q + t0, rb, _twiddle16(y[q], t0 * q, -1))

    def fwd_token(q, odd):
        z = []
        for rb in range(NRB):
            a, b, c, d = (get(fa_v, 4 * q + t0, rb) for t0 in range(4))
            if odd:
                z.append(_cross(_csub(a, c), _csub(b, d))[::-1])
            else:
                u, v = _cadd(a, c), _cadd(b, d)
                z.append((_cadd(u, v), _csub(u, v)))
        for k, zk in zip(harmonics(q, odd), zip(*z)):
            for rb, y in enumerate(token_dft(zk, fwd_v, k)):
                put(fb_v, k, rb, y)

    def inv_token(q, odd):
        outs = []
        for k in harmonics(q, odd):
            z = [_cmul(get(fb_v, k, rb), (filter_rows(k, rb, 0), filter_rows(k, rb, 1)))
                 for rb in range(NRB)]
            outs.append(token_dft(z, inv_v, k))
        for rb, (a, c) in enumerate(zip(*outs)):
            u, v = _cadd(a, c), _csub(a, c)
            if odd:
                p, m = get(fa_v, q, rb), get(fa_v, 4 + q, rb)
                y1, y3 = _cross(m, v)
                for t0, y in enumerate((_cadd(p, u), y1, _csub(p, u), y3)):
                    put(fa_v, 4 * t0 + q, rb, _twiddle16(y, t0 * q, +1))
            else:
                put(fa_v, q, rb, u)
                put(fa_v, 4 + q, rb, v)

    def inv_channel(g, t0):
        z = [_radix4([get(fa_v, 4 * t0 + q, rb) for q in range(4)], +1) for rb in groups[g]]
        for t, zt in zip(range(t0, NT, 4), zip(*z)):
            parts = [v for pair in zt for v in pair]
            if g < 4:
                fb_v[t, _tile(g), :] = _dot(channel_matrix(5 + g), _stack_bf16(parts))
            else:
                fb_v[t, 512:576, :] = _dot(channel_matrix(9, 64),
                                           _stack_bf16([*parts, jnp.zeros((48, 128), f32)]))

    start(cp_mlp[1])
    wait(cp_forward)
    for i in range(20):
        fwd_channel(*divmod(i, 4))
    for i, r in enumerate(rounds):
        if i == 2:
            wait(cp_filter)
        fwd_token(*r)
        if 2 <= i < 6:
            for t in range(4 * i - 8, 4 * i - 4):
                filter_out(t)
        elif i >= 6:
            for k in harmonics(*rounds[i - 6]):
                filter_back(k)
    for i, r in enumerate(rounds):
        if i < 6:
            for k in harmonics(*rounds[i + 2]):
                filter_back(k)
        inv_token(*r)
    wait(cp_inverse)
    for i in range(20):
        inv_channel(*divmod(i, 4))
        if MOD_PARTS[1][0] + i < MOD_PARTS[1][1]:
            store_mod(MOD_PARTS[1][0] + i)

    def opposite(j):
        return j, j + NT // 2

    def residual(t):
        for p in range(8):
            uv = [(fb_v[t, _blk(16 * g + 2 * p), :], fb_v[t, _blk(16 * g + 2 * p + 1), :])
                  for g in range(4)]
            for a, y in enumerate(_radix9_transposed(fb_v[t, _blk(64 + p), :], uv)):
                b = 8 * a + p
                x = res_v[t, _blk(b), :] + mod(2, b) * y
                res_v[t, _blk(b), :] = x
                yield x

    def modulated(t):
        rstd = stat_v[1, t]
        for b in range(NB):
            h = fa_v[t, _blk(b), :] * rstd * mod(4, b) + mod(3, b)
            fb_v[t, _blk(b), :] = h
            yield h

    def mlp_operands(j, _):
        stats = [(t, stat_v[2, t], stat_v[3, t]) for t in (j + 4 * c for c in range(4))]
        for r0 in range(0, HB, 16):
            h = {(r, c): jnp.concatenate([(fb_v[t, q:q + 8, :] - mean) * rstd
                                          for q in (HB * r + r0, HB * r + r0 + 8)], axis=0)
                 for r in range(4) for c, (t, mean, rstd) in enumerate(stats)}
            for i, a in enumerate(_operands(_LEFT, lambda _, r, c: h[r, c])):
                a_v[i, j, r0:r0 + 16, :] = a

    _skewed([(1, NB, lambda j: inv_std(opposite(j), 1, res_v, fa_v)),
             (0, NB, lambda j: statistic(opposite(j), 0, residual))], _in_turn, NT // 2)
    _skewed([(1, NB, lambda j: inv_std(opposite(j), 3, fb_v)),
             (0, NB, lambda j: statistic(opposite(j), 2, modulated))], _in_turn, NT // 2)
    lax.fori_loop(0, 4, mlp_operands, None)

    zero = pl.program_id(0)

    def weights(ref, top, height, left, width):
        def block(tag, r, c):
            rows = pl.ds(pl.multiple_of(top + r * height + 16 * tag * zero, 16), height)
            first = (left + c * width) // 128
            return jnp.concatenate([ref[t, rows, :].astype(f32)
                                    for t in range(first, first + width // 128)], axis=1)
        return _operands(_RIGHT, block)

    def hidden(j):
        lo, n = STARTS[j], CHUNKS[j] // 4
        bias = [jnp.concatenate([b1[t:t + 1, :] for t in range((lo + c * n) // 128,
                                                               (lo + c * n + n) // 128)], axis=1)
                for c in range(4)]
        return {(r, c): _gelu(u + bias[c]) for (r, c), u in _blocks(
            _dot(jnp.concatenate([a_v[i, t] for t in range(4)], axis=1), w)
            for i, w in enumerate(weights(w1_v, 0, SB, lo, n)))}

    def products(j, g):
        return enumerate(map(_dot, _operands(_LEFT, lambda _, r, c: g[r, c]),
                             weights(w2_v, STARTS[j], CHUNKS[j] // 4, 0, SB)))

    wait(cp_mlp[0])
    start(cp_mlp[2])
    b1, b2 = b1_v[...].astype(f32), b2_v[...].astype(f32)
    g0 = hidden(0)
    wait(cp_mlp[1])
    start(cp_mlp[3])
    g1 = hidden(1)
    for i, m in products(0, g0):
        acc_v[i] = m
    wait(cp_mlp[2])
    start(cp_mlp[4])
    g2 = hidden(2)
    wait(cp_mlp[3] + cp_mlp[4])
    for i, m in products(1, g1):
        acc_v[i] += m
    for (r, c), y in _blocks(acc_v[i] + m for i, m in products(2, g2)):
        rows = slice(HB * r, HB * (r + 1))
        gate = mod_v[5 * D + HB * r:5 * D + HB * (r + 1), :]
        for t in range(4 * c, 4 * c + 4):
            branch = y[:, _tile(t - 4 * c)] + b2[t:t + 1, :]
            half_v[t, rows, :] = (res_v[t, rows, :] + gate * branch).astype(bf16)
            pltpu.make_async_copy(
                half_v.at[t, rows], out_hbm.at[rows, _tile(t)], sem_out).start()
    pltpu.make_async_copy(out_hbm, out_hbm, sem_out).wait()


@jax.jit
def pallas_adaLN_cond__spectral_gfnet__mixer_token_mlp__prompt_kernel(
    A_x: jax.Array,
    A_w_r: jax.Array,
    A_w_i: jax.Array,
    B_x: jax.Array,
    B_w1: jax.Array,
    B_b1: jax.Array,
    B_w2: jax.Array,
    B_b2: jax.Array,
    c: jax.Array,
    w_mod: jax.Array,
):
    del B_x
    vmem = pltpu.VMEM
    scratch = [
        vmem((D, S), bf16), vmem((DF, S), bf16), vmem((DF, S), bf16),
        vmem((F // 128, S, 128), bf16), vmem((F // 128, 128), bf16),
        vmem((NT, F, 128), bf16), vmem((NT, 128), bf16),
        vmem((1, D), bf16), vmem((D, 6 * D), bf16),
        vmem(_CHANNEL_MATRICES.shape, u32), vmem(_TOKEN_SEEDS.shape, f32),
        vmem((6 * D, 128), f32),
        vmem((NT, 3, 128, 128), bf16),
        vmem((NT, 3, 128, 128), bf16),
        vmem((3, S + 128, 128), u32),
        vmem((NT, 8 * NRB, 128), u32),
        vmem((NT, D, 128), bf16),
        vmem((NT, 16 * NRB, 128), f32),
        vmem((NT, 16 * NRB, 128), f32),
        vmem((NT, D, 128), f32),
        vmem((4, NT, 8, 128), f32),
        vmem((49, 4, HB, 128), bf16),
        vmem((49, HB, SB), f32),
        pltpu.SemaphoreType.DMA((14,)),
    ]
    out = pl.pallas_call(
        _kernel,
        grid=(1,),
        in_specs=[pl.BlockSpec(memory_space=pl.ANY)] * 11,
        out_specs=pl.BlockSpec(memory_space=pl.ANY),
        out_shape=jax.ShapeDtypeStruct((D, S), bf16),
        scratch_shapes=scratch,
        compiler_params=pltpu.CompilerParams(vmem_limit_bytes=124 * 1024 * 1024),
    )(A_x.reshape(S, D).T, A_w_r.T, A_w_i.T, B_w1, B_b1.reshape(F // 128, 128), B_w2,
      B_b2.reshape(NT, 128), c, w_mod, _CHANNEL_MATRICES, _TOKEN_SEEDS)
    return out.T.reshape(1, S, D)
```
